```python
import jax
import jax.numpy as jnp

def _softmax(x, axis=-1):
    return jax.nn.softmax(x, axis=axis)

def _gelu(x):
    return jax.nn.gelu(x, approximate=True)

def _silu(x):
    return jax.nn.silu(x)

def _sigmoid(x):
    return jax.nn.sigmoid(x)

def _layernorm(x, axis=-1, eps=1e-05):
    m = jnp.mean(x, axis=axis, keepdims=True)
    v = jnp.var(x, axis=axis, keepdims=True)
    return (x - m) / jnp.sqrt(v + eps)

def _scatter_add(tgt, idx, src, axis=0):
    return tgt.at[idx].add(src)

def _segment_sum(src, seg, n):
    return jax.ops.segment_sum(src, seg, n)

class _Rng:

    def __init__(self, key):
        self._k = key

    def _next(self):
        self._k, sub = jax.random.split(self._k)
        return sub

    def normal(self, shape):
        return jax.random.normal(self._next(), shape, dtype=jnp.bfloat16)

    def randint(self, lo, hi, shape):
        return jax.random.randint(self._next(), shape, lo, hi, dtype=jnp.int32)

    def uniform(self, shape, lo=0.0, hi=1.0):
        return jax.random.uniform(self._next(), shape, jnp.bfloat16, lo, hi)

    def permutation(self, n):
        return jax.random.permutation(self._next(), n)
kernel_name = 'adaLN_cond__compressed_kv_cla__mixer_s_mlp__prompt'

def setup_inputs():
    _rng = _Rng(jax.random.key(int.from_bytes(__import__("os").urandom(4), "little")))
    _w = lambda a: (lambda t: t.astype(jnp.bfloat16) if jnp.issubdtype(t.dtype, jnp.floating) else t)(jnp.asarray(a))

    def _A_setup():
        B, H, Sq, Sk, D, M = (1, 32, 2048, 2048, 128, 640)
        Dc = 4 * D
        return {'x': _w((lambda *s: _rng.normal(s) * 0.05)(B, Sq, M)), 'c_kv': _w((lambda *s: _rng.normal(s) * 0.05)(B, Sk, Dc)), 'w_q': _w((lambda *s: _rng.normal(s) * 0.05)(M, H, D) * M ** (-0.5)), 'w_uk': _w((lambda *s: _rng.normal(s) * 0.05)(Dc, H, D) * Dc ** (-0.5)), 'w_uv': _w((lambda *s: _rng.normal(s) * 0.05)(Dc, H, D) * Dc ** (-0.5)), 'w_o': _w((lambda *s: _rng.normal(s) * 0.05)(H, D, M) * (H * D) ** (-0.5))}
    _A_in = _A_setup()

    def _B_setup():
        B, S, D, F = (1, 2048, 640, 1728)
        return {'x': _w((lambda *s: _rng.normal(s) * 0.05)(B, S, D)), 'w1': _w((lambda *s: _rng.normal(s) * 0.05)(D, D) * D ** (-0.5)), 'w2': _w((lambda *s: _rng.normal(s) * 0.05)(D, D) * D ** (-0.5)), 'w3': _w((lambda *s: _rng.normal(s) * 0.05)(D, F) * D ** (-0.5)), 'w4': _w((lambda *s: _rng.normal(s) * 0.05)(F, D) * F ** (-0.5))}
    _B_in = _B_setup()
    return {'A_x': _A_in['x'], 'A_c_kv': _A_in['c_kv'], 'A_w_q': _A_in['w_q'], 'A_w_uk': _A_in['w_uk'], 'A_w_uv': _A_in['w_uv'], 'A_w_o': _A_in['w_o'], 'B_x': _B_in['x'], 'B_w1': _B_in['w1'], 'B_w2': _B_in['w2'], 'B_w3': _B_in['w3'], 'B_w4': _B_in['w4'], 'c': _w((lambda *s: _rng.normal(s) * 0.05)(1, 640)), 'w_mod': _w((lambda *s: _rng.normal(s) * 0.05)(640, 6 * 640) * 640 ** (-0.5))}

def reference(A_x, A_c_kv, A_w_q, A_w_uk, A_w_uv, A_w_o, B_x, B_w1, B_w2, B_w3, B_w4, c, w_mod):

    def _A_ref(x, c_kv, w_q, w_uk, w_uv, w_o):
        B, Sq, M = (x.shape[0], x.shape[1], x.shape[2])
        Sk = c_kv.shape[1]
        H, D = (w_q.shape[1], w_q.shape[2])
        q = jnp.einsum('bqm,mhd->bhqd', x, w_q)
        k = jnp.einsum('bkc,chd->bhkd', c_kv, w_uk)
        v = jnp.einsum('bkc,chd->bhkd', c_kv, w_uv)
        scores = jnp.einsum('bhqd,bhkd->bhqk', q, k) * D ** (-0.5)
        off = Sk - Sq
        qi = jnp.arange(Sq)[:, None]
        kj = jnp.arange(Sk)[None, :]
        cmask = kj <= qi + off
        scores = jnp.where(cmask[None, None], scores, -1000000000.0)
        p = _softmax(scores, axis=-1)
        ctx = jnp.einsum('bhqk,bhkd->bhqd', p, v)
        return jnp.einsum('bhqd,hdm->bqm', ctx, w_o)

    def _B_ref(x, w1, w2, w3, w4):
        B, S, D = x.shape
        h = _gelu(_layernorm(x, axis=-1) @ w1)
        c = D // 4
        g0 = jnp.pad(h[:, :, 0 * c:1 * c], ((0, 0), (1, 0), (0, 0)))[:, :S, :]
        g1 = jnp.pad(h[:, :, 1 * c:2 * c], ((0, 0), (0, 1), (0, 0)))[:, 1:, :]
        g2 = jnp.pad(h[:, :, 2 * c:3 * c], ((0, 0), (2, 0), (0, 0)))[:, :S, :]
        g3 = jnp.pad(h[:, :, 3 * c:], ((0, 0), (0, 2), (0, 0)))[:, 2:, :]
        hs = jnp.concatenate([g0, g1, g2, g3], axis=-1) @ w2
        x1 = x + hs
        h2 = _gelu(_layernorm(x1, axis=-1) @ w3) @ w4
        return x1 + h2
    x = A_x
    mod = (_silu(c) @ w_mod).reshape(c.shape[0], 6, 1, -1)
    sa, ca, ga, sb, cb, gb = (mod[:, 0].copy(), mod[:, 1].copy(), mod[:, 2].copy(), mod[:, 3].copy(), mod[:, 4].copy(), mod[:, 5].copy())
    h = _layernorm(x, axis=-1) * (1 + ca) + sa
    x = x + ga * _A_ref(h, A_c_kv, A_w_q, A_w_uk, A_w_uv, A_w_o)
    h = _layernorm(x, axis=-1) * (1 + cb) + sb
    x = x + gb * _B_ref(h, B_w1, B_w2, B_w3, B_w4)
    return x
```

```python
import functools
import jax
import jax.numpy as jnp
import numpy as np
from jax.experimental import pallas as pl
from jax.experimental.pallas import tpu as pltpu

S = 2048; M = 640; H = 32; D = 128; DC = 512; F = 1728
NP = H // 2
EPS = 1e-5
LOG2E = 1.4426950408889634
QSCALE = float(D ** -0.5 * LOG2E)
NEG = -1e30
bf16 = jnp.bfloat16; f32 = jnp.float32


def _ln(x):
    m = jnp.mean(x, axis=-1, keepdims=True)
    xc = x - m
    v = jnp.mean(xc * xc, axis=-1, keepdims=True)
    return xc * jax.lax.rsqrt(v + EPS)


def _gelu(x):
    c = 0.7978845608028654
    return 0.5 * x * (1.0 + jnp.tanh(c * (x + 0.044715 * (x * x * x))))


def _rcp(l):
    r = pl.reciprocal(l, approx=True)
    return r * (2.0 - l * r)


def _dot(a, b):
    return jnp.dot(a, b, preferred_element_type=f32)


def _unpack_pair(w32):
    lo = pltpu.bitcast(w32 << 16, f32).astype(bf16)
    hi = pltpu.bitcast(w32 & jnp.uint32(0xFFFF0000), f32).astype(bf16)
    return lo, hi


def make_kernel(cfg):
    TQ = cfg.get("TQ", 128)
    PR = cfg.get("PR", 128)
    TM = cfg.get("TM", 256)
    NB = S // TM

    def kernel(x_hbm, ckv_hbm, wq_hbm, wuk_hbm, wuv_hbm, wo_hbm, w1_hbm, w2_hbm, w3_hbm, w4_hbm, c_ref, wmod_hbm,
               out_hbm,
               x_v, ckv_v, h_v, wmod_v, wq32, wk32, wv32, wq_s, wk_s, wv_s, q_v, kT_v, v_v, ctx_v,
               wo_v, w1_v, w2_v, w3_v, w4_v, u_v, x1_v, h2_v, o_v, sem, wsem, osem):
        def cp(src, dst, i):
            return pltpu.make_async_copy(src, dst, sem.at[i])

        def wcopies(g, slot):
            return (pltpu.make_async_copy(wq_hbm.bitcast(jnp.uint32).at[:, g, :], wq32.at[slot], wsem.at[0, slot]),
                    pltpu.make_async_copy(wuk_hbm.bitcast(jnp.uint32).at[:, g, :], wk32.at[slot], wsem.at[1, slot]),
                    pltpu.make_async_copy(wuv_hbm.bitcast(jnp.uint32).at[:, g, :], wv32.at[slot], wsem.at[2, slot]))

        c_ckv = cp(ckv_hbm, ckv_v, 0); c_x = cp(x_hbm, x_v, 2)
        c_wma = cp(wmod_hbm.at[:, 0:2 * M], wmod_v.at[:, 0:2 * M], 1)
        c_wmb = cp(wmod_hbm.at[:, 2 * M:6 * M], wmod_v.at[:, 2 * M:6 * M], 8)
        w0 = wcopies(0, 0)
        w0[1].start(); w0[2].start(); c_ckv.start()
        c_wma.start(); c_x.start(); w0[0].start()
        late = [cp(wo_hbm, wo_v, 3), cp(w1_hbm, w1_v, 4), cp(w2_hbm, w2_v, 5), cp(w3_hbm, w3_v, 6), cp(w4_hbm, w4_v, 7), c_wmb]

        def proj_kv(bs, r0):
            rows = slice(r0, r0 + PR)
            c = ckv_v[rows, :]
            k = _dot(c, wk_s[...])
            for hh in range(2):
                for t in range(PR // 128):
                    kT_v[bs, hh, (r0 // 128) + t] = k[t * 128:(t + 1) * 128, hh * 128:(hh + 1) * 128].T.astype(bf16)
            v = _dot(c, wv_s[...]).astype(bf16)
            v_v[bs, 0, rows, :] = v[:, :128]; v_v[bs, 1, rows, :] = v[:, 128:]

        def proj_q(bs, r0):
            rows = slice(r0, r0 + PR)
            q = (_dot(h_v[rows, :], wq_s[...]) * QSCALE).astype(bf16)
            q_v[bs, 0, rows, :] = q[:, :128]; q_v[bs, 1, rows, :] = q[:, 128:]

        def proj_piece(ws, bs, r0):
            proj_kv(bs, r0); proj_q(bs, r0)

        def relayout(ws, which=(0, 1, 2)):
            for src, dst in [((wk32, wk_s), (wv32, wv_s), (wq32, wq_s))[i] for i in which]:
                lo, hi = _unpack_pair(src[ws])
                dst[:, 0:128] = lo
                dst[:, 128:256] = hi

        tri = jax.lax.broadcasted_iota(jnp.int32, (128, 128), 1) <= jax.lax.broadcasted_iota(jnp.int32, (128, 128), 0)

        def qk(bs, hh, i):
            r0 = i * TQ; nt = i + 1
            q = q_v[bs, hh, r0:r0 + TQ, :]
            tiles = [_dot(q, kT_v[bs, hh, t]) for t in range(nt)]
            tiles[-1] = jnp.where(tri, tiles[-1], NEG)
            mx = tiles[0]
            for t in tiles[1:]:
                mx = jnp.maximum(mx, t)
            m = jnp.max(mx, axis=1, keepdims=True)
            return tiles, m

        def smpv(bs, g, hh, i, st):
            tiles, m = st
            r0 = i * TQ
            acc = None; ls = None
            for t, s in enumerate(tiles):
                p = jnp.exp2(s - m)
                ls = p if ls is None else ls + p
                o = _dot(p.astype(bf16), v_v[bs, hh, t * 128:(t + 1) * 128, :])
                acc = o if acc is None else acc + o
            l = jnp.sum(ls, axis=1, keepdims=True)
            ctx_v[2 * g + hh, r0:r0 + TQ, :] = (acc * _rcp(l)).astype(bf16)

        def attention(bs, g, ws_next=None):
            items = [(hh, i) for hh in range(2) for i in (range(S // TQ) if not cfg.get('REV') else reversed(range(S // TQ)))]
            npieces = S // PR
            every = len(items) // npieces
            st = qk(bs, *items[0])
            for n, it in enumerate(items):
                nxt = qk(bs, *items[n + 1]) if n + 1 < len(items) else None
                smpv(bs, g, *it, st)
                st = nxt
                if ws_next is not None and n % every == cfg.get("POFF", 0):
                    proj_piece(ws_next, 1 - bs, (n // every) * PR)

        w0[1].wait(); w0[2].wait()
        relayout(0, (0, 1))
        c_ckv.wait()
        for r in range(S // PR):
            proj_kv(0, r * PR)
        for d in wcopies(1, 1): d.start()
        c_wma.wait()
        cc = c_ref[...].astype(f32)
        sc = (cc * jax.nn.sigmoid(cc)).astype(bf16)
        sc8 = jnp.broadcast_to(sc, (8, M))
        moda = _dot(sc8, wmod_v[:, 0:2 * M])
        sa = moda[0:1, 0:M]; ca1 = 1.0 + moda[0:1, M:2 * M]
        c_x.wait()
        w0[0].wait()
        relayout(0, (2,))
        LR = cfg.get("LR", 64)
        for r in range(S // PR):
            for rr in range(r * PR, (r + 1) * PR, LR):
                rows = slice(rr, rr + LR)
                h_v[rows, :] = (_ln(x_v[rows, :].astype(f32)) * ca1 + sa).astype(bf16)
            proj_q(0, r * PR)
        for d in late: d.start()

        def body(g, carry):
            bs = g % 2
            ws = (g + 1) % 2
            if not cfg.get("NODMA"):
                for d in wcopies(g + 1, ws): d.wait()

                @pl.when(g + 2 < cfg.get('NIT', NP - 1) + 1)
                def _():
                    for d in wcopies(g + 2, bs): d.start()
            relayout(ws)
            attention(bs, g, ws)
            return carry
        jax.lax.fori_loop(0, cfg.get('NIT', NP - 1), body, 0)
        attention(cfg.get('NIT', NP - 1) % 2, NP - 1, None)

        for d in late: d.wait()
        modb = _dot(sc8, wmod_v[:, 2 * M:6 * M])
        ga = modb[0:1, 0:M]; sb = modb[0:1, M:2 * M]; cb1 = 1.0 + modb[0:1, 2 * M:3 * M]; gb = modb[0:1, 3 * M:4 * M]
        zero8 = jnp.zeros((8, M), f32)
        u_v[0:8, :] = zero8; u_v[8 + S:16 + S, :] = zero8
        lane = jax.lax.broadcasted_iota(jnp.int32, (TM, 128), 1)

        def A1(r, slot):
            r0 = pl.multiple_of(r * TM, TM)
            cx = jnp.concatenate([ctx_v[hh, pl.ds(r0, TM), :] for hh in range(H)], axis=1)
            return _dot(cx, wo_v[...])

        def A2(r, slot, a):
            r0 = pl.multiple_of(r * TM, TM)
            outs = []
            for rr in range(0, TM, LR):
                x1 = x_v[pl.ds(r0 + rr, LR), :].astype(f32) + ga * a[rr:rr + LR]
                h2 = _ln(x1) * cb1 + sb
                x1_v[slot, rr:rr + LR, :] = x1; h2_v[slot, rr:rr + LR, :] = h2
                outs.append(_ln(h2).astype(bf16))
            return jnp.concatenate(outs, axis=0)

        def A3(r, slot, l2):
            r0 = pl.multiple_of(r * TM, TM)
            u_v[pl.ds(r0 + 8, TM), :] = _gelu(_dot(l2, w1_v[...]))

        def B1(r, slot):
            r0 = pl.multiple_of(r * TM, TM)
            def sh(delta, j):
                win = u_v[pl.ds(r0, TM + 16), j * 128:(j + 1) * 128]
                return win[8 + delta:8 + delta + TM]
            t0 = sh(-1, 0)
            t1 = jnp.where(lane < 32, sh(-1, 1), sh(1, 1))
            t2 = jnp.where(lane < 64, sh(1, 2), sh(-2, 2))
            t3 = jnp.where(lane < 96, sh(-2, 3), sh(2, 3))
            t4 = sh(2, 4)
            return jnp.concatenate([t0, t1, t2, t3, t4], axis=1).astype(bf16)

        def B2(r, slot, us):
            return _dot(us, w2_v[...])

        def B3(r, slot, hs):
            outs = []
            for rr in range(0, TM, LR):
                xb1 = h2_v[slot, rr:rr + LR, :] + hs[rr:rr + LR]
                h2_v[slot, rr:rr + LR, :] = xb1
                outs.append(_ln(xb1).astype(bf16))
            return jnp.concatenate(outs, axis=0)

        def B4(r, slot, l3):
            return _gelu(jax.lax.dot_general(l3, w3_v[...], (((1,), (1,)), ((), ())), preferred_element_type=f32)).astype(bf16)

        def B5(r, slot, gg):
            y = _dot(gg, w4_v[...])
            o_v[slot] = (x1_v[slot] + gb * (h2_v[slot] + y)).astype(bf16)

        def ocopy(r, slot):
            r0 = pl.multiple_of(r * TM, TM)
            return pltpu.make_async_copy(o_v.at[slot], out_hbm.at[pl.ds(r0, TM)], osem.at[slot])

        A3(0, 0, A2(0, 0, A1(0, 0)))

        def fbody(r, carry):
            slot = r % 2

            @pl.when(r >= 2)
            def _():
                ocopy(r - 2, slot).wait()
            us = B1(r, slot)
            a = A1(r + 1, 1 - slot)
            hs = B2(r, slot, us)
            l2 = A2(r + 1, 1 - slot, a)
            A3(r + 1, 1 - slot, l2)
            l3 = B3(r, slot, hs)
            gg = B4(r, slot, l3)
            B5(r, slot, gg)
            ocopy(r, slot).start()
            return carry
        NBB = cfg.get('FIT', NB - 1) + 1
        jax.lax.fori_loop(0, NBB - 1, fbody, 0)
        ocopy(NBB - 3, (NBB - 1) % 2).wait()
        sl = (NBB - 1) % 2
        B5(NBB - 1, sl, B4(NBB - 1, sl, B3(NBB - 1, sl, B2(NBB - 1, sl, B1(NBB - 1, sl)))))
        ocopy(NBB - 1, sl).start()
        ocopy(NBB - 2, (NBB - 2) % 2).wait()
        ocopy(NBB - 1, sl).wait()

    return kernel


def build(cfg):
    TM = cfg.get("TM", 256)
    any_spec = pl.BlockSpec(memory_space=pltpu.MemorySpace.HBM)
    scratch = [
        pltpu.VMEM((S, M), bf16),
        pltpu.VMEM((S, DC), bf16),
        pltpu.VMEM((S, M), bf16),
        pltpu.VMEM((M, 6 * M), bf16),
        pltpu.VMEM((2, M, D), jnp.uint32),
        pltpu.VMEM((2, DC, D), jnp.uint32),
        pltpu.VMEM((2, DC, D), jnp.uint32),
        pltpu.VMEM((M, 256), bf16), pltpu.VMEM((DC, 256), bf16), pltpu.VMEM((DC, 256), bf16),
        pltpu.VMEM((2, 2, S, D), bf16),
        pltpu.VMEM((2, 2, S // 128, D, 128), bf16),
        pltpu.VMEM((2, 2, S, D), bf16),
        pltpu.VMEM((H, S, D), bf16),
        pltpu.VMEM((H * D, M), bf16),
        pltpu.VMEM((M, M), bf16), pltpu.VMEM((M, M), bf16), pltpu.VMEM((F, M), bf16), pltpu.VMEM((F, M), bf16),
        pltpu.VMEM((S + 16, M), f32),
        pltpu.VMEM((2, TM, M), f32), pltpu.VMEM((2, TM, M), f32), pltpu.VMEM((2, TM, M), bf16),
        pltpu.SemaphoreType.DMA((9,)), pltpu.SemaphoreType.DMA((3, 2)), pltpu.SemaphoreType.DMA((2,)),
    ]
    return pl.pallas_call(
        make_kernel(cfg),
        out_shape=jax.ShapeDtypeStruct((S, M), bf16),
        in_specs=[any_spec] * 10 + [pl.BlockSpec(memory_space=pltpu.VMEM), any_spec],
        out_specs=any_spec,
        scratch_shapes=scratch,
        compiler_params=pltpu.CompilerParams(vmem_limit_bytes=cfg.get("VMEM", 110) * 2**20),
        name="fused_block",
    )


def run(cfg, A_x, A_c_kv, A_w_q, A_w_uk, A_w_uv, A_w_o, B_x, B_w1, B_w2, B_w3, B_w4, c, w_mod):
    out = build(cfg)(A_x.reshape(S, M), A_c_kv.reshape(S, DC), A_w_q, A_w_uk, A_w_uv, A_w_o.reshape(H * D, M),
                     B_w1, B_w2, B_w3.T, B_w4, c, w_mod)
    return out.reshape(1, S, M)


_CFG = {'REV': 1, 'POFF': 1}


@jax.jit
def pallas_adaLN_cond__compressed_kv_cla__mixer_s_mlp__prompt_kernel(A_x, A_c_kv, A_w_q, A_w_uk, A_w_uv, A_w_o, B_x, B_w1, B_w2, B_w3, B_w4, c, w_mod):
    return run(_CFG, A_x, A_c_kv, A_w_q, A_w_uk, A_w_uv, A_w_o, B_x, B_w1, B_w2, B_w3, B_w4, c, w_mod)
```

```python
import functools
import jax
import jax.numpy as jnp
import numpy as np
from jax.experimental import pallas as pl
from jax.experimental.pallas import tpu as pltpu

S = 2048; M = 640; H = 32; D = 128; DC = 512; F = 1728
NP = H // 2
EPS = 1e-5
LOG2E = 1.4426950408889634
QSCALE = float(D ** -0.5 * LOG2E)
NEG = -1e30
bf16 = jnp.bfloat16; f32 = jnp.float32


def _ln(x):
    m = jnp.mean(x, axis=-1, keepdims=True)
    xc = x - m
    v = jnp.mean(xc * xc, axis=-1, keepdims=True)
    return xc * jax.lax.rsqrt(v + EPS)


def _gelu(x):
    c = 0.7978845608028654
    return 0.5 * x * (1.0 + jnp.tanh(c * (x + 0.044715 * (x * x * x))))


def _rcp(l):
    r = pl.reciprocal(l, approx=True)
    return r * (2.0 - l * r)


def _dot(a, b):
    return jnp.dot(a, b, preferred_element_type=f32)


def _unpack_pair(w32):
    lo = pltpu.bitcast(w32 << 16, f32).astype(bf16)
    hi = pltpu.bitcast(w32 & jnp.uint32(0xFFFF0000), f32).astype(bf16)
    return lo, hi


def make_kernel(cfg):
    TQ = 128
    PR = cfg.get("PR", 128)
    TM = cfg.get("TM", 256)
    LR = cfg.get("LR", 64)
    NB = S // TM
    NCK = cfg.get("NCK", 4)

    import contextlib
    def sc_(name):
        on = cfg.get("SCOPE")
        if isinstance(on, str): on = name in on.split(",")
        return jax.named_scope(name) if on else contextlib.nullcontext()

    U32 = cfg.get("U32", "")
    def st_(val, key):
        return pltpu.bitcast(val, jnp.uint32) if key in U32 else val
    def ld_(val, key):
        return pltpu.bitcast(val, bf16) if key in U32 else val
    def rs_(r0, n, key):
        return slice(r0 // 2, (r0 + n) // 2) if key in U32 else slice(r0, r0 + n)

    def kernel(x_hbm, ckv_hbm, wq_hbm, wuk_hbm, wuv_hbm, wo_hbm, w1_hbm, w2_hbm, w3_hbm, w4_hbm, c_ref, wmod_hbm,
               out_hbm,
               x_v, ckv_v, h_v, wmod_v, mod_v, wq32, wk32, wv32, wq_s, wk_s, wv_s, q_v, kT_v, v_v, ctx_v,
               wo_v, w1_v, w2_v, w3_v, w4_v, u_v, x1_v, h2_v, o_v, sem, ksem, wsem, osem):
        def cp(src, dst, i):
            return pltpu.make_async_copy(src, dst, sem.at[i])

        def wkcopy(g):
            return pltpu.make_async_copy(wuk_hbm.bitcast(jnp.uint32).at[:, g, :], wk32.at[g], ksem.at[g])

        def wcopies(g, slot):
            return (pltpu.make_async_copy(wq_hbm.bitcast(jnp.uint32).at[:, g, :], wq32.at[slot], wsem.at[0, slot]),
                    pltpu.make_async_copy(wuv_hbm.bitcast(jnp.uint32).at[:, g, :], wv32.at[slot], wsem.at[1, slot]))

        CR = S // NCK
        c_ckv = [cp(ckv_hbm.at[j * CR:(j + 1) * CR], ckv_v.at[j * CR:(j + 1) * CR], j) for j in range(NCK)]
        c_x = cp(x_hbm, x_v, 8); c_wmod = cp(wmod_hbm, wmod_v, 9)
        late = [cp(wo_hbm, wo_v, 10), cp(w1_hbm, w1_v, 11), cp(w2_hbm, w2_v, 12), cp(w3_hbm, w3_v, 13), cp(w4_hbm, w4_v, 14)]
        wkcopy(0).start(); c_ckv[0].start()
        if cfg.get("ST", 0) == 0:
            for j in range(1, NCK): c_ckv[j].start()
            wkcopy(1).start(); wkcopy(2).start()

        AL = cfg.get("AL", "")
        def vref(bs, hh):
            return ctx_v.at[H + 2 * bs + hh] if "v" in AL else v_v.at[bs, hh]
        def wq_load():
            if "c" in AL:
                return jnp.concatenate([ctx_v[H + 4, 0:M, :], ctx_v[H + 4, M:2 * M, :]], axis=1)
            return wq_s[...]
        def relayout_q(src):
            if "c" in AL:
                lo, hi = _unpack_pair(src[...])
                ctx_v[H + 4, 0:M, :] = lo
                ctx_v[H + 4, M:2 * M, :] = hi
            else:
                relayout(src, wq_s)

        def relayout(src, dst):
            lo, hi = _unpack_pair(src[...])
            dst[:, 0:128] = lo
            dst[:, 128:256] = hi

        def proj_k(g, par, r0):
            rows = slice(r0, r0 + PR)
            k = _dot(ckv_v[rows, :], wk_s[par])
            for hh in range(2):
                for t in range(PR // 128):
                    kT_v[2 * g + hh, (r0 // 128) + t] = st_(k[t * 128:(t + 1) * 128, hh * 128:(hh + 1) * 128].T.astype(bf16), "k")

        def proj_v(bs, r0):
            rows = slice(r0, r0 + PR)
            v = _dot(ckv_v[rows, :], wv_s[...]).astype(bf16)
            for hh in range(2): vref(bs, hh)[rs_(r0, PR, "v"), :] = st_(v[:, hh * 128:(hh + 1) * 128], "v")

        def proj_q(bs, r0):
            rows = slice(r0, r0 + PR)
            q = (_dot(h_v[rows, :], wq_load()) * QSCALE).astype(bf16)
            for hh in range(2): q_v[bs, hh, rs_(r0, PR, "q"), :] = st_(q[:, hh * 128:(hh + 1) * 128], "q")

        LAG = cfg.get("LAG", 0)
        tri = jax.lax.broadcasted_iota(jnp.int32, (128, 128), 1) <= jax.lax.broadcasted_iota(jnp.int32, (128, 128), 0)

        def qk(bs, g, hh, i):
            r0 = i * TQ; nt = i + 1
            q = ld_(q_v[bs, hh, rs_(r0, TQ, "q"), :], "q")
            tiles = [_dot(q, ld_(kT_v[2 * g + hh, t], "k")) for t in range(nt)]
            tiles[-1] = jnp.where(tri, tiles[-1], NEG)
            mx = tiles[0]
            for t in tiles[1:]:
                mx = jnp.maximum(mx, t)
            m = jnp.max(mx, axis=1, keepdims=True)
            return tiles, m

        def smpv(bs, g, hh, i, st):
            tiles, m = st
            r0 = i * TQ
            acc = None; ls = None
            for t, s in enumerate(tiles):
                p = jnp.exp2(s - m)
                ls = p if ls is None else ls + p
                o = _dot(p.astype(bf16), ld_(vref(bs, hh)[rs_(t * 128, 128, "v"), :], "v"))
                acc = o if acc is None else acc + o
            def fin():
                l = jnp.sum(ls, axis=1, keepdims=True)
                ctx_v[2 * g + hh, r0:r0 + TQ, :] = (acc * _rcp(l)).astype(bf16)
            return fin

        def attention(bs, g, items, pieces):
            st = qk(bs, g, *items[0])
            pend = []
            for n, it in enumerate(items):
                nxt = qk(bs, g, *items[n + 1]) if n + 1 < len(items) else None
                pend.append(smpv(bs, g, *it, st))
                if len(pend) > LAG:
                    pend.pop(0)()
                st = nxt
                if n in pieces:
                    if pieces[n][0] == "flush":
                        for f in pend: f()
                        pend = []
                    for f in pieces[n]:
                        if f != "flush": f()
            for f in pend: f()

        NI = S // TQ
        items_rev = [(hh, i) for hh in range(2) for i in reversed(range(NI))]

        def do_mod():
            c_wmod.wait()
            cc = c_ref[...].astype(f32)
            sc = (cc * jax.nn.sigmoid(cc)).astype(bf16)
            mod_v[...] = _dot(jnp.broadcast_to(sc, (8, M)), wmod_v[...])

        def do_h(rr):
            rows = slice(rr, rr + LR)
            h_v[rows, :] = (_ln(x_v[rows, :].astype(f32)) * (1.0 + mod_v[0:1, M:2 * M]) + mod_v[0:1, 0:M]).astype(bf16)

        def kpair(g, par, nxt, first=False):
            for r in range(S // PR):
                if first and (r * PR) % CR == 0:
                    c_ckv[(r * PR) // CR].wait()
                proj_k(g, par, r * PR)
                if r == cfg.get("RLP", 8):
                    if first:
                        wkcopy(1).wait()
                        for g2 in range(3, NP): wkcopy(g2).start()
                    relayout(wk32.at[nxt], wk_s.at[1 - par])

        with sc_("s1_kphase"):
          with sc_("s1_wait0"):
            wkcopy(0).wait()
          if cfg.get("ST", 0) == 1:
            for j in range(1, NCK): c_ckv[j].start()
            wkcopy(1).start(); wkcopy(2).start()
          relayout(wk32.at[0], wk_s.at[0])
          kpair(0, 0, 1, first=True)
          wkcopy(2).wait()
          kpair(1, 1, 2)

          def kbody(j, carry):
            g = 2 * j
            wkcopy(g + 1).wait()

            @pl.when(g + 2 < NP)
            def _():
                wkcopy(g + 2).wait()

            @pl.when(j == 1)
            def _():
                c_x.start(); c_wmod.start()
            kpair(g, 0, g + 1)
            kpair(g + 1, 1, jnp.minimum(g + 2, NP - 1))
            return carry
          with sc_("s1_kloop"):
            jax.lax.fori_loop(1, NP // 2, kbody, 0)

        with sc_("s2_vq0"):
            for d in wcopies(0, 0): d.start()
            for d in wcopies(1, 1): d.start()
            do_mod()
            for d in wcopies(0, 0): d.wait()
            c_x.wait()
            relayout(wv32.at[0], wv_s); relayout_q(wq32.at[0])
            for r in range(S // PR):
                proj_v(0, r * PR)
                for rr in range(r * PR, (r + 1) * PR, LR): do_h(rr)
                if r > 0: proj_q(0, (r - 1) * PR)
            proj_q(0, S - PR)

        for d in late: d.start()
        def body(g, carry):
            bs = g & 1
            ws = 1 - bs
            for d in wcopies(jnp.minimum(g + 2, NP - 1), bs): d.start()
            with sc_("sj_wait"):
                for d in wcopies(g + 1, ws): d.wait()
            with sc_("sk_relay"):
                relayout(wv32.at[ws], wv_s); relayout_q(wq32.at[ws])
            npieces = S // PR
            its = items_rev if cfg.get("REV", 1) == 1 else ([(hh, i) for hh in range(2) for i in range(NI)] if cfg.get("REV") == 0 else
                  [(0, i) for i in reversed(range(NI))] + [(1, i) for i in range(NI)])
            every = len(items_rev) // npieces
            pieces = {}
            for k in range(npieces):
                pieces[k * every + cfg.get("POFF", 1)] = [functools.partial(proj_v, ws, k * PR), functools.partial(proj_q, ws, k * PR)]
            with sc_("si_iter"):
                attention(bs, g, its, pieces)
            return carry
        with sc_("s5_main"):
            jax.lax.fori_loop(0, NP - 1, body, 0)
        for d in wcopies(NP - 1, (NP - 2) % 2): d.wait()

        for d in late: d.wait()
        zero8 = jnp.zeros((8, M), f32)
        u_v[0:8, :] = zero8; u_v[8 + S:16 + S, :] = zero8
        lane = jax.lax.broadcasted_iota(jnp.int32, (TM, 128), 1)
        def modv(j): return mod_v[0:1, j * M:(j + 1) * M]

        def A1(r, slot):
            r0 = pl.multiple_of(r * TM, TM)
            cx = jnp.concatenate([ctx_v[hh, pl.ds(r0, TM), :] for hh in range(H)], axis=1)
            return _dot(cx, wo_v[...])

        def A2(r, slot, a):
            r0 = pl.multiple_of(r * TM, TM)
            outs = []
            for rr in range(0, TM, LR):
                x1 = x_v[pl.ds(r0 + rr, LR), :].astype(f32) + modv(2) * a[rr:rr + LR]
                h2 = _ln(x1) * (1.0 + modv(4)) + modv(3)
                x1_v[slot, rr:rr + LR, :] = x1; h2_v[slot, rr:rr + LR, :] = h2
                outs.append(_ln(h2).astype(bf16))
            return jnp.concatenate(outs, axis=0)

        def A3(r, slot, l2):
            r0 = pl.multiple_of(r * TM, TM)
            u_v[pl.ds(r0 + 8, TM), :] = _gelu(_dot(l2, w1_v[...]))

        def B1(r, slot):
            r0 = pl.multiple_of(r * TM, TM)
            def sh(delta, j):
                win = u_v[pl.ds(r0, TM + 16), j * 128:(j + 1) * 128]
                return win[8 + delta:8 + delta + TM]
            t0 = sh(-1, 0)
            t1 = jnp.where(lane < 32, sh(-1, 1), sh(1, 1))
            t2 = jnp.where(lane < 64, sh(1, 2), sh(-2, 2))
            t3 = jnp.where(lane < 96, sh(-2, 3), sh(2, 3))
            t4 = sh(2, 4)
            return jnp.concatenate([t0, t1, t2, t3, t4], axis=1).astype(bf16)

        def B2(r, slot, us):
            return _dot(us, w2_v[...])

        def B3(r, slot, hs):
            outs = []
            for rr in range(0, TM, LR):
                xb1 = h2_v[slot, rr:rr + LR, :] + hs[rr:rr + LR]
                h2_v[slot, rr:rr + LR, :] = xb1
                outs.append(_ln(xb1).astype(bf16))
            return jnp.concatenate(outs, axis=0)

        def B4(r, slot, l3):
            return _gelu(jax.lax.dot_general(l3, w3_v[...], (((1,), (1,)), ((), ())), preferred_element_type=f32)).astype(bf16)

        def B5(r, slot, gg):
            y = _dot(gg, w4_v[...])
            o_v[slot] = (x1_v[slot] + modv(5) * (h2_v[slot] + y)).astype(bf16)

        def ocopy(r, slot):
            r0 = pl.multiple_of(r * TM, TM)
            return pltpu.make_async_copy(o_v.at[slot], out_hbm.at[pl.ds(r0, TM)], osem.at[slot])

        with sc_("s6_attn_last"):
            nf = TM // TQ
            if cfg.get("FUSEA0", 1):
                items = [(hh, i) for hh in range(2) for i in range(nf)] + [(hh, i) for hh in range(2) for i in reversed(range(nf, NI))]
                st = {}
                n0 = 2 * nf + cfg.get("A0POS", 1)
                pieces = {n0: ["flush", lambda: st.__setitem__("a", A1(0, 0))],
                          n0 + cfg.get("A0D", 4): [lambda: A3(0, 0, A2(0, 0, st["a"]))]}
                attention((NP - 1) % 2, NP - 1, items, pieces)
            else:
                attention((NP - 1) % 2, NP - 1, items_rev, {})
                A3(0, 0, A2(0, 0, A1(0, 0)))

        def fbody(r, carry):
            slot = r & 1

            @pl.when(r >= 2)
            def _():
                ocopy(r - 2, slot).wait()
            us = B1(r, slot)
            a = A1(r + 1, 1 - slot)
            hs = B2(r, slot, us)
            l2 = A2(r + 1, 1 - slot, a)
            A3(r + 1, 1 - slot, l2)
            l3 = B3(r, slot, hs)
            gg = B4(r, slot, l3)
            B5(r, slot, gg)
            ocopy(r, slot).start()
            return carry
        with sc_("s8_floop"):
            jax.lax.fori_loop(0, NB - 1, fbody, 0)
        ocopy(NB - 3, (NB - 1) % 2).wait()
        sl = (NB - 1) % 2
        with sc_("s9_Blast"):
            B5(NB - 1, sl, B4(NB - 1, sl, B3(NB - 1, sl, B2(NB - 1, sl, B1(NB - 1, sl)))))
        with sc_("sa_outwait"):
            ocopy(NB - 1, sl).start()
            ocopy(NB - 2, (NB - 2) % 2).wait()
            ocopy(NB - 1, sl).wait()

    return kernel


def build(cfg):
    TM = cfg.get("TM", 256)
    hbm = pl.BlockSpec(memory_space=pltpu.MemorySpace.HBM)
    def hv(shape, key):
        if key in cfg.get("U32", ""):
            return pltpu.VMEM(shape[:-2] + (shape[-2] // 2, shape[-1]), jnp.uint32)
        return pltpu.VMEM(shape, bf16)
    scratch = [
        pltpu.VMEM((S, M), bf16),
        pltpu.VMEM((S, DC), bf16),
        pltpu.VMEM((S, M), bf16),
        pltpu.VMEM((M, 6 * M), bf16),
        pltpu.VMEM((8, 6 * M), f32),
        pltpu.VMEM((2, M, D), jnp.uint32),
        pltpu.VMEM((NP, DC, D), jnp.uint32),
        pltpu.VMEM((2, DC, D), jnp.uint32),
        pltpu.VMEM((M, 256), bf16), pltpu.VMEM((2, DC, 256), bf16), pltpu.VMEM((DC, 256), bf16),
        hv((2, 2, S, D), "q"),
        hv((H, S // 128, D, 128), "k"),
        hv((2, 2, S, D), "v"),
        pltpu.VMEM((H + (5 if cfg.get("AL") else 0), S, D), bf16),
        pltpu.VMEM((H * D, M), bf16),
        pltpu.VMEM((M, M), bf16), pltpu.VMEM((M, M), bf16), pltpu.VMEM((F, M), bf16), pltpu.VMEM((F, M), bf16),
        pltpu.VMEM((S + 16, M), f32),
        pltpu.VMEM((2, TM, M), f32), pltpu.VMEM((2, TM, M), f32), pltpu.VMEM((2, TM, M), bf16),
        pltpu.SemaphoreType.DMA((16,)), pltpu.SemaphoreType.DMA((NP,)), pltpu.SemaphoreType.DMA((2, 2)), pltpu.SemaphoreType.DMA((2,)),
    ]
    return pl.pallas_call(
        make_kernel(cfg),
        out_shape=jax.ShapeDtypeStruct((S, M), bf16),
        in_specs=[hbm] * 10 + [pl.BlockSpec(memory_space=pltpu.VMEM), hbm],
        out_specs=hbm,
        scratch_shapes=scratch,
        compiler_params=pltpu.CompilerParams(vmem_limit_bytes=cfg.get("VMEM", 120) * 2**20),
        name="fused_block",
    )


def run(cfg, A_x, A_c_kv, A_w_q, A_w_uk, A_w_uv, A_w_o, B_x, B_w1, B_w2, B_w3, B_w4, c, w_mod):
    out = build(cfg)(A_x.reshape(S, M), A_c_kv.reshape(S, DC), A_w_q, A_w_uk, A_w_uv, A_w_o.reshape(H * D, M),
                     B_w1, B_w2, B_w3.T, B_w4, c, w_mod)
    return out.reshape(1, S, M)


_CFG = {'U32': 'kv'}


@jax.jit
def pallas_adaLN_cond__compressed_kv_cla__mixer_s_mlp__prompt_kernel(A_x, A_c_kv, A_w_q, A_w_uk, A_w_uv, A_w_o, B_x, B_w1, B_w2, B_w3, B_w4, c, w_mod):
    return run(_CFG, A_x, A_c_kv, A_w_q, A_w_uk, A_w_uv, A_w_o, B_x, B_w1, B_w2, B_w3, B_w4, c, w_mod)
```

```python
import functools
import jax
import jax.numpy as jnp
import numpy as np
from jax.experimental import pallas as pl
from jax.experimental.pallas import tpu as pltpu

S = 2048; M = 640; H = 32; D = 128; DC = 512; F = 1728
NP = H // 2
EPS = 1e-5
LOG2E = 1.4426950408889634
QSCALE = float(D ** -0.5 * LOG2E)
NEG = -1e30
bf16 = jnp.bfloat16; f32 = jnp.float32


def _ln(x):
    m = jnp.mean(x, axis=-1, keepdims=True)
    xc = x - m
    v = jnp.mean(xc * xc, axis=-1, keepdims=True)
    return xc * jax.lax.rsqrt(v + EPS)


def _gelu(x):
    c = 0.7978845608028654
    return 0.5 * x * (1.0 + jnp.tanh(c * (x + 0.044715 * (x * x * x))))


def _rcp(l):
    r = pl.reciprocal(l, approx=True)
    return r * (2.0 - l * r)


def _dot(a, b):
    return jnp.dot(a, b, preferred_element_type=f32)


def _unpack_pair(w32):
    lo = pltpu.bitcast(w32 << 16, f32).astype(bf16)
    hi = pltpu.bitcast(w32 & jnp.uint32(0xFFFF0000), f32).astype(bf16)
    return lo, hi


SCR_NAMES = ['x_v', 'ckv_v', 'h_v', 'wmod_v', 'mod_v', 'wq32', 'wk32', 'wv32', 'wq_s', 'wk_s', 'wv_s', 'q_v', 'kT_v', 'v_v', 'ctx_v', 'wo_v', 'w1_v', 'w2_v', 'w3_v', 'w4_v', 'u_v', 'x1_v', 'h2_v', 'o_v', 'sem', 'ksem', 'wsem', 'osem']


def scratch_order(cfg):
    first = cfg.get("ORD", [])
    last = cfg.get("ORL", [])
    return list(first) + [n for n in SCR_NAMES if n not in first and n not in last] + list(last)


def make_kernel(cfg):
    TQ = 128
    PR = cfg.get("PR", 128)
    TM = cfg.get("TM", 256)
    LR = cfg.get("LR", 64)
    NB = S // TM
    NCK = cfg.get("NCK", 4)
    KPI = cfg.get("KPI", 3); P0 = cfg.get("P0", 1)
    assert (NP - P0) % KPI == 0

    import contextlib
    def sc_(name):
        on = cfg.get("SCOPE")
        if name == "barrier": on = cfg.get("BAR", 1)
        if isinstance(on, str): on = name in on.split(",")
        return jax.named_scope(name) if on else contextlib.nullcontext()

    U32 = cfg.get("U32", "")
    def st_(val, key):
        return pltpu.bitcast(val, jnp.uint32) if key in U32 else val
    def ld_(val, key):
        return pltpu.bitcast(val, bf16) if key in U32 else val
    def rs_(r0, n, key):
        return slice(r0 // 2, (r0 + n) // 2) if key in U32 else slice(r0, r0 + n)

    def kernel(x_hbm, ckv_hbm, wq_hbm, wuk_hbm, wuv_hbm, wo_hbm, w1_hbm, w2_hbm, w3_hbm, w4_hbm, c_ref, wmod_hbm,
               out_hbm, *scr):
        R = dict(zip(scratch_order(cfg), scr))
        (x_v, ckv_v, h_v, wmod_v, mod_v, wq32, wk32, wv32, wq_s, wk_s, wv_s, q_v, kT_v, v_v, ctx_v, wo_v, w1_v, w2_v, w3_v, w4_v, u_v, x1_v, h2_v, o_v, sem, ksem, wsem, osem) = [R[n] for n in SCR_NAMES]
        def cp(src, dst, i):
            return pltpu.make_async_copy(src, dst, sem.at[i])

        def wkcopy(g):
            return pltpu.make_async_copy(wuk_hbm.bitcast(jnp.uint32).at[:, g, :], wk32.at[g], ksem.at[g])

        def wcopies(g, slot):
            return (pltpu.make_async_copy(wq_hbm.bitcast(jnp.uint32).at[:, g, :], wq32.at[slot], wsem.at[0, slot]),
                    pltpu.make_async_copy(wuv_hbm.bitcast(jnp.uint32).at[:, g, :], wv32.at[slot], wsem.at[1, slot]))

        CR = S // NCK
        c_ckv = [cp(ckv_hbm.at[j * CR:(j + 1) * CR], ckv_v.at[j * CR:(j + 1) * CR], j) for j in range(NCK)]
        c_x = cp(x_hbm, x_v, 8); c_wmod = cp(wmod_hbm, wmod_v, 9)
        late = [cp(wo_hbm, wo_v, 10), cp(w1_hbm, w1_v, 11), cp(w2_hbm, w2_v, 12), cp(w3_hbm, w3_v, 13), cp(w4_hbm, w4_v, 14)]
        wkcopy(0).start(); c_ckv[0].start()
        def rest_start():
            for j in range(1, NCK): c_ckv[j].start()
            for g2 in range(1, P0 + 1): wkcopy(g2).start()
        if not cfg.get("ST"): rest_start()

        AL = cfg.get("AL", "")
        def vref(bs, hh):
            return ctx_v.at[H + 2 * bs + hh] if "v" in AL else v_v.at[bs, hh]
        def wq_load():
            if "c" in AL:
                return jnp.concatenate([ctx_v[H + 4, 0:M, :], ctx_v[H + 4, M:2 * M, :]], axis=1)
            return wq_s[...]
        def relayout_q(src):
            if "c" in AL:
                lo, hi = _unpack_pair(src[...])
                ctx_v[H + 4, 0:M, :] = lo
                ctx_v[H + 4, M:2 * M, :] = hi
            else:
                relayout(src, wq_s)

        def relayout(src, dst):
            lo, hi = _unpack_pair(src[...])
            dst[:, 0:128] = lo
            dst[:, 128:256] = hi

        def proj_k(g, par, r0):
            rows = slice(r0, r0 + PR)
            k = _dot(ckv_v[rows, :], wk_s[par])
            for hh in range(2):
                for t in range(PR // 128):
                    kT_v[2 * g + hh, (r0 // 128) + t] = st_(k[t * 128:(t + 1) * 128, hh * 128:(hh + 1) * 128].T.astype(bf16), "k")

        def proj_v(bs, r0):
            rows = slice(r0, r0 + PR)
            v = _dot(ckv_v[rows, :], wv_s[...]).astype(bf16)
            for hh in range(2): vref(bs, hh)[rs_(r0, PR, "v"), :] = st_(v[:, hh * 128:(hh + 1) * 128], "v")

        def proj_q(bs, r0):
            rows = slice(r0, r0 + PR)
            q = (_dot(h_v[rows, :], wq_load()) * QSCALE).astype(bf16)
            for hh in range(2): q_v[bs, hh, rs_(r0, PR, "q"), :] = st_(q[:, hh * 128:(hh + 1) * 128], "q")

        LAG = cfg.get("LAG", 0)
        tri = jax.lax.broadcasted_iota(jnp.int32, (128, 128), 1) <= jax.lax.broadcasted_iota(jnp.int32, (128, 128), 0)

        def qk(bs, g, hh, i):
            r0 = i * TQ; nt = i + 1
            q = ld_(q_v[bs, hh, rs_(r0, TQ, "q"), :], "q")
            tiles = [_dot(q, ld_(kT_v[(0 if cfg.get("KFIX") else 2 * g) + hh, t], "k")) for t in range(nt)]
            tiles[-1] = jnp.where(tri, tiles[-1], NEG)
            mx = tiles[0]
            for t in tiles[1:]:
                mx = jnp.maximum(mx, t)
            m = jnp.max(mx, axis=1, keepdims=True)
            return tiles, m

        def smpv(bs, g, hh, i, st):
            tiles, m = st
            r0 = i * TQ
            acc = None; ls = None
            for t, s in enumerate(tiles):
                p = jnp.exp2(s - m)
                ls = p if ls is None else ls + p
                o = _dot(p.astype(bf16), ld_(vref(bs, hh)[rs_(t * 128, 128, "v"), :], "v"))
                acc = o if acc is None else acc + o
            def fin():
                l = jnp.sum(ls, axis=1, keepdims=True)
                ctx_v[(0 if cfg.get("CFIX") else 2 * g) + hh, r0:r0 + TQ, :] = (acc * (_rcp(l) if cfg.get("NEWTON", 1) else pl.reciprocal(l, approx=True))).astype(bf16)
            return fin

        def attention(bs, g, items, pieces):
            st = qk(bs, g, *items[0])
            pend = []
            for n, it in enumerate(items):
                nxt = qk(bs, g, *items[n + 1]) if n + 1 < len(items) else None
                pend.append(smpv(bs, g, *it, st))
                if len(pend) > LAG:
                    pend.pop(0)()
                st = nxt
                if n in pieces:
                    if pieces[n][0] == "flush":
                        for f in pend: f()
                        pend = []
                    for f in pieces[n]:
                        if f != "flush": f()
            for f in pend: f()

        NI = S // TQ
        items_rev = [(hh, i) for hh in range(2) for i in reversed(range(NI))]


        def do_h(rr):
            rows = slice(rr, rr + LR)
            h_v[rows, :] = (_ln(x_v[rows, :].astype(f32)) * (1.0 + mod_v[0:1, M:2 * M]) + mod_v[0:1, 0:M]).astype(bf16)

        def kpair(g, par, nxt, npar, first=False):
            for r in range(S // PR):
                if first and (r * PR) % CR == 0 and not (r == 0 and cfg.get("ST") == 2):
                    c_ckv[(r * PR) // CR].wait()
                proj_k(g, par, r * PR)
                if r == cfg.get("RLP", (S // PR) // 2):
                    if first:
                        for g2 in range(1, P0 + 1): wkcopy(g2).wait()
                        for g2 in range(P0 + 1, NP): wkcopy(g2).start()
                    relayout(wk32.at[nxt], wk_s.at[npar])

        with sc_("s1_kphase"):
          with sc_("s1_wait0"):
            wkcopy(0).wait()
            if cfg.get("ST") == 2: c_ckv[0].wait()
          if cfg.get("ST"): rest_start()
          relayout(wk32.at[0], wk_s.at[0])
          for g in range(P0):
              kpair(g, g % KPI, g + 1, (g + 1) % KPI if g + 1 < P0 else 0, first=(g == 0))

          def kbody(j, carry):
            g = P0 + KPI * j
            c_g = [pltpu.make_async_copy(wuk_hbm.bitcast(jnp.uint32).at[:, jnp.minimum(g + k, NP - 1), :], wk32.at[jnp.minimum(g + k, NP - 1)],
                                         ksem.at[jnp.minimum(g + k, NP - 1)]) for k in range(1, KPI + 1)]
            for k in range(KPI - 1): c_g[k].wait()

            @pl.when(g + KPI < NP)
            def _():
                c_g[KPI - 1].wait()

            @pl.when(j == cfg.get("XJ", 0))
            def _():
                c_x.start(); c_wmod.start()
                for d in wcopies(0, 0): d.start()
                for d in wcopies(1, 1): d.start()
            with sc_("barrier"):
              for k in range(KPI):
                kpair(g + k, k, jnp.minimum(g + k + 1, NP - 1), (k + 1) % KPI)
            return carry
          with sc_("s1_kloop"):
            jax.lax.fori_loop(0, (NP - P0) // KPI, kbody, 0)

        def do_mod(a, b):
            cc = c_ref[...].astype(f32)
            sc = (cc * jax.nn.sigmoid(cc)).astype(bf16)
            mod_v[:, a:b] = _dot(jnp.broadcast_to(sc, (8, M)), wmod_v[:, a:b])

        with sc_("s2_vq0"):
            for d in wcopies(0, 0): d.wait()
            c_x.wait(); c_wmod.wait()
            for d in late: d.start()
            relayout(wv32.at[0], wv_s); relayout_q(wq32.at[0])
            NR = S // PR
            def vstep(r):
                if r < NR: proj_v(0, r * PR)
                if r == 0: do_mod(0, 2 * M)
                if r == cfg.get("MODB", 8): do_mod(2 * M, 6 * M)
                if 1 <= r <= NR:
                    for rr in range((r - 1) * PR, r * PR, LR): do_h(rr)
                if r >= 2: proj_q(0, (r - 2) * PR)
            BV = cfg.get("BARV", 99)
            for r0_ in range(0, NR + 2, BV):
                with jax.named_scope("vq%d" % r0_):
                    for r in range(r0_, min(NR + 2, r0_ + BV)): vstep(r)

        for d in late[0:0]: d.start()
        def body(g, carry):
            bs = g & 1
            ws = 1 - bs
            for d in wcopies(jnp.minimum(g + 2, NP - 1), bs): d.start()
            with sc_("sj_wait"):
                for d in wcopies(g + 1, ws): d.wait()
            with sc_("sk_relay"):
                relayout(wv32.at[ws], wv_s); relayout_q(wq32.at[ws])
            npieces = S // PR
            its = items_rev if cfg.get("REV", 1) == 1 else ([(hh, i) for hh in range(2) for i in range(NI)] if cfg.get("REV") == 0 else
                  [(0, i) for i in reversed(range(NI))] + [(1, i) for i in range(NI)])
            every = len(items_rev) // npieces
            pieces = {}
            for k in range(npieces):
                pieces[k * every + cfg.get("POFF", 1)] = [functools.partial(proj_v, ws, k * PR), functools.partial(proj_q, ws, k * PR)]
            with sc_("si_iter"):
                attention(bs, g, its, pieces)
            return carry
        with sc_("s5_main"):
            jax.lax.fori_loop(0, NP - 1, body, 0)
        for d in wcopies(NP - 1, (NP - 2) % 2): d.wait()

        for d in late: d.wait()
        zero8 = jnp.zeros((8, M), f32)
        u_v[0:8, :] = zero8; u_v[8 + S:16 + S, :] = zero8
        def modv(j): return mod_v[0:1, j * M:(j + 1) * M]

        def A1(r, slot):
            r0 = pl.multiple_of(r * TM, TM)
            cx = jnp.concatenate([ctx_v[hh, pl.ds(r0, TM), :] for hh in range(H)], axis=1)
            return _dot(cx, wo_v[...])

        def A2(r, slot, a):
            r0 = pl.multiple_of(r * TM, TM)
            outs = []
            for rr in range(0, TM, LR):
                x1 = x_v[pl.ds(r0 + rr, LR), :].astype(f32) + modv(2) * a[rr:rr + LR]
                h2 = _ln(x1) * (1.0 + modv(4)) + modv(3)
                x1_v[slot, rr:rr + LR, :] = x1; h2_v[slot, rr:rr + LR, :] = h2
                outs.append(_ln(h2).astype(bf16))
            return jnp.concatenate(outs, axis=0)

        def A3(r, slot, l2):
            r0 = pl.multiple_of(r * TM, TM)
            u_v[pl.ds(r0 + 8, TM), :] = _gelu(_dot(l2, w1_v[...]))

        def B1(r, slot, ro=0, n=TM):
            r0 = pl.multiple_of(r * TM, TM) + ro
            lane = jax.lax.broadcasted_iota(jnp.int32, (n, 128), 1)
            def sh(delta, j):
                win = u_v[pl.ds(r0, n + 16), j * 128:(j + 1) * 128]
                return win[8 + delta:8 + delta + n]
            t0 = sh(-1, 0)
            t1 = jnp.where(lane < 32, sh(-1, 1), sh(1, 1))
            t2 = jnp.where(lane < 64, sh(1, 2), sh(-2, 2))
            t3 = jnp.where(lane < 96, sh(-2, 3), sh(2, 3))
            t4 = sh(2, 4)
            return jnp.concatenate([t0, t1, t2, t3, t4], axis=1).astype(bf16)

        def B2(r, slot, us):
            return _dot(us, w2_v[...])

        def B3(r, slot, hs, ro=0, n=TM):
            outs = []
            for rr in range(0, n, LR):
                xb1 = h2_v[slot, ro + rr:ro + rr + LR, :] + hs[rr:rr + LR]
                h2_v[slot, ro + rr:ro + rr + LR, :] = xb1
                outs.append(_ln(xb1).astype(bf16))
            return jnp.concatenate(outs, axis=0)

        def B4(r, slot, l3):
            return _gelu(jax.lax.dot_general(l3, w3_v[...], (((1,), (1,)), ((), ())), preferred_element_type=f32)).astype(bf16)

        def B5(r, slot, gg, ro=0, n=TM):
            y = _dot(gg, w4_v[...])
            o_v[slot, ro:ro + n, :] = (x1_v[slot, ro:ro + n, :] + modv(5) * (h2_v[slot, ro:ro + n, :] + y)).astype(bf16)

        def ocopy(r, slot):
            r0 = pl.multiple_of(r * TM, TM)
            return pltpu.make_async_copy(o_v.at[slot], out_hbm.at[pl.ds(r0, TM)], osem.at[slot])

        with sc_("s6_attn_last"):
            nf = TM // TQ
            if cfg.get("FUSEA0", 1):
                items = [(hh, i) for hh in range(2) for i in range(nf)] + [(hh, i) for hh in range(2) for i in reversed(range(nf, NI))]
                st = {}
                n0 = 2 * nf + cfg.get("A0POS", 1)
                pieces = {n0: ["flush", lambda: st.__setitem__("a", A1(0, 0))],
                          n0 + cfg.get("A0D", 4): [lambda: A3(0, 0, A2(0, 0, st["a"]))]}
                attention((NP - 1) % 2, NP - 1, items, pieces)
            else:
                attention((NP - 1) % 2, NP - 1, items_rev, {})
                A3(0, 0, A2(0, 0, A1(0, 0)))

        def fbody(r, carry):
            slot = r & 1

            @pl.when(r >= 2)
            def _():
                ocopy(r - 2, slot).wait()
            st = {}
            ops = {
                "B1": lambda: st.__setitem__("us", B1(r, slot)),
                "A1": lambda: st.__setitem__("a", A1(r + 1, 1 - slot)),
                "B2": lambda: st.__setitem__("hs", B2(r, slot, st["us"])),
                "A2": lambda: st.__setitem__("l2", A2(r + 1, 1 - slot, st["a"])),
                "A3": lambda: A3(r + 1, 1 - slot, st["l2"]),
                "B3": lambda: st.__setitem__("l3", B3(r, slot, st["hs"])),
                "B4": lambda: st.__setitem__("gg", B4(r, slot, st["l3"])),
                "B5": lambda: B5(r, slot, st["gg"]),
            }
            for name in cfg.get("FORD", "B1 B2 A1 B3 B4 A2 A3 B5").split():
                if name == "|":
                    with jax.named_scope("fb"):
                        pass
                else:
                    ops[name]()
            ocopy(r, slot).start()
            return carry
        with sc_("s8_floop"):
            jax.lax.fori_loop(0, NB - 1, fbody, 0)
        ocopy(NB - 3, (NB - 1) % 2).wait()
        sl = (NB - 1) % 2
        with sc_("s9_Blast"):
            nsp = cfg.get("BSPL", 2); n = TM // nsp
            r = NB - 1
            hs = [B2(r, sl, B1(r, sl, i * n, n)) for i in range(nsp)]
            gg = [B4(r, sl, B3(r, sl, hs[i], i * n, n)) for i in range(nsp)]
            for i in range(nsp): B5(r, sl, gg[i], i * n, n)
        with sc_("sa_outwait"):
            ocopy(NB - 1, sl).start()
            ocopy(NB - 2, (NB - 2) % 2).wait()
            ocopy(NB - 1, sl).wait()

    return kernel


def build(cfg):
    TM = cfg.get("TM", 256)
    hbm = pl.BlockSpec(memory_space=pltpu.MemorySpace.HBM)
    def hv(shape, key):
        if key in cfg.get("U32", ""):
            return pltpu.VMEM(shape[:-2] + (shape[-2] // 2, shape[-1]), jnp.uint32)
        return pltpu.VMEM(shape, bf16)
    scratch = [
        pltpu.VMEM((S, M), bf16),
        pltpu.VMEM((S, DC), bf16),
        pltpu.VMEM((S, M), bf16),
        pltpu.VMEM((M, 6 * M), bf16),
        pltpu.VMEM((8, 6 * M), f32),
        pltpu.VMEM((2, M, D), jnp.uint32),
        pltpu.VMEM((NP, DC, D), jnp.uint32),
        pltpu.VMEM((2, DC, D), jnp.uint32),
        pltpu.VMEM((M, 256), bf16), pltpu.VMEM((max(2, cfg.get("KPI", 3)), DC, 256), bf16), pltpu.VMEM((DC, 256), bf16),
        hv((2, 2, S, D), "q"),
        hv((H, S // 128, D, 128), "k"),
        hv((2, 2, S, D), "v"),
        pltpu.VMEM((H + (5 if cfg.get("AL") else 0), S, D), bf16),
        pltpu.VMEM((H * D, M), bf16),
        pltpu.VMEM((M, M), bf16), pltpu.VMEM((M, M), bf16), pltpu.VMEM((F, M), bf16), pltpu.VMEM((F, M), bf16),
        pltpu.VMEM((S + 16, M), f32),
        pltpu.VMEM((2, TM, M), f32), pltpu.VMEM((2, TM, M), f32), pltpu.VMEM((2, TM, M), bf16),
        pltpu.SemaphoreType.DMA((16,)), pltpu.SemaphoreType.DMA((NP,)), pltpu.SemaphoreType.DMA((2, 2)), pltpu.SemaphoreType.DMA((2,)),
    ]
    sd = dict(zip(SCR_NAMES, scratch))
    assert len(scratch) == len(SCR_NAMES)
    scratch = [sd[n] if n in sd else pltpu.VMEM((8 * int(n.split("_")[1]), 128), f32) for n in scratch_order(cfg)]
    return pl.pallas_call(
        make_kernel(cfg),
        out_shape=jax.ShapeDtypeStruct((S, M), bf16),
        in_specs=[hbm] * 10 + [pl.BlockSpec(memory_space=pltpu.VMEM), hbm],
        out_specs=hbm,
        scratch_shapes=scratch,
        compiler_params=pltpu.CompilerParams(vmem_limit_bytes=cfg.get("VMEM", 120) * 2**20),
        name="fused_block",
    )


def run(cfg, A_x, A_c_kv, A_w_q, A_w_uk, A_w_uv, A_w_o, B_x, B_w1, B_w2, B_w3, B_w4, c, w_mod):
    out = build(cfg)(A_x.reshape(S, M), A_c_kv.reshape(S, DC), A_w_q, A_w_uk, A_w_uv, A_w_o.reshape(H * D, M),
                     B_w1, B_w2, B_w3.T, B_w4, c, w_mod)
    return out.reshape(1, S, M)


_CFG = {'U32': 'kv', 'ORD': ['ctx_v', 'kT_v'], 'ST': 2, 'NCK': 4, 'A0POS': 8, 'A0D': 8}


@jax.jit
def pallas_adaLN_cond__compressed_kv_cla__mixer_s_mlp__prompt_kernel(A_x, A_c_kv, A_w_q, A_w_uk, A_w_uv, A_w_o, B_x, B_w1, B_w2, B_w3, B_w4, c, w_mod):
    return run(_CFG, A_x, A_c_kv, A_w_q, A_w_uk, A_w_uv, A_w_o, B_x, B_w1, B_w2, B_w3, B_w4, c, w_mod)
```

```python
import functools
import jax
import jax.numpy as jnp
import numpy as np
from jax.experimental import pallas as pl
from jax.experimental.pallas import tpu as pltpu

S = 2048; M = 640; H = 32; D = 128; DC = 512; F = 1728
NP = H // 2
EPS = 1e-5
LOG2E = 1.4426950408889634
QSCALE = float(D ** -0.5 * LOG2E)
NEG = -1e30
bf16 = jnp.bfloat16; f32 = jnp.float32


def _ln(x):
    m = jnp.mean(x, axis=-1, keepdims=True)
    xc = x - m
    v = jnp.mean(xc * xc, axis=-1, keepdims=True)
    return xc * jax.lax.rsqrt(v + EPS)


def _gelu(x):
    c = 0.7978845608028654
    return 0.5 * x * (1.0 + jnp.tanh(c * (x + 0.044715 * (x * x * x))))


def _rcp(l):
    r = pl.reciprocal(l, approx=True)
    return r * (2.0 - l * r)


def _dot(a, b):
    return jnp.dot(a, b, preferred_element_type=f32)


def _unpack_pair(w32):
    lo = pltpu.bitcast(w32 << 16, f32).astype(bf16)
    hi = pltpu.bitcast(w32 & jnp.uint32(0xFFFF0000), f32).astype(bf16)
    return lo, hi


SCR_NAMES = ['x_v', 'ckv_v', 'h_v', 'wmod_v', 'mod_v', 'wq32', 'wk32', 'wv32', 'wq_s', 'wk_s', 'wv_s', 'q_v', 'kT_v', 'v_v', 'ctx_v', 'wo_v', 'w1_v', 'w2_v', 'w3_v', 'w4_v', 'u_v', 'x1_v', 'h2_v', 'o_v', 'sem', 'ksem', 'wsem', 'osem', 'fsem', 'zs_ref']


def scratch_order(cfg):
    first = cfg.get("ORD", [])
    last = cfg.get("ORL", [])
    return list(first) + [n for n in SCR_NAMES if n not in first and n not in last] + list(last)


def make_kernel(cfg):
    TQ = 128
    PR = cfg.get("PR", 128)
    TM = cfg.get("TM", 256)
    LR = cfg.get("LR", 64)
    NB = S // TM
    NCK = cfg.get("NCK", 4)
    KPI = cfg.get("KPI", 3); P0 = cfg.get("P0", 1)
    assert (NP - P0) % KPI == 0

    import contextlib
    def sc_(name):
        on = cfg.get("SCOPE")
        if name == "barrier": on = cfg.get("BAR", 1)
        if isinstance(on, str): on = name in on.split(",")
        return jax.named_scope(name) if on else contextlib.nullcontext()

    U32 = cfg.get("U32", "")
    def st_(val, key):
        return pltpu.bitcast(val, jnp.uint32) if key in U32 else val
    def ld_(val, key):
        return pltpu.bitcast(val, bf16) if key in U32 else val
    def rs_(r0, n, key):
        return slice(r0 // 2, (r0 + n) // 2) if key in U32 else slice(r0, r0 + n)

    def kernel(x_hbm, ckv_hbm, wq_hbm, wuk_hbm, wuv_hbm, wo_hbm, w1_hbm, w2_hbm, w3_hbm, w4_hbm, c_ref, wmod_hbm,
               out_hbm, *scr):
        R = dict(zip(scratch_order(cfg), scr))
        (x_v, ckv_v, h_v, wmod_v, mod_v, wq32, wk32, wv32, wq_s, wk_s, wv_s, q_v, kT_v, v_v, ctx_v, wo_v, w1_v, w2_v, w3_v, w4_v, u_v, x1_v, h2_v, o_v, sem, ksem, wsem, osem, fsem, zs_ref) = [R[n] for n in SCR_NAMES]
        def cp(src, dst, i):
            return pltpu.make_async_copy(src, dst, sem.at[i])

        def wkcopy(g):
            return pltpu.make_async_copy(wuk_hbm.bitcast(jnp.uint32).at[:, g, :], wk32.at[g], ksem.at[g])

        def wcopies(g, slot):
            return (pltpu.make_async_copy(wq_hbm.bitcast(jnp.uint32).at[:, g, :], wq32.at[slot], wsem.at[0, slot]),
                    pltpu.make_async_copy(wuv_hbm.bitcast(jnp.uint32).at[:, g, :], wv32.at[slot], wsem.at[1, slot]))

        CR = S // NCK
        c_ckv = [cp(ckv_hbm.at[j * CR:(j + 1) * CR], ckv_v.at[j * CR:(j + 1) * CR], j) for j in range(NCK)]
        c_x = cp(x_hbm, x_v, 8); c_wmod = cp(wmod_hbm, wmod_v, 9)
        late = [cp(wo_hbm, wo_v, 10), cp(w1_hbm, w1_v, 11), cp(w2_hbm, w2_v, 12), cp(w3_hbm, w3_v, 13), cp(w4_hbm, w4_v, 14)]
        wkcopy(0).start(); c_ckv[0].start()
        def rest_start():
            for j in range(1, NCK): c_ckv[j].start()
            for g2 in range(1, P0 + 1): wkcopy(g2).start()
        if not cfg.get("ST"): rest_start()

        AL = cfg.get("AL", "")
        def vref(bs, hh):
            return ctx_v.at[H + 2 * bs + hh] if "v" in AL else v_v.at[bs, hh]
        def wq_load():
            if "c" in AL:
                return jnp.concatenate([ctx_v[H + 4, 0:M, :], ctx_v[H + 4, M:2 * M, :]], axis=1)
            return wq_s[...]
        def relayout_q(src):
            if "c" in AL:
                lo, hi = _unpack_pair(src[...])
                ctx_v[H + 4, 0:M, :] = lo
                ctx_v[H + 4, M:2 * M, :] = hi
            else:
                relayout(src, wq_s)

        def relayout(src, dst):
            lo, hi = _unpack_pair(src[...])
            dst[:, 0:128] = lo
            dst[:, 128:256] = hi

        def proj_k(g, par, r0):
            rows = slice(r0, r0 + PR)
            k = _dot(ckv_v[rows, :], wk_s[par])
            for hh in range(2):
                for t in range(PR // 128):
                    kT_v[2 * g + hh, (r0 // 128) + t] = st_(k[t * 128:(t + 1) * 128, hh * 128:(hh + 1) * 128].T.astype(bf16), "k")

        def proj_v(bs, r0):
            rows = slice(r0, r0 + PR)
            v = _dot(ckv_v[rows, :], wv_s[...]).astype(bf16)
            for hh in range(2): vref(bs, hh)[rs_(r0, PR, "v"), :] = st_(v[:, hh * 128:(hh + 1) * 128], "v")

        def proj_q(bs, r0):
            rows = slice(r0, r0 + PR)
            q = (_dot(h_v[rows, :], wq_load()) * QSCALE).astype(bf16)
            for hh in range(2): q_v[bs, hh, rs_(r0, PR, "q"), :] = st_(q[:, hh * 128:(hh + 1) * 128], "q")

        LAG = cfg.get("LAG", 0)
        nv_ = {}
        def never():
            return nv_["m"]
        tri = jax.lax.broadcasted_iota(jnp.int32, (128, 128), 1) <= jax.lax.broadcasted_iota(jnp.int32, (128, 128), 0)

        def qk(bs, g, hh, i):
            r0 = i * TQ; nt = i + 1
            q = ld_(q_v[bs, hh, rs_(r0, TQ, "q"), :], "q")
            tiles = [_dot(q, ld_(kT_v[(0 if cfg.get("KFIX") else 2 * g) + hh, t], "k")) for t in range(nt)]
            tiles[-1] = jnp.where(tri, tiles[-1], NEG)
            mx = tiles[0]
            for t in tiles[1:]:
                mx = jnp.maximum(mx, t)
            m = jnp.max(mx, axis=1, keepdims=True)
            return tiles, m

        def smpv(bs, g, hh, i, st):
            tiles, m = st
            r0 = i * TQ
            acc = None; ls = None
            FR = cfg.get("FR", 0) if nv_["on"] else 0
            rold = None
            if FR and len(nv_["rq"]) >= FR:
                rold = jnp.broadcast_to(nv_["rq"].pop(0), (TQ, 128))
            for t, s in enumerate(tiles):
                p = jnp.exp2(s - m)
                FK = cfg.get("FK", 0) if nv_["on"] else 0
                pm = p
                if FK == 1 and ls is not None:
                    pm = jnp.where(never(), ls, p)
                ls = p if ls is None else ls + p
                if FK == 2:
                    pm = jnp.where(never(), ls, p) if t > 0 else p
                if rold is not None and t == min(cfg.get("FRT", 0), len(tiles) - 1):
                    pm = jnp.where(never(), rold, pm)
                o = _dot(pm.astype(bf16), ld_(vref(bs, hh)[rs_(t * 128, 128, "v"), :], "v"))
                acc = o if acc is None else acc + o
            if FR:
                rr_ = _rcp(jnp.sum(ls, axis=1, keepdims=True))
                nv_["rq"].append(rr_)
            def fin():
                r = rr_ if FR else _rcp(jnp.sum(ls, axis=1, keepdims=True))
                ctx_v[2 * g + hh, r0:r0 + TQ, :] = (acc * r).astype(bf16)
            return fin

        def attention(bs, g, items, pieces, fk=True):
            nv_["on"] = fk; nv_["rq"] = []
            if cfg.get("FK"):
                sv = mod_v[0:8, 0:128]
                nv_["m"] = jnp.broadcast_to((sv != sv)[0:1], (128, 128))
                nv_["m1"] = jnp.broadcast_to((sv != sv)[0:1, 0:1], (128, 1))
            st = qk(bs, g, *items[0])
            pend = []
            for n, it in enumerate(items):
                nxt = qk(bs, g, *items[n + 1]) if n + 1 < len(items) else None
                pend.append(smpv(bs, g, *it, st))
                if len(pend) > LAG:
                    pend.pop(0)()
                st = nxt
                if n in pieces:
                    if pieces[n][0] == "flush":
                        for f in pend: f()
                        pend = []
                    for f in pieces[n]:
                        if f != "flush": f()
            for f in pend: f()

        NI = S // TQ
        items_rev = [(hh, i) for hh in range(2) for i in reversed(range(NI))]


        def do_h(rr, dyn=None):
            rows = slice(rr, rr + LR) if dyn is None else pl.ds(pl.multiple_of(dyn + rr, LR), LR)
            h_v[rows, :] = (_ln(x_v[rows, :].astype(f32)) * (1.0 + mod_v[0:1, M:2 * M]) + mod_v[0:1, 0:M]).astype(bf16)

        def do_mod(a, b):
            cc = c_ref[...].astype(f32)
            sc = (cc * jax.nn.sigmoid(cc)).astype(bf16)
            mod_v[:, a:b] = _dot(jnp.broadcast_to(sc, (8, M)), wmod_v[:, a:b])

        HL = cfg.get("HL", 0)
        def kpair(g, par, nxt, npar, first=False, extra=None):
            for r in range(S // PR):
                if first and (r * PR) % CR == 0 and not (r == 0 and cfg.get("ST") == 2):
                    c_ckv[(r * PR) // CR].wait()
                proj_k(g, par, r * PR)
                if r == cfg.get("RLP", (S // PR) // 2):
                    if first:
                        for g2 in range(1, P0 + 1): wkcopy(g2).wait()
                        for g2 in range(P0 + 1, NP): wkcopy(g2).start()
                    relayout(wk32.at[nxt], wk_s.at[npar])
                if extra is not None and r in extra: extra[r]()

        with sc_("s1_kphase"):
          with sc_("s1_wait0"):
            wkcopy(0).wait()
            if cfg.get("ST") == 2: c_ckv[0].wait()
          if cfg.get("ST"): rest_start()
          relayout(wk32.at[0], wk_s.at[(0 - P0) % KPI])
          for g in range(P0):
              ex = {}
              if HL:
                  if g == 1:
                      def st1():
                          c_x.start(); c_wmod.start()
                      ex[0] = st1
                  if g == P0 - 2:
                      def st2():
                          for d in wcopies(0, 0): d.start()
                          for d in wcopies(1, 1): d.start()
                      ex[0] = st2
                  if g == P0 - 1:
                      def m1():
                          c_wmod.wait(); do_mod(0, 2 * M)
                      ex[2] = m1
                      ex[9] = lambda: do_mod(2 * M, 4 * M)
                      def m3():
                          do_mod(4 * M, 6 * M); c_x.wait()
                      ex[13] = m3
              kpair(g, (g - P0) % KPI, g + 1, (g + 1 - P0) % KPI, first=(g == 0), extra=ex)

          def kbody(j, carry):
            g = P0 + KPI * j
            c_g = [pltpu.make_async_copy(wuk_hbm.bitcast(jnp.uint32).at[:, jnp.minimum(g + k, NP - 1), :], wk32.at[jnp.minimum(g + k, NP - 1)],
                                         ksem.at[jnp.minimum(g + k, NP - 1)]) for k in range(1, KPI + 1)]
            for k in range(KPI - 1): c_g[k].wait()

            @pl.when(g + KPI < NP)
            def _():
                c_g[KPI - 1].wait()

            if not HL:
                @pl.when(j == cfg.get("XJ", 0))
                def _():
                    c_x.start(); c_wmod.start()
                    for d in wcopies(0, 0): d.start()
                    for d in wcopies(1, 1): d.start()
            NIT_ = (NP - P0) // KPI
            HR = S // NIT_
            nch = HR // LR
            with sc_("barrier"):
              for k in range(KPI):
                ex = {}
                if HL:
                    NR_ = S // PR
                    for ci in range(nch):
                        pos = (ci * KPI * NR_) // nch + 1
                        if pos // NR_ == k:
                            ex[pos % NR_] = functools.partial(do_h, ci * LR, j * HR)
                kpair(g + k, k, jnp.minimum(g + k + 1, NP - 1), (k + 1) % KPI, extra=ex)
            return carry
          with sc_("s1_kloop"):
            jax.lax.fori_loop(0, (NP - P0) // KPI, kbody, 0)

        with sc_("s2_vq0"):
            for d in wcopies(0, 0): d.wait()
            if not HL:
                c_x.wait(); c_wmod.wait()
            for d in late: d.start()
            relayout(wv32.at[0], wv_s); relayout_q(wq32.at[0])
            NR = S // PR
            def vstep(r):
                if r < NR: proj_v(0, r * PR)
                if HL:
                    if r < NR: proj_q(0, r * PR)
                    return
                if r == 0: do_mod(0, 2 * M)
                if r == cfg.get("MODB", 8): do_mod(2 * M, 6 * M)
                if 1 <= r <= NR:
                    for rr in range((r - 1) * PR, r * PR, LR): do_h(rr)
                if r >= 2: proj_q(0, (r - 2) * PR)
            HS = cfg.get("HS", NR)
            if cfg.get("VQ2", 1) and not HL:
                with jax.named_scope("s2_a"):
                    do_mod(0, 2 * M)
                    for r in range(NR):
                        proj_v(0, r * PR)
                        if r < HS:
                            for rr in range(r * PR, (r + 1) * PR, LR): do_h(rr)
                with jax.named_scope("s2_b"):
                    if HS == 0:
                        for rr in range(0, PR * cfg.get("HLEAD", 1), LR): do_h(rr)
                    for r in range(NR):
                        hh_ = (HS if HS > 0 else cfg.get("HLEAD", 1)) + r
                        if HS == 0 and hh_ < NR:
                            for rr in range(hh_ * PR, (hh_ + 1) * PR, LR): do_h(rr)
                        proj_q(0, r * PR)
                        if HS > 0 and hh_ < NR:
                            for rr in range(hh_ * PR, (hh_ + 1) * PR, LR): do_h(rr)
                        if r == cfg.get("MODB", 8): do_mod(2 * M, 6 * M)
            else:
                BV = cfg.get("BARV", 99)
                for r0_ in range(0, NR + 2, BV):
                    with jax.named_scope("vq%d" % r0_):
                        for r in range(r0_, min(NR + 2, r0_ + BV)): vstep(r)

        for d in late[0:0]: d.start()
        def body(g, carry):
            bs = g & 1
            ws = 1 - bs
            for d in wcopies(jnp.minimum(g + 2, NP - 1), bs): d.start()
            with sc_("sj_wait"):
                for d in wcopies(g + 1, ws): d.wait()
            with sc_("sk_relay"):
                relayout(wv32.at[ws], wv_s); relayout_q(wq32.at[ws])
            npieces = S // PR
            its = items_rev if cfg.get("REV", 1) == 1 else ([(hh, i) for hh in range(2) for i in range(NI)] if cfg.get("REV") == 0 else
                  [(0, i) for i in reversed(range(NI))] + [(1, i) for i in range(NI)])
            every = len(items_rev) // npieces
            pieces = {}
            for k in range(npieces):
                pieces[k * every + cfg.get("POFF", 1)] = [functools.partial(proj_v, ws, k * PR), functools.partial(proj_q, ws, k * PR)]
            with sc_("si_iter"):
                attention(bs, g, its, pieces)
            return carry
        with sc_("s5_main"):
            jax.lax.fori_loop(0, NP - 1, body, 0)
        for d in wcopies(NP - 1, (NP - 2) % 2): d.wait()

        for d in late: d.wait()
        zero8 = jnp.zeros((8, M), f32)
        u_v[0:8, :] = zero8; u_v[8 + S:16 + S, :] = zero8
        def modv(j): return mod_v[0:1, j * M:(j + 1) * M]

        def A1(r, slot):
            r0 = pl.multiple_of(r * TM, TM)
            cx = jnp.concatenate([ctx_v[hh, pl.ds(r0, TM), :] for hh in range(H)], axis=1)
            return _dot(cx, wo_v[...])

        def A2(r, slot, a):
            r0 = pl.multiple_of(r * TM, TM)
            outs = []
            for rr in range(0, TM, LR):
                x1 = x_v[pl.ds(r0 + rr, LR), :].astype(f32) + modv(2) * a[rr:rr + LR]
                h2 = _ln(x1) * (1.0 + modv(4)) + modv(3)
                x1_v[slot, rr:rr + LR, :] = x1; h2_v[slot, rr:rr + LR, :] = h2
                outs.append(_ln(h2).astype(bf16))
            return jnp.concatenate(outs, axis=0)

        def A3(r, slot, l2):
            r0 = pl.multiple_of(r * TM, TM)
            u_v[pl.ds(r0 + 8, TM), :] = _gelu(_dot(l2, w1_v[...]))

        def B1(r, slot, ro=0, n=TM):
            r0 = pl.multiple_of(r * TM, TM) + ro
            lane = jax.lax.broadcasted_iota(jnp.int32, (n, 128), 1)
            def sh(delta, j):
                win = u_v[pl.ds(r0, n + 16), j * 128:(j + 1) * 128]
                return win[8 + delta:8 + delta + n]
            t0 = sh(-1, 0)
            t1 = jnp.where(lane < 32, sh(-1, 1), sh(1, 1))
            t2 = jnp.where(lane < 64, sh(1, 2), sh(-2, 2))
            t3 = jnp.where(lane < 96, sh(-2, 3), sh(2, 3))
            t4 = sh(2, 4)
            return jnp.concatenate([t0, t1, t2, t3, t4], axis=1).astype(bf16)

        def B2(r, slot, us):
            return _dot(us, w2_v[...])

        def B3(r, slot, hs, ro=0, n=TM):
            outs = []
            for rr in range(0, n, LR):
                xb1 = h2_v[slot, ro + rr:ro + rr + LR, :] + hs[rr:rr + LR]
                h2_v[slot, ro + rr:ro + rr + LR, :] = xb1
                outs.append(_ln(xb1).astype(bf16))
            return jnp.concatenate(outs, axis=0)

        def B4(r, slot, l3):
            return _gelu(jax.lax.dot_general(l3, w3_v[...], (((1,), (1,)), ((), ())), preferred_element_type=f32)).astype(bf16)

        def B5(r, slot, gg, ro=0, n=TM):
            y = _dot(gg, w4_v[...])
            o_v[slot, ro:ro + n, :] = (x1_v[slot, ro:ro + n, :] + modv(5) * (h2_v[slot, ro:ro + n, :] + y)).astype(bf16)

        def ocopy(r, slot):
            r0 = pl.multiple_of(r * TM, TM)
            return pltpu.make_async_copy(o_v.at[slot], out_hbm.at[pl.ds(r0, TM)], osem.at[slot])

        with sc_("s6_attn_last"):
            nf = TM // TQ
            if cfg.get("FUSEA0", 1):
                items = [(hh, i) for hh in range(2) for i in range(nf)] + [(hh, i) for hh in range(2) for i in reversed(range(nf, NI))]
                st = {}
                n0 = 2 * nf + cfg.get("A0POS", 1)
                pieces = {n0: ["flush", lambda: st.__setitem__("a", A1(0, 0))],
                          n0 + cfg.get("A0D", 4): [lambda: A3(0, 0, A2(0, 0, st["a"]))]}
                attention((NP - 1) % 2, NP - 1, items, pieces, fk=cfg.get("FKL", 0))
            else:
                attention((NP - 1) % 2, NP - 1, items_rev, {})
                A3(0, 0, A2(0, 0, A1(0, 0)))

        def fbody(r, carry):
            slot = r & 1

            @pl.when(r >= 2)
            def _():
                ocopy(r - 2, slot).wait()
            st = {}
            ops = {
                "B1": lambda: st.__setitem__("us", B1(r, slot)),
                "A1": lambda: st.__setitem__("a", A1(r + 1, 1 - slot)),
                "B2": lambda: st.__setitem__("hs", B2(r, slot, st["us"])),
                "A2": lambda: st.__setitem__("l2", A2(r + 1, 1 - slot, st["a"])),
                "A3": lambda: A3(r + 1, 1 - slot, st["l2"]),
                "B3": lambda: st.__setitem__("l3", B3(r, slot, st["hs"])),
                "B4": lambda: st.__setitem__("gg", B4(r, slot, st["l3"])),
                "B5": lambda: B5(r, slot, st["gg"]),
            }
            for name in cfg.get("FORD", "B1 B2 A1 B3 B4 A2 A3 B5").split():
                if name == "|":
                    with jax.named_scope("zfb"):
                        pass
                else:
                    ops[name]()
            ocopy(r, slot).start()
            return carry
        with sc_("s8_floop"):
            jax.lax.fori_loop(0, NB - 1, fbody, 0)
        ocopy(NB - 3, (NB - 1) % 2).wait()
        sl = (NB - 1) % 2
        with sc_("s9_Blast"):
            nsp = cfg.get("BSPL", 2); n = TM // nsp
            r = NB - 1
            hs = [B2(r, sl, B1(r, sl, i * n, n)) for i in range(nsp)]
            gg = [B4(r, sl, B3(r, sl, hs[i], i * n, n)) for i in range(nsp)]
            fin_cp = [pltpu.make_async_copy(o_v.at[sl, i * n:(i + 1) * n, :], out_hbm.at[r * TM + i * n:r * TM + (i + 1) * n, :], fsem.at[i]) for i in range(nsp)]
            for i in range(nsp):
                B5(r, sl, gg[i], i * n, n)
                fin_cp[i].start()
        with sc_("sa_outwait"):
            ocopy(NB - 2, (NB - 2) % 2).wait()
            for d in fin_cp: d.wait()

    return kernel


def build(cfg):
    TM = cfg.get("TM", 256)
    hbm = pl.BlockSpec(memory_space=pltpu.MemorySpace.HBM)
    def hv(shape, key):
        if key in cfg.get("U32", ""):
            return pltpu.VMEM(shape[:-2] + (shape[-2] // 2, shape[-1]), jnp.uint32)
        return pltpu.VMEM(shape, bf16)
    scratch = [
        pltpu.VMEM((S, M), bf16),
        pltpu.VMEM((S, DC), bf16),
        pltpu.VMEM((S, M), bf16),
        pltpu.VMEM((M, 6 * M), bf16),
        pltpu.VMEM((8, 6 * M), f32),
        pltpu.VMEM((2, M, D), jnp.uint32),
        pltpu.VMEM((NP, DC, D), jnp.uint32),
        pltpu.VMEM((2, DC, D), jnp.uint32),
        pltpu.VMEM((M, 256), bf16), pltpu.VMEM((max(2, cfg.get("KPI", 3)), DC, 256), bf16), pltpu.VMEM((DC, 256), bf16),
        hv((2, 2, S, D), "q"),
        hv((H, S // 128, D, 128), "k"),
        hv((2, 2, S, D), "v"),
        pltpu.VMEM((H + (5 if cfg.get("AL") else 0), S, D), bf16),
        pltpu.VMEM((H * D, M), bf16),
        pltpu.VMEM((M, M), bf16), pltpu.VMEM((M, M), bf16), pltpu.VMEM((F, M), bf16), pltpu.VMEM((F, M), bf16),
        pltpu.VMEM((S + 16, M), f32),
        pltpu.VMEM((2, TM, M), f32), pltpu.VMEM((2, TM, M), f32), pltpu.VMEM((2, TM, M), bf16),
        pltpu.SemaphoreType.DMA((16,)), pltpu.SemaphoreType.DMA((NP,)), pltpu.SemaphoreType.DMA((2, 2)), pltpu.SemaphoreType.DMA((2,)), pltpu.SemaphoreType.DMA((4,)), pltpu.SMEM((1,), jnp.int32),
    ]
    sd = dict(zip(SCR_NAMES, scratch))
    assert len(scratch) == len(SCR_NAMES)
    scratch = [sd[n] if n in sd else pltpu.VMEM((8 * int(n.split("_")[1]), 128), f32) for n in scratch_order(cfg)]
    return pl.pallas_call(
        make_kernel(cfg),
        out_shape=jax.ShapeDtypeStruct((S, M), bf16),
        in_specs=[hbm] * 10 + [pl.BlockSpec(memory_space=pltpu.VMEM), hbm],
        out_specs=hbm,
        scratch_shapes=scratch,
        compiler_params=pltpu.CompilerParams(vmem_limit_bytes=cfg.get("VMEM", 120) * 2**20),
        name="fused_block",
    )


def run(cfg, A_x, A_c_kv, A_w_q, A_w_uk, A_w_uv, A_w_o, B_x, B_w1, B_w2, B_w3, B_w4, c, w_mod):
    out = build(cfg)(A_x.reshape(S, M), A_c_kv.reshape(S, DC), A_w_q, A_w_uk, A_w_uv, A_w_o.reshape(H * D, M),
                     B_w1, B_w2, B_w3.T, B_w4, c, w_mod)
    return out.reshape(1, S, M)


_CFG = {'U32': 'kv', 'ORD': ['ctx_v', 'kT_v'], 'ST': 2, 'NCK': 4, 'A0POS': 8, 'A0D': 8, 'HS': 0, 'FK': 2}


@jax.jit
def pallas_adaLN_cond__compressed_kv_cla__mixer_s_mlp__prompt_kernel(A_x, A_c_kv, A_w_q, A_w_uk, A_w_uv, A_w_o, B_x, B_w1, B_w2, B_w3, B_w4, c, w_mod):
    return run(_CFG, A_x, A_c_kv, A_w_q, A_w_uk, A_w_uv, A_w_o, B_x, B_w1, B_w2, B_w3, B_w4, c, w_mod)
```

```python
import functools
import jax
import jax.numpy as jnp
import numpy as np
from jax.experimental import pallas as pl
from jax.experimental.pallas import tpu as pltpu

S = 2048; M = 640; H = 32; D = 128; DC = 512; F = 1728
NP = H // 2
EPS = 1e-5
LOG2E = 1.4426950408889634
QSCALE = float(D ** -0.5 * LOG2E)
NEG = -1e30
bf16 = jnp.bfloat16; f32 = jnp.float32


def _ln(x):
    m = jnp.mean(x, axis=-1, keepdims=True)
    xc = x - m
    v = jnp.mean(xc * xc, axis=-1, keepdims=True)
    return xc * jax.lax.rsqrt(v + EPS)


def _gelu(x):
    c = 0.7978845608028654
    return 0.5 * x * (1.0 + jnp.tanh(c * (x + 0.044715 * (x * x * x))))


def _rcp(l):
    r = pl.reciprocal(l, approx=True)
    return r * (2.0 - l * r)


def _dot(a, b):
    return jnp.dot(a, b, preferred_element_type=f32)


def _unpack_pair(w32):
    lo = pltpu.bitcast(w32 << 16, f32).astype(bf16)
    hi = pltpu.bitcast(w32 & jnp.uint32(0xFFFF0000), f32).astype(bf16)
    return lo, hi


SCR_NAMES = ['x_v', 'ckv_v', 'h_v', 'wmod_v', 'mod_v', 'wq32', 'wk32', 'wv32', 'wq_s', 'wk_s', 'wv_s', 'q_v', 'kT_v', 'v_v', 'ctx_v', 'wo_v', 'w1_v', 'w2_v', 'w3_v', 'w4_v', 'u_v', 'x1_v', 'h2_v', 'o_v', 'sem', 'ksem', 'wsem', 'osem', 'fsem', 'zs_ref']


def scratch_order(cfg):
    first = cfg.get("ORD", [])
    last = cfg.get("ORL", [])
    return list(first) + [n for n in SCR_NAMES if n not in first and n not in last] + list(last)


def make_kernel(cfg):
    TQ = 128
    PR = cfg.get("PR", 128)
    TM = cfg.get("TM", 256)
    LR = cfg.get("LR", 64)
    NB = S // TM
    NCK = cfg.get("NCK", 4)
    KPI = cfg.get("KPI", 3); P0 = cfg.get("P0", 1)
    assert (NP - P0) % KPI == 0

    import contextlib
    def sc_(name):
        on = cfg.get("SCOPE")
        if name == "barrier": on = cfg.get("BAR", 1)
        if isinstance(on, str): on = name in on.split(",")
        return jax.named_scope(name) if on else contextlib.nullcontext()

    U32 = cfg.get("U32", "")
    def st_(val, key):
        return pltpu.bitcast(val, jnp.uint32) if key in U32 else val
    def ld_(val, key):
        return pltpu.bitcast(val, bf16) if key in U32 else val
    def rs_(r0, n, key):
        return slice(r0 // 2, (r0 + n) // 2) if key in U32 else slice(r0, r0 + n)

    def kernel(x_hbm, ckv_hbm, wq_hbm, wuk_hbm, wuv_hbm, wo_hbm, w1_hbm, w2_hbm, w3_hbm, w4_hbm, c_ref, wmod_hbm,
               out_hbm, *scr):
        R = dict(zip(scratch_order(cfg), scr))
        (x_v, ckv_v, h_v, wmod_v, mod_v, wq32, wk32, wv32, wq_s, wk_s, wv_s, q_v, kT_v, v_v, ctx_v, wo_v, w1_v, w2_v, w3_v, w4_v, u_v, x1_v, h2_v, o_v, sem, ksem, wsem, osem, fsem, zs_ref) = [R[n] for n in SCR_NAMES]
        def cp(src, dst, i):
            return pltpu.make_async_copy(src, dst, sem.at[i])

        def wkcopy(g):
            return pltpu.make_async_copy(wuk_hbm.bitcast(jnp.uint32).at[:, g, :], wk32.at[g], ksem.at[g])

        def wcopies(g, slot):
            return (pltpu.make_async_copy(wq_hbm.bitcast(jnp.uint32).at[:, g, :], wq32.at[slot], wsem.at[0, slot]),
                    pltpu.make_async_copy(wuv_hbm.bitcast(jnp.uint32).at[:, g, :], wv32.at[slot], wsem.at[1, slot]))

        CKB = cfg.get("CKB", [S * j // NCK for j in range(NCK + 1)])
        NCK_ = len(CKB) - 1
        if "C" in U32:
            c_ckv = [cp(ckv_hbm.bitcast(jnp.uint32).at[CKB[j] // 2:CKB[j + 1] // 2], ckv_v.at[CKB[j] // 2:CKB[j + 1] // 2], j) for j in range(NCK_)]
        else:
            c_ckv = [cp(ckv_hbm.at[CKB[j]:CKB[j + 1]], ckv_v.at[CKB[j]:CKB[j + 1]], j) for j in range(NCK_)]
        c_x = cp(x_hbm, x_v, 8); c_wmod = cp(wmod_hbm, wmod_v, 9)
        bc_ = (lambda r_: r_.bitcast(jnp.uint32)) if "W" in U32 else (lambda r_: r_)
        late = [cp(bc_(wo_hbm), wo_v, 10), cp(bc_(w1_hbm), w1_v, 11), cp(bc_(w2_hbm), w2_v, 12), cp(bc_(w3_hbm), w3_v, 13), cp(bc_(w4_hbm), w4_v, 14)]
        wkcopy(0).start(); c_ckv[0].start()
        def rest_start():
            for j in range(1, NCK_): c_ckv[j].start()
            for g2 in range(1, P0 + 1): wkcopy(g2).start()
        if not cfg.get("ST"): rest_start()

        AL = cfg.get("AL", "")
        def vref(bs, hh):
            return ctx_v.at[H + 2 * bs + hh] if "v" in AL else v_v.at[bs, hh]
        def wq_load():
            if "c" in AL:
                return jnp.concatenate([ctx_v[H + 4, 0:M, :], ctx_v[H + 4, M:2 * M, :]], axis=1)
            return ld_(wq_s[...], "w")
        def relayout_q(src):
            if "c" in AL:
                lo, hi = _unpack_pair(src[...])
                ctx_v[H + 4, 0:M, :] = lo
                ctx_v[H + 4, M:2 * M, :] = hi
            else:
                relayout(src, wq_s)

        def relayout(src, dst):
            lo, hi = _unpack_pair(src[...])
            dst[:, 0:128] = st_(lo, "w")
            dst[:, 128:256] = st_(hi, "w")

        def proj_k(g, par, r0):
            rows = slice(r0, r0 + PR)
            k = _dot(ld_(ckv_v[rs_(r0, PR, "C"), :], "C"), ld_(wk_s[par], "w"))
            for hh in range(2):
                for t in range(PR // 128):
                    kT_v[2 * g + hh, (r0 // 128) + t] = st_(k[t * 128:(t + 1) * 128, hh * 128:(hh + 1) * 128].T.astype(bf16), "k")

        def proj_v(bs, r0):
            rows = slice(r0, r0 + PR)
            v = _dot(ld_(ckv_v[rs_(r0, PR, "C"), :], "C"), ld_(wv_s[...], "w")).astype(bf16)
            for hh in range(2): vref(bs, hh)[rs_(r0, PR, "v"), :] = st_(v[:, hh * 128:(hh + 1) * 128], "v")

        def proj_q(bs, r0):
            rows = slice(r0, r0 + PR)
            q = (_dot(ld_(h_v[rs_(r0, PR, "h"), :], "h"), wq_load()) * QSCALE).astype(bf16)
            for hh in range(2): q_v[bs, hh, rs_(r0, PR, "q"), :] = st_(q[:, hh * 128:(hh + 1) * 128], "q")

        LAG = cfg.get("LAG", 0)
        nv_ = {}
        def never():
            return nv_["m"]
        tri = jax.lax.broadcasted_iota(jnp.int32, (128, 128), 1) <= jax.lax.broadcasted_iota(jnp.int32, (128, 128), 0)

        def qk(bs, g, hh, i):
            r0 = i * TQ; nt = i + 1
            q = ld_(q_v[bs, hh, rs_(r0, TQ, "q"), :], "q")
            tiles = [_dot(q, ld_(kT_v[(0 if cfg.get("KFIX") else 2 * g) + hh, t], "k")) for t in range(nt)]
            tiles[-1] = jnp.where(tri, tiles[-1], NEG)
            mx = tiles[0]
            for t in tiles[1:]:
                mx = jnp.maximum(mx, t)
            m = jnp.max(mx, axis=1, keepdims=True)
            return tiles, m

        def smpv(bs, g, hh, i, st):
            tiles, m = st
            r0 = i * TQ
            acc = None; ls = None
            FR = cfg.get("FR", 0) if nv_["on"] else 0
            rold = None
            if FR and len(nv_["rq"]) >= FR:
                rold = jnp.broadcast_to(nv_["rq"].pop(0), (TQ, 128))
            for t, s in enumerate(tiles):
                p = jnp.exp2(s - m)
                FK = cfg.get("FK", 0) if nv_["on"] else 0
                pm = p
                if FK == 1 and ls is not None:
                    pm = jnp.where(never(), ls, p)
                ls = p if ls is None else ls + p
                if FK == 2:
                    pm = jnp.where(never(), ls, p) if t > 0 else p
                if rold is not None and t == min(cfg.get("FRT", 0), len(tiles) - 1):
                    pm = jnp.where(never(), rold, pm)
                o = _dot(pm.astype(bf16), ld_(vref(bs, hh)[rs_(t * 128, 128, "v"), :], "v"))
                acc = o if acc is None else acc + o
            if FR:
                rr_ = _rcp(jnp.sum(ls, axis=1, keepdims=True))
                nv_["rq"].append(rr_)
            def fin():
                r = rr_ if FR else _rcp(jnp.sum(ls, axis=1, keepdims=True))
                ctx_v[2 * g + hh, rs_(r0, TQ, "c"), :] = st_((acc * r).astype(bf16), "c")
            return fin

        def attention(bs, g, items, pieces, fk=True):
            nv_["on"] = fk; nv_["rq"] = []
            if cfg.get("FK"):
                sv = mod_v[0:8, 0:128]
                nv_["m"] = jnp.broadcast_to((sv != sv)[0:1], (128, 128))
                nv_["m1"] = jnp.broadcast_to((sv != sv)[0:1, 0:1], (128, 1))
            st = qk(bs, g, *items[0])
            pend = []
            for n, it in enumerate(items):
                nxt = qk(bs, g, *items[n + 1]) if n + 1 < len(items) else None
                pend.append(smpv(bs, g, *it, st))
                if len(pend) > LAG:
                    pend.pop(0)()
                st = nxt
                if n in pieces:
                    if pieces[n][0] == "flush":
                        for f in pend: f()
                        pend = []
                    for f in pieces[n]:
                        if f != "flush": f()
            for f in pend: f()

        NI = S // TQ
        items_rev = [(hh, i) for hh in range(2) for i in reversed(range(NI))]


        def do_h(rr, dyn=None):
            rows = slice(rr, rr + LR) if dyn is None else pl.ds(pl.multiple_of(dyn + rr, LR), LR)
            hrows = rs_(rr, LR, "h") if dyn is None else rows
            h_v[hrows, :] = st_((_ln(x_v[rows, :].astype(f32)) * (1.0 + mod_v[0:1, M:2 * M]) + mod_v[0:1, 0:M]).astype(bf16), "h")

        def do_mod(a, b):
            cc = c_ref[...].astype(f32)
            sc = (cc * jax.nn.sigmoid(cc)).astype(bf16)
            mod_v[:, a:b] = _dot(jnp.broadcast_to(sc, (8, M)), wmod_v[:, a:b])

        HL = cfg.get("HL", 0)
        def kpair(g, par, nxt, npar, first=False, extra=None):
            for r in range(S // PR):
                if first and (r * PR) in CKB[:-1] and not (r == 0 and cfg.get("ST") == 2):
                    c_ckv[CKB.index(r * PR)].wait()
                proj_k(g, par, r * PR)
                if r == cfg.get("RLP", (S // PR) // 2):
                    if first:
                        for g2 in range(1, P0 + 1): wkcopy(g2).wait()
                        for g2 in range(P0 + 1, NP): wkcopy(g2).start()
                    relayout(wk32.at[nxt], wk_s.at[npar])
                if extra is not None and r in extra: extra[r]()

        with sc_("s1_kphase"):
          with sc_("s1_wait0"):
            wkcopy(0).wait()
            if cfg.get("ST") == 2: c_ckv[0].wait()
          if cfg.get("ST"): rest_start()
          relayout(wk32.at[0], wk_s.at[(0 - P0) % KPI])
          for g in range(P0):
              ex = {}
              if HL:
                  if g == 1:
                      def st1():
                          c_x.start(); c_wmod.start()
                      ex[0] = st1
                  if g == P0 - 2:
                      def st2():
                          for d in wcopies(0, 0): d.start()
                          for d in wcopies(1, 1): d.start()
                      ex[0] = st2
                  if g == P0 - 1:
                      def m1():
                          c_wmod.wait(); do_mod(0, 2 * M)
                      ex[2] = m1
                      ex[9] = lambda: do_mod(2 * M, 4 * M)
                      def m3():
                          do_mod(4 * M, 6 * M); c_x.wait()
                      ex[13] = m3
              kpair(g, (g - P0) % KPI, g + 1, (g + 1 - P0) % KPI, first=(g == 0), extra=ex)

          def kbody(j, carry):
            g = P0 + KPI * j
            c_g = [pltpu.make_async_copy(wuk_hbm.bitcast(jnp.uint32).at[:, jnp.minimum(g + k, NP - 1), :], wk32.at[jnp.minimum(g + k, NP - 1)],
                                         ksem.at[jnp.minimum(g + k, NP - 1)]) for k in range(1, KPI + 1)]
            for k in range(KPI - 1): c_g[k].wait()

            @pl.when(g + KPI < NP)
            def _():
                c_g[KPI - 1].wait()

            if not HL:
                @pl.when(j == cfg.get("XJ", 0))
                def _():
                    c_x.start(); c_wmod.start()
                    for d in wcopies(0, 0): d.start()
                    for d in wcopies(1, 1): d.start()
            NIT_ = (NP - P0) // KPI
            HR = S // NIT_
            nch = HR // LR
            with sc_("barrier"):
              for k in range(KPI):
                ex = {}
                if HL:
                    NR_ = S // PR
                    for ci in range(nch):
                        pos = (ci * KPI * NR_) // nch + 1
                        if pos // NR_ == k:
                            ex[pos % NR_] = functools.partial(do_h, ci * LR, j * HR)
                kpair(g + k, k, jnp.minimum(g + k + 1, NP - 1), (k + 1) % KPI, extra=ex)
            return carry
          with sc_("s1_kloop"):
            jax.lax.fori_loop(0, (NP - P0) // KPI, kbody, 0)

        with sc_("s2_vq0"):
            for d in wcopies(0, 0): d.wait()
            if not HL:
                c_x.wait(); c_wmod.wait()
            for d in late: d.start()
            relayout(wv32.at[0], wv_s); relayout_q(wq32.at[0])
            NR = S // PR
            def vstep(r):
                if r < NR: proj_v(0, r * PR)
                if HL:
                    if r < NR: proj_q(0, r * PR)
                    return
                if r == 0: do_mod(0, 2 * M)
                if r == cfg.get("MODB", NR // 2): do_mod(2 * M, 6 * M)
                if 1 <= r <= NR:
                    for rr in range((r - 1) * PR, r * PR, LR): do_h(rr)
                if r >= 2: proj_q(0, (r - 2) * PR)
            HS = cfg.get("HS", NR)
            if cfg.get("VQ2", 1) and not HL:
                with jax.named_scope("s2_a"):
                    do_mod(0, 2 * M)
                    for r in range(NR):
                        proj_v(0, r * PR)
                        if r < HS:
                            for rr in range(r * PR, (r + 1) * PR, LR): do_h(rr)
                with jax.named_scope("s2_b"):
                    if HS == 0:
                        for rr in range(0, PR * cfg.get("HLEAD", 1), LR): do_h(rr)
                    for r in range(NR):
                        hh_ = (HS if HS > 0 else cfg.get("HLEAD", 1)) + r
                        if HS == 0 and hh_ < NR:
                            for rr in range(hh_ * PR, (hh_ + 1) * PR, LR): do_h(rr)
                        proj_q(0, r * PR)
                        if HS > 0 and hh_ < NR:
                            for rr in range(hh_ * PR, (hh_ + 1) * PR, LR): do_h(rr)
                        if r == cfg.get("MODB", NR // 2): do_mod(2 * M, 6 * M)
            else:
                BV = cfg.get("BARV", 99)
                for r0_ in range(0, NR + 2, BV):
                    with jax.named_scope("vq%d" % r0_):
                        for r in range(r0_, min(NR + 2, r0_ + BV)): vstep(r)

        for d in late[0:0]: d.start()
        def body(g, carry):
            bs = g & 1
            ws = 1 - bs
            for d in wcopies(jnp.minimum(g + 2, NP - 1), bs): d.start()
            with sc_("sj_wait"):
                for d in wcopies(g + 1, ws): d.wait()
            with sc_("sk_relay"):
                relayout(wv32.at[ws], wv_s); relayout_q(wq32.at[ws])
            npieces = S // PR
            its = items_rev if cfg.get("REV", 1) == 1 else ([(hh, i) for hh in range(2) for i in range(NI)] if cfg.get("REV") == 0 else
                  [(0, i) for i in reversed(range(NI))] + [(1, i) for i in range(NI)])
            every = len(items_rev) // npieces
            pieces = {}
            for k in range(npieces):
                pieces[k * every + cfg.get("POFF", 1)] = [functools.partial(proj_v, ws, k * PR), functools.partial(proj_q, ws, k * PR)]
            with sc_("si_iter"):
                attention(bs, g, its, pieces)
            return carry
        with sc_("s5_main"):
            jax.lax.fori_loop(0, NP - 1, body, 0)
        for d in wcopies(NP - 1, (NP - 2) % 2): d.wait()

        for d in late: d.wait()
        zero8 = jnp.zeros((8, M), f32)
        u_v[0:8, :] = zero8; u_v[8 + S:16 + S, :] = zero8
        def modv(j): return mod_v[0:1, j * M:(j + 1) * M]

        def A1(r, slot):
            r0 = pl.multiple_of(r * TM, TM)
            if "c" in U32:
                r0h = pl.multiple_of(r * (TM // 2), TM // 2)
                cx = jnp.concatenate([ld_(ctx_v[hh, pl.ds(r0h, TM // 2), :], "c") for hh in range(H)], axis=1)
            else:
                cx = jnp.concatenate([ctx_v[hh, pl.ds(r0, TM), :] for hh in range(H)], axis=1)
            return _dot(cx, ld_(wo_v[...], "W"))

        def A2(r, slot, a):
            r0 = pl.multiple_of(r * TM, TM)
            outs = []
            for rr in range(0, TM, LR):
                x1 = x_v[pl.ds(r0 + rr, LR), :].astype(f32) + modv(2) * a[rr:rr + LR]
                h2 = _ln(x1) * (1.0 + modv(4)) + modv(3)
                x1_v[slot, rr:rr + LR, :] = x1; h2_v[slot, rr:rr + LR, :] = h2
                outs.append(_ln(h2).astype(bf16))
            return jnp.concatenate(outs, axis=0)

        def A3(r, slot, l2):
            r0 = pl.multiple_of(r * TM, TM)
            u_v[pl.ds(r0 + 8, TM), :] = _gelu(_dot(l2, ld_(w1_v[...], "W")))

        def B1(r, slot, ro=0, n=TM):
            r0 = pl.multiple_of(r * TM, TM) + ro
            lane = jax.lax.broadcasted_iota(jnp.int32, (n, 128), 1)
            def sh(delta, j):
                win = u_v[pl.ds(r0, n + 16), j * 128:(j + 1) * 128]
                return win[8 + delta:8 + delta + n]
            t0 = sh(-1, 0)
            t1 = jnp.where(lane < 32, sh(-1, 1), sh(1, 1))
            t2 = jnp.where(lane < 64, sh(1, 2), sh(-2, 2))
            t3 = jnp.where(lane < 96, sh(-2, 3), sh(2, 3))
            t4 = sh(2, 4)
            return jnp.concatenate([t0, t1, t2, t3, t4], axis=1).astype(bf16)

        def B2(r, slot, us):
            return _dot(us, ld_(w2_v[...], "W"))

        def B3(r, slot, hs, ro=0, n=TM):
            outs = []
            for rr in range(0, n, LR):
                xb1 = h2_v[slot, ro + rr:ro + rr + LR, :] + hs[rr:rr + LR]
                h2_v[slot, ro + rr:ro + rr + LR, :] = xb1
                outs.append(_ln(xb1).astype(bf16))
            return jnp.concatenate(outs, axis=0)

        def B4(r, slot, l3):
            return _gelu(jax.lax.dot_general(l3, ld_(w3_v[...], "W"), (((1,), (1,)), ((), ())), preferred_element_type=f32)).astype(bf16)

        def B5(r, slot, gg, ro=0, n=TM):
            y = _dot(gg, ld_(w4_v[...], "W"))
            o_v[slot, ro:ro + n, :] = (x1_v[slot, ro:ro + n, :] + modv(5) * (h2_v[slot, ro:ro + n, :] + y)).astype(bf16)

        def ocopy(r, slot):
            r0 = pl.multiple_of(r * TM, TM)
            return pltpu.make_async_copy(o_v.at[slot], out_hbm.at[pl.ds(r0, TM)], osem.at[slot])

        with sc_("s6_attn_last"):
            nf = TM // TQ
            if cfg.get("FUSEA0", 1):
                items = [(hh, i) for hh in range(2) for i in range(nf)] + [(hh, i) for hh in range(2) for i in reversed(range(nf, NI))]
                st = {}
                n0 = 2 * nf + cfg.get("A0POS", 1)
                pieces = {n0: ["flush", lambda: st.__setitem__("a", A1(0, 0))],
                          n0 + cfg.get("A0D", 4): [lambda: A3(0, 0, A2(0, 0, st["a"]))]}
                attention((NP - 1) % 2, NP - 1, items, pieces, fk=cfg.get("FKL", 0))
            else:
                attention((NP - 1) % 2, NP - 1, items_rev, {})
                A3(0, 0, A2(0, 0, A1(0, 0)))

        def fbody(r, carry):
            slot = r & 1

            @pl.when(r >= 2)
            def _():
                ocopy(r - 2, slot).wait()
            st = {}
            ops = {
                "B1": lambda: st.__setitem__("us", B1(r, slot)),
                "A1": lambda: st.__setitem__("a", A1(r + 1, 1 - slot)),
                "B2": lambda: st.__setitem__("hs", B2(r, slot, st["us"])),
                "A2": lambda: st.__setitem__("l2", A2(r + 1, 1 - slot, st["a"])),
                "A3": lambda: A3(r + 1, 1 - slot, st["l2"]),
                "B3": lambda: st.__setitem__("l3", B3(r, slot, st["hs"])),
                "B4": lambda: st.__setitem__("gg", B4(r, slot, st["l3"])),
                "B5": lambda: B5(r, slot, st["gg"]),
            }
            for name in cfg.get("FORD", "B1 B2 A1 B3 B4 A2 A3 B5").split():
                if name == "|":
                    with jax.named_scope("zfb"):
                        pass
                else:
                    ops[name]()
            ocopy(r, slot).start()
            return carry
        with sc_("s8_floop"):
            jax.lax.fori_loop(0, NB - 1, fbody, 0)
        ocopy(NB - 3, (NB - 1) % 2).wait()
        sl = (NB - 1) % 2
        with sc_("s9_Blast"):
            nsp = cfg.get("BSPL", 2); n = TM // nsp
            r = NB - 1
            hs = [B2(r, sl, B1(r, sl, i * n, n)) for i in range(nsp)]
            gg = [B4(r, sl, B3(r, sl, hs[i], i * n, n)) for i in range(nsp)]
            fin_cp = [pltpu.make_async_copy(o_v.at[sl, i * n:(i + 1) * n, :], out_hbm.at[r * TM + i * n:r * TM + (i + 1) * n, :], fsem.at[i]) for i in range(nsp)]
            for i in range(nsp):
                B5(r, sl, gg[i], i * n, n)
                fin_cp[i].start()
        with sc_("sa_outwait"):
            ocopy(NB - 2, (NB - 2) % 2).wait()
            for d in fin_cp: d.wait()

    return kernel


def build(cfg):
    TM = cfg.get("TM", 256)
    hbm = pl.BlockSpec(memory_space=pltpu.MemorySpace.HBM)
    def hv(shape, key):
        if key in cfg.get("U32", ""):
            return pltpu.VMEM(shape[:-2] + (shape[-2] // 2, shape[-1]), jnp.uint32)
        return pltpu.VMEM(shape, bf16)
    scratch = [
        pltpu.VMEM((S, M), bf16),
        hv((S, DC), "C"),
        hv((S, M), "h"),
        pltpu.VMEM((M, 6 * M), bf16),
        pltpu.VMEM((8, 6 * M), f32),
        pltpu.VMEM((2, M, D), jnp.uint32),
        pltpu.VMEM((NP, DC, D), jnp.uint32),
        pltpu.VMEM((2, DC, D), jnp.uint32),
        hv((M, 256), "w"), hv((max(2, cfg.get("KPI", 3)), DC, 256), "w"), hv((DC, 256), "w"),
        hv((2, 2, S, D), "q"),
        hv((H, S // 128, D, 128), "k"),
        hv((2, 2, S, D), "v"),
        hv((H + (5 if cfg.get("AL") else 0), S, D), "c"),
        hv((H * D, M), "W"),
        hv((M, M), "W"), hv((M, M), "W"), hv((F, M), "W"), hv((F, M), "W"),
        pltpu.VMEM((S + 16, M), f32),
        pltpu.VMEM((2, TM, M), f32), pltpu.VMEM((2, TM, M), f32), pltpu.VMEM((2, TM, M), bf16),
        pltpu.SemaphoreType.DMA((16,)), pltpu.SemaphoreType.DMA((NP,)), pltpu.SemaphoreType.DMA((2, 2)), pltpu.SemaphoreType.DMA((2,)), pltpu.SemaphoreType.DMA((4,)), pltpu.SMEM((1,), jnp.int32),
    ]
    sd = dict(zip(SCR_NAMES, scratch))
    assert len(scratch) == len(SCR_NAMES)
    scratch = [sd[n] if n in sd else pltpu.VMEM((8 * int(n.split("_")[1]), 128), f32) for n in scratch_order(cfg)]
    return pl.pallas_call(
        make_kernel(cfg),
        out_shape=jax.ShapeDtypeStruct((S, M), bf16),
        in_specs=[hbm] * 10 + [pl.BlockSpec(memory_space=pltpu.VMEM), hbm],
        out_specs=hbm,
        scratch_shapes=scratch,
        compiler_params=pltpu.CompilerParams(vmem_limit_bytes=cfg.get("VMEM", 120) * 2**20),
        name="fused_block",
    )


def run(cfg, A_x, A_c_kv, A_w_q, A_w_uk, A_w_uv, A_w_o, B_x, B_w1, B_w2, B_w3, B_w4, c, w_mod):
    out = build(cfg)(A_x.reshape(S, M), A_c_kv.reshape(S, DC), A_w_q, A_w_uk, A_w_uv, A_w_o.reshape(H * D, M),
                     B_w1, B_w2, B_w3.T, B_w4, c, w_mod)
    return out.reshape(1, S, M)


_CFG = {'U32': 'kvwhCcW', 'ORD': ['ctx_v', 'kT_v'], 'ST': 2, 'NCK': 4, 'A0POS': 8, 'A0D': 8, 'HS': 0, 'FK': 2, 'PR': 256, 'POFF': 1, 'RLP': 4}


@jax.jit
def pallas_adaLN_cond__compressed_kv_cla__mixer_s_mlp__prompt_kernel(A_x, A_c_kv, A_w_q, A_w_uk, A_w_uv, A_w_o, B_x, B_w1, B_w2, B_w3, B_w4, c, w_mod):
    return run(_CFG, A_x, A_c_kv, A_w_q, A_w_uk, A_w_uv, A_w_o, B_x, B_w1, B_w2, B_w3, B_w4, c, w_mod)
```

```python
import functools
import jax
import jax.numpy as jnp
import numpy as np
from jax.experimental import pallas as pl
from jax.experimental.pallas import tpu as pltpu

S = 2048; M = 640; H = 32; D = 128; DC = 512; F = 1728
NP = H // 2
EPS = 1e-5
LOG2E = 1.4426950408889634
QSCALE = float(D ** -0.5 * LOG2E)
NEG = -1e30
bf16 = jnp.bfloat16; f32 = jnp.float32


def _ln(x):
    m = jnp.mean(x, axis=-1, keepdims=True)
    xc = x - m
    v = jnp.mean(xc * xc, axis=-1, keepdims=True)
    return xc * jax.lax.rsqrt(v + EPS)


def _gelu(x):
    c = 0.7978845608028654
    return 0.5 * x * (1.0 + jnp.tanh(c * (x + 0.044715 * (x * x * x))))


def _rcp(l):
    r = pl.reciprocal(l, approx=True)
    return r * (2.0 - l * r)


def _dot(a, b):
    return jnp.dot(a, b, preferred_element_type=f32)


def _unpack_pair(w32):
    lo = pltpu.bitcast(w32 << 16, f32).astype(bf16)
    hi = pltpu.bitcast(w32 & jnp.uint32(0xFFFF0000), f32).astype(bf16)
    return lo, hi


SCR_NAMES = ['x_v', 'ckv_v', 'h_v', 'wmod_v', 'mod_v', 'wq32', 'wk32', 'wv32', 'wq_s', 'wk_s', 'wv_s', 'q_v', 'kT_v', 'v_v', 'ctx_v', 'wo_v', 'w1_v', 'w2_v', 'w3_v', 'w4_v', 'u_v', 'x1_v', 'h2_v', 'o_v', 'sem', 'ksem', 'wsem', 'osem', 'fsem', 'zs_ref']


def scratch_order(cfg):
    first = cfg.get("ORD", [])
    last = cfg.get("ORL", [])
    return list(first) + [n for n in SCR_NAMES if n not in first and n not in last] + list(last)


def make_kernel(cfg):
    TQ = 128
    PR = cfg.get("PR", 128)
    TM = cfg.get("TM", 256)
    LR = cfg.get("LR", 64)
    NB = S // TM
    NCK = cfg.get("NCK", 4)
    KPI = cfg.get("KPI", 3); P0 = cfg.get("P0", 1)
    assert (NP - P0) % KPI == 0

    import contextlib
    def sc_(name):
        on = cfg.get("SCOPE")
        if name == "barrier": on = cfg.get("BAR", 1)
        if isinstance(on, str): on = name in on.split(",")
        return jax.named_scope(name) if on else contextlib.nullcontext()

    U32 = cfg.get("U32", "")
    def st_(val, key):
        return pltpu.bitcast(val, jnp.uint32) if key in U32 else val
    def ld_(val, key):
        return pltpu.bitcast(val, bf16) if key in U32 else val
    def rs_(r0, n, key):
        return slice(r0 // 2, (r0 + n) // 2) if key in U32 else slice(r0, r0 + n)

    def kernel(x_hbm, ckv_hbm, wq_hbm, wuk_hbm, wuv_hbm, wo_hbm, w1_hbm, w2_hbm, w3_hbm, w4_hbm, c_ref, wmod_hbm,
               out_hbm, *scr):
        R = dict(zip(scratch_order(cfg), scr))
        (x_v, ckv_v, h_v, wmod_v, mod_v, wq32, wk32, wv32, wq_s, wk_s, wv_s, q_v, kT_v, v_v, ctx_v, wo_v, w1_v, w2_v, w3_v, w4_v, u_v, x1_v, h2_v, o_v, sem, ksem, wsem, osem, fsem, zs_ref) = [R[n] for n in SCR_NAMES]
        def cp(src, dst, i):
            return pltpu.make_async_copy(src, dst, sem.at[i])

        def wkcopy(g):
            return pltpu.make_async_copy(wuk_hbm.bitcast(jnp.uint32).at[:, g, :], wk32.at[g], ksem.at[g])

        def wcopies(g, slot):
            return (pltpu.make_async_copy(wq_hbm.bitcast(jnp.uint32).at[:, g, :], wq32.at[slot], wsem.at[0, slot]),
                    pltpu.make_async_copy(wuv_hbm.bitcast(jnp.uint32).at[:, g, :], wv32.at[slot], wsem.at[1, slot]))

        CKB = cfg.get("CKB", [S * j // NCK for j in range(NCK + 1)])
        NCK_ = len(CKB) - 1
        if "C" in U32:
            c_ckv = [cp(ckv_hbm.bitcast(jnp.uint32).at[CKB[j] // 2:CKB[j + 1] // 2], ckv_v.at[CKB[j] // 2:CKB[j + 1] // 2], j) for j in range(NCK_)]
        else:
            c_ckv = [cp(ckv_hbm.at[CKB[j]:CKB[j + 1]], ckv_v.at[CKB[j]:CKB[j + 1]], j) for j in range(NCK_)]
        c_x = cp(x_hbm, x_v, 8); c_wmod = cp(wmod_hbm, wmod_v, 9)
        bc_ = (lambda r_: r_.bitcast(jnp.uint32)) if "W" in U32 else (lambda r_: r_)
        late = [cp(bc_(wo_hbm), wo_v, 10), cp(bc_(w1_hbm), w1_v, 11), cp(bc_(w2_hbm), w2_v, 12), cp(bc_(w3_hbm), w3_v, 13), cp(bc_(w4_hbm), w4_v, 14)]
        wkcopy(0).start(); c_ckv[0].start()
        def rest_start():
            for j in range(1, NCK_): c_ckv[j].start()
            for g2 in range(1, P0 + 1): wkcopy(g2).start()
        if not cfg.get("ST"): rest_start()

        AL = cfg.get("AL", "")
        def vref(bs, hh):
            return ctx_v.at[H + 2 * bs + hh] if "v" in AL else v_v.at[bs, hh]
        def wq_load():
            if "c" in AL:
                return jnp.concatenate([ctx_v[H + 4, 0:M, :], ctx_v[H + 4, M:2 * M, :]], axis=1)
            return ld_(wq_s[...], "w")
        def relayout_q(src):
            if "c" in AL:
                lo, hi = _unpack_pair(src[...])
                ctx_v[H + 4, 0:M, :] = lo
                ctx_v[H + 4, M:2 * M, :] = hi
            else:
                relayout(src, wq_s)

        def relayout(src, dst):
            lo, hi = _unpack_pair(src[...])
            dst[:, 0:128] = st_(lo, "w")
            dst[:, 128:256] = st_(hi, "w")

        def proj_k(g, par, r0):
            rows = slice(r0, r0 + PR)
            k = _dot(ld_(ckv_v[rs_(r0, PR, "C"), :], "C"), ld_(wk_s[par], "w"))
            for hh in range(2):
                for t in range(PR // 128):
                    kT_v[2 * g + hh, (r0 // 128) + t] = st_(k[t * 128:(t + 1) * 128, hh * 128:(hh + 1) * 128].T.astype(bf16), "k")

        def proj_v(bs, r0):
            rows = slice(r0, r0 + PR)
            v = _dot(ld_(ckv_v[rs_(r0, PR, "C"), :], "C"), ld_(wv_s[...], "w")).astype(bf16)
            for hh in range(2): vref(bs, hh)[rs_(r0, PR, "v"), :] = st_(v[:, hh * 128:(hh + 1) * 128], "v")

        def proj_q(bs, r0):
            rows = slice(r0, r0 + PR)
            q = (_dot(ld_(h_v[rs_(r0, PR, "h"), :], "h"), wq_load()) * QSCALE).astype(bf16)
            for hh in range(2): q_v[bs, hh, rs_(r0, PR, "q"), :] = st_(q[:, hh * 128:(hh + 1) * 128], "q")

        LAG = cfg.get("LAG", 0)
        nv_ = {}
        def never():
            return nv_["m"]
        tri = jax.lax.broadcasted_iota(jnp.int32, (128, 128), 1) <= jax.lax.broadcasted_iota(jnp.int32, (128, 128), 0)

        def qk(bs, g, hh, i):
            r0 = i * TQ; nt = i + 1
            q = ld_(q_v[bs, hh, rs_(r0, TQ, "q"), :], "q")
            tiles = [_dot(q, ld_(kT_v[(0 if cfg.get("KFIX") else 2 * g) + hh, t], "k")) for t in range(nt)]
            tiles[-1] = jnp.where(tri, tiles[-1], NEG)
            mx = tiles[0]
            for t in tiles[1:]:
                mx = jnp.maximum(mx, t)
            m = jnp.max(mx, axis=1, keepdims=True)
            return tiles, m

        def smpv(bs, g, hh, i, st):
            tiles, m = st
            r0 = i * TQ
            acc = None; ls = None
            FR = cfg.get("FR", 0) if nv_["on"] else 0
            rold = None
            if FR and len(nv_["rq"]) >= FR:
                rold = jnp.broadcast_to(nv_["rq"].pop(0), (TQ, 128))
            for t, s in enumerate(tiles):
                p = jnp.exp2(s - m)
                FK = cfg.get("FK", 0) if nv_["on"] else 0
                pm = p
                if FK == 1 and ls is not None:
                    pm = jnp.where(never(), ls, p)
                ls = p if ls is None else ls + p
                if FK == 2:
                    pm = jnp.where(never(), ls, p) if t > 0 else p
                if rold is not None and t == min(cfg.get("FRT", 0), len(tiles) - 1):
                    pm = jnp.where(never(), rold, pm)
                o = _dot(pm.astype(bf16), ld_(vref(bs, hh)[rs_(t * 128, 128, "v"), :], "v"))
                acc = o if acc is None else acc + o
            if FR:
                rr_ = _rcp(jnp.sum(ls, axis=1, keepdims=True))
                nv_["rq"].append(rr_)
            def fin():
                r = rr_ if FR else _rcp(jnp.sum(ls, axis=1, keepdims=True))
                ctx_v[2 * g + hh, rs_(r0, TQ, "c"), :] = st_((acc * r).astype(bf16), "c")
            return fin

        def attention(bs, g, items, pieces, fk=True):
            nv_["on"] = fk; nv_["rq"] = []
            if cfg.get("FK"):
                sv = mod_v[0:8, 0:128]
                nv_["m"] = jnp.broadcast_to((sv != sv)[0:1], (128, 128))
                nv_["m1"] = jnp.broadcast_to((sv != sv)[0:1, 0:1], (128, 1))
            st = qk(bs, g, *items[0])
            pend = []
            for n, it in enumerate(items):
                nxt = qk(bs, g, *items[n + 1]) if n + 1 < len(items) else None
                pend.append(smpv(bs, g, *it, st))
                if len(pend) > LAG:
                    pend.pop(0)()
                st = nxt
                if n in pieces:
                    if pieces[n][0] == "flush":
                        for f in pend: f()
                        pend = []
                    for f in pieces[n]:
                        if f != "flush": f()
            for f in pend: f()

        NI = S // TQ
        items_rev = [(hh, i) for hh in range(2) for i in reversed(range(NI))]


        def do_h(rr, dyn=None):
            rows = slice(rr, rr + LR) if dyn is None else pl.ds(pl.multiple_of(dyn + rr, LR), LR)
            hrows = rs_(rr, LR, "h") if dyn is None else rows
            h_v[hrows, :] = st_((_ln(x_v[rows, :].astype(f32)) * (1.0 + mod_v[0:1, M:2 * M]) + mod_v[0:1, 0:M]).astype(bf16), "h")

        def do_mod(a, b):
            cc = c_ref[...].astype(f32)
            sc = (cc * jax.nn.sigmoid(cc)).astype(bf16)
            mod_v[:, a:b] = _dot(jnp.broadcast_to(sc, (8, M)), wmod_v[:, a:b])

        HL = cfg.get("HL", 0)
        def kpair(g, par, nxt, npar, first=False, extra=None):
            for r in range(S // PR):
                if first and (r * PR) in CKB[:-1] and not (r == 0 and cfg.get("ST") == 2):
                    c_ckv[CKB.index(r * PR)].wait()
                proj_k(g, par, r * PR)
                if r == cfg.get("RLP", (S // PR) // 2):
                    if first:
                        for g2 in range(1, P0 + 1): wkcopy(g2).wait()
                        for g2 in range(P0 + 1, min(NP, P0 + 1 + cfg.get("WKE", 99))): wkcopy(g2).start()
                    relayout(wk32.at[nxt], wk_s.at[npar])
                if first and r == S // PR - 1:
                    for g2 in range(P0 + 1 + cfg.get("WKE", 99), NP): wkcopy(g2).start()
                if extra is not None and r in extra: extra[r]()

        with sc_("s1_kphase"):
          with sc_("s1_wait0"):
            wkcopy(0).wait()
            if cfg.get("ST") == 2: c_ckv[0].wait()
          if cfg.get("ST"): rest_start()
          relayout(wk32.at[0], wk_s.at[(0 - P0) % KPI])
          for g in range(P0):
              ex = {}
              if HL:
                  if g == 1:
                      def st1():
                          c_x.start(); c_wmod.start()
                      ex[0] = st1
                  if g == P0 - 2:
                      def st2():
                          for d in wcopies(0, 0): d.start()
                          for d in wcopies(1, 1): d.start()
                      ex[0] = st2
                  if g == P0 - 1:
                      def m1():
                          c_wmod.wait(); do_mod(0, 2 * M)
                      ex[2] = m1
                      ex[9] = lambda: do_mod(2 * M, 4 * M)
                      def m3():
                          do_mod(4 * M, 6 * M); c_x.wait()
                      ex[13] = m3
              kpair(g, (g - P0) % KPI, g + 1, (g + 1 - P0) % KPI, first=(g == 0), extra=ex)

          def kbody(j, carry):
            g = P0 + KPI * j
            c_g = [pltpu.make_async_copy(wuk_hbm.bitcast(jnp.uint32).at[:, jnp.minimum(g + k, NP - 1), :], wk32.at[jnp.minimum(g + k, NP - 1)],
                                         ksem.at[jnp.minimum(g + k, NP - 1)]) for k in range(1, KPI + 1)]
            for k in range(KPI - 1): c_g[k].wait()

            @pl.when(g + KPI < NP)
            def _():
                c_g[KPI - 1].wait()

            if not HL:
                @pl.when(j == cfg.get("XJ", 0))
                def _():
                    c_x.start(); c_wmod.start()
                    for d in wcopies(0, 0): d.start()
                    for d in wcopies(1, 1): d.start()
            NIT_ = (NP - P0) // KPI
            HR = S // NIT_
            nch = HR // LR
            with sc_("barrier"):
              for k in range(KPI):
                ex = {}
                if HL:
                    NR_ = S // PR
                    for ci in range(nch):
                        pos = (ci * KPI * NR_) // nch + 1
                        if pos // NR_ == k:
                            ex[pos % NR_] = functools.partial(do_h, ci * LR, j * HR)
                kpair(g + k, k, jnp.minimum(g + k + 1, NP - 1), (k + 1) % KPI, extra=ex)
            return carry
          with sc_("s1_kloop"):
            jax.lax.fori_loop(0, (NP - P0) // KPI, kbody, 0)

        with sc_("s2_vq0"):
            for d in wcopies(0, 0): d.wait()
            if not HL:
                c_x.wait(); c_wmod.wait()
            for d in late: d.start()
            relayout(wv32.at[0], wv_s); relayout_q(wq32.at[0])
            NR = S // PR
            def vstep(r):
                if r < NR: proj_v(0, r * PR)
                if HL:
                    if r < NR: proj_q(0, r * PR)
                    return
                if r == 0: do_mod(0, 2 * M)
                if r == cfg.get("MODB", NR // 2): do_mod(2 * M, 6 * M)
                if 1 <= r <= NR:
                    for rr in range((r - 1) * PR, r * PR, LR): do_h(rr)
                if r >= 2: proj_q(0, (r - 2) * PR)
            HS = cfg.get("HS", NR)
            if cfg.get("VQ2", 1) and not HL:
                with jax.named_scope("s2_a"):
                    do_mod(0, 2 * M)
                    for r in range(NR):
                        proj_v(0, r * PR)
                        if r < HS:
                            for rr in range(r * PR, (r + 1) * PR, LR): do_h(rr)
                with jax.named_scope("s2_b"):
                    if HS == 0:
                        for rr in range(0, PR * cfg.get("HLEAD", 1), LR): do_h(rr)
                    for r in range(NR):
                        hh_ = (HS if HS > 0 else cfg.get("HLEAD", 1)) + r
                        if HS == 0 and hh_ < NR:
                            for rr in range(hh_ * PR, (hh_ + 1) * PR, LR): do_h(rr)
                        proj_q(0, r * PR)
                        if HS > 0 and hh_ < NR:
                            for rr in range(hh_ * PR, (hh_ + 1) * PR, LR): do_h(rr)
                        if cfg.get("MODS", 1):
                            nt_ = 4 * M // 128
                            a_ = (r * nt_) // NR; b_ = ((r + 1) * nt_) // NR
                            if b_ > a_: do_mod(2 * M + a_ * 128, 2 * M + b_ * 128)
                        elif r == cfg.get("MODB", NR // 2): do_mod(2 * M, 6 * M)
            else:
                BV = cfg.get("BARV", 99)
                for r0_ in range(0, NR + 2, BV):
                    with jax.named_scope("vq%d" % r0_):
                        for r in range(r0_, min(NR + 2, r0_ + BV)): vstep(r)

        for d in late[0:0]: d.start()
        def body(g, carry):
            bs = g & 1
            ws = 1 - bs
            for d in wcopies(jnp.minimum(g + 2, NP - 1), bs): d.start()
            with sc_("sj_wait"):
                for d in wcopies(g + 1, ws): d.wait()
            with sc_("sk_relay"):
                relayout(wv32.at[ws], wv_s); relayout_q(wq32.at[ws])
            npieces = S // PR
            its = items_rev if cfg.get("REV", 1) == 1 else ([(hh, i) for hh in range(2) for i in range(NI)] if cfg.get("REV") == 0 else
                  [(0, i) for i in reversed(range(NI))] + [(1, i) for i in range(NI)])
            every = len(items_rev) // npieces
            pieces = {}
            for k in range(npieces):
                pieces[k * every + cfg.get("POFF", 1)] = [functools.partial(proj_v, ws, k * PR), functools.partial(proj_q, ws, k * PR)]
            with sc_("si_iter"):
                attention(bs, g, its, pieces)
            return carry
        with sc_("s5_main"):
            jax.lax.fori_loop(0, NP - 1, body, 0)
        for d in wcopies(NP - 1, (NP - 2) % 2): d.wait()

        for d in late: d.wait()
        zero8 = jnp.zeros((8, M), f32)
        u_v[0:8, :] = zero8; u_v[8 + S:16 + S, :] = zero8
        def modv(j): return mod_v[0:1, j * M:(j + 1) * M]

        def A1(r, slot):
            r0 = pl.multiple_of(r * TM, TM)
            if "c" in U32:
                r0h = pl.multiple_of(r * (TM // 2), TM // 2)
                cx = jnp.concatenate([ld_(ctx_v[hh, pl.ds(r0h, TM // 2), :], "c") for hh in range(H)], axis=1)
            else:
                cx = jnp.concatenate([ctx_v[hh, pl.ds(r0, TM), :] for hh in range(H)], axis=1)
            return _dot(cx, ld_(wo_v[...], "W"))

        def A2(r, slot, a):
            r0 = pl.multiple_of(r * TM, TM)
            outs = []
            for rr in range(0, TM, LR):
                x1 = x_v[pl.ds(r0 + rr, LR), :].astype(f32) + modv(2) * a[rr:rr + LR]
                h2 = _ln(x1) * (1.0 + modv(4)) + modv(3)
                x1_v[slot, rr:rr + LR, :] = x1; h2_v[slot, rr:rr + LR, :] = h2
                outs.append(_ln(h2).astype(bf16))
            return jnp.concatenate(outs, axis=0)

        def A3(r, slot, l2):
            r0 = pl.multiple_of(r * TM, TM)
            u_v[pl.ds(r0 + 8, TM), :] = _gelu(_dot(l2, ld_(w1_v[...], "W")))

        def B1(r, slot, ro=0, n=TM):
            r0 = pl.multiple_of(r * TM, TM) + ro
            lane = jax.lax.broadcasted_iota(jnp.int32, (n, 128), 1)
            def sh(delta, j):
                win = u_v[pl.ds(r0, n + 16), j * 128:(j + 1) * 128]
                return win[8 + delta:8 + delta + n]
            t0 = sh(-1, 0)
            t1 = jnp.where(lane < 32, sh(-1, 1), sh(1, 1))
            t2 = jnp.where(lane < 64, sh(1, 2), sh(-2, 2))
            t3 = jnp.where(lane < 96, sh(-2, 3), sh(2, 3))
            t4 = sh(2, 4)
            return jnp.concatenate([t0, t1, t2, t3, t4], axis=1).astype(bf16)

        def B2(r, slot, us):
            return _dot(us, ld_(w2_v[...], "W"))

        def B3(r, slot, hs, ro=0, n=TM):
            outs = []
            for rr in range(0, n, LR):
                xb1 = h2_v[slot, ro + rr:ro + rr + LR, :] + hs[rr:rr + LR]
                h2_v[slot, ro + rr:ro + rr + LR, :] = xb1
                outs.append(_ln(xb1).astype(bf16))
            return jnp.concatenate(outs, axis=0)

        def B4(r, slot, l3):
            return _gelu(jax.lax.dot_general(l3, ld_(w3_v[...], "W"), (((1,), (1,)), ((), ())), preferred_element_type=f32)).astype(bf16)

        def B5(r, slot, gg, osl, ro=0, n=TM):
            y = _dot(gg, ld_(w4_v[...], "W"))
            o_v[osl, ro:ro + n, :] = (x1_v[slot, ro:ro + n, :] + modv(5) * (h2_v[slot, ro:ro + n, :] + y)).astype(bf16)

        def ocopy(r, slot):
            r0 = pl.multiple_of(r * TM, TM)
            return pltpu.make_async_copy(o_v.at[slot], out_hbm.at[pl.ds(r0, TM)], osem.at[slot])

        with sc_("s6_attn_last"):
            nf = 2 * TM // TQ
            items = [(hh, i) for hh in range(2) for i in range(nf)] + [(hh, i) for hh in range(2) for i in reversed(range(nf, NI))]
            st = {}
            n0 = 2 * nf + cfg.get("A0POS", 1); dd = cfg.get("A0D", 4)
            pieces = {n0: ["flush", lambda: st.__setitem__("a0", A1(0, 0))],
                      n0 + dd: [lambda: st.__setitem__("l0", A2(0, 0, st["a0"]))],
                      n0 + 2 * dd: [lambda: st.__setitem__("a1", A1(1, 1))],
                      n0 + 3 * dd: [lambda: A3(0, 0, st["l0"])],
                      min(n0 + 4 * dd, len(items) - 1): [lambda: A3(1, 1, A2(1, 1, st["a1"]))]}
            assert len(pieces) == 5
            attention((NP - 1) % 2, NP - 1, items, pieces, fk=cfg.get("FKL", 0))

        def fbody(t, sa):
            sb = jnp.where(sa == 2, 0, sa + 1)
            osl = t & 1

            @pl.when(t >= 2)
            def _():
                ocopy(t - 2, osl).wait()
            st = {}
            ops = {
                "B1": lambda: st.__setitem__("us", B1(t, sb)),
                "A1": lambda: st.__setitem__("a", A1(t + 2, sa)),
                "B2": lambda: st.__setitem__("hs", B2(t, sb, st["us"])),
                "A2": lambda: st.__setitem__("l2", A2(t + 2, sa, st["a"])),
                "A3": lambda: A3(t + 2, sa, st["l2"]),
                "B3": lambda: st.__setitem__("l3", B3(t, sb, st["hs"])),
                "B4": lambda: st.__setitem__("gg", B4(t, sb, st["l3"])),
                "B5": lambda: B5(t, sb, st["gg"], osl),
            }
            for name in cfg.get("FORD", "B1 B2 A1 B3 B4 A2 A3 B5").split():
                ops[name]()
            ocopy(t, osl).start()
            return sb
        with sc_("s8_floop"):
            jax.lax.fori_loop(0, NB - 2, fbody, 2)
        with sc_("s9_Blast"):
            ocopy(NB - 4, 0).wait(); ocopy(NB - 3, 1).wait()
            rs2 = (NB - 2, NB - 1)
            hs = [B2(r, r % 3, B1(r, r % 3)) for r in rs2]
            gg = [B4(r, r % 3, B3(r, r % 3, hs[i])) for i, r in enumerate(rs2)]
            for i, r in enumerate(rs2):
                B5(r, r % 3, gg[i], r & 1)
                ocopy(r, r & 1).start()
        with sc_("sa_outwait"):
            ocopy(NB - 2, 0).wait()
            ocopy(NB - 1, 1).wait()

    return kernel


def build(cfg):
    TM = cfg.get("TM", 256)
    hbm = pl.BlockSpec(memory_space=pltpu.MemorySpace.HBM)
    def hv(shape, key):
        if key in cfg.get("U32", ""):
            return pltpu.VMEM(shape[:-2] + (shape[-2] // 2, shape[-1]), jnp.uint32)
        return pltpu.VMEM(shape, bf16)
    scratch = [
        pltpu.VMEM((S, M), bf16),
        hv((S, DC), "C"),
        hv((S, M), "h"),
        pltpu.VMEM((M, 6 * M), bf16),
        pltpu.VMEM((8, 6 * M), f32),
        pltpu.VMEM((2, M, D), jnp.uint32),
        pltpu.VMEM((NP, DC, D), jnp.uint32),
        pltpu.VMEM((2, DC, D), jnp.uint32),
        hv((M, 256), "w"), hv((max(2, cfg.get("KPI", 3)), DC, 256), "w"), hv((DC, 256), "w"),
        hv((2, 2, S, D), "q"),
        hv((H, S // 128, D, 128), "k"),
        hv((2, 2, S, D), "v"),
        hv((H + (5 if cfg.get("AL") else 0), S, D), "c"),
        hv((H * D, M), "W"),
        hv((M, M), "W"), hv((M, M), "W"), hv((F, M), "W"), hv((F, M), "W"),
        pltpu.VMEM((S + 16, M), f32),
        pltpu.VMEM((3, TM, M), f32), pltpu.VMEM((3, TM, M), f32), pltpu.VMEM((2, TM, M), bf16),
        pltpu.SemaphoreType.DMA((16,)), pltpu.SemaphoreType.DMA((NP,)), pltpu.SemaphoreType.DMA((2, 2)), pltpu.SemaphoreType.DMA((2,)), pltpu.SemaphoreType.DMA((4,)), pltpu.SMEM((1,), jnp.int32),
    ]
    sd = dict(zip(SCR_NAMES, scratch))
    assert len(scratch) == len(SCR_NAMES)
    scratch = [sd[n] if n in sd else pltpu.VMEM((8 * int(n.split("_")[1]), 128), f32) for n in scratch_order(cfg)]
    return pl.pallas_call(
        make_kernel(cfg),
        out_shape=jax.ShapeDtypeStruct((S, M), bf16),
        in_specs=[hbm] * 10 + [pl.BlockSpec(memory_space=pltpu.VMEM), hbm],
        out_specs=hbm,
        scratch_shapes=scratch,
        compiler_params=pltpu.CompilerParams(vmem_limit_bytes=cfg.get("VMEM", 120) * 2**20),
        name="fused_block",
    )


def run(cfg, A_x, A_c_kv, A_w_q, A_w_uk, A_w_uv, A_w_o, B_x, B_w1, B_w2, B_w3, B_w4, c, w_mod):
    out = build(cfg)(A_x.reshape(S, M), A_c_kv.reshape(S, DC), A_w_q, A_w_uk, A_w_uv, A_w_o.reshape(H * D, M),
                     B_w1, B_w2, B_w3.T, B_w4, c, w_mod)
    return out.reshape(1, S, M)


_CFG = {'U32': 'kvwhCcW', 'ORD': ['ctx_v', 'kT_v'], 'ST': 0, 'NCK': 4, 'A0POS': 2, 'A0D': 4, 'HS': 0, 'FK': 2, 'PR': 256, 'POFF': 1, 'RLP': 4, 'WKE': 3, 'CKB': [0, 1024, 2048]}


@jax.jit
def pallas_adaLN_cond__compressed_kv_cla__mixer_s_mlp__prompt_kernel(A_x, A_c_kv, A_w_q, A_w_uk, A_w_uv, A_w_o, B_x, B_w1, B_w2, B_w3, B_w4, c, w_mod):
    return run(_CFG, A_x, A_c_kv, A_w_q, A_w_uk, A_w_uv, A_w_o, B_x, B_w1, B_w2, B_w3, B_w4, c, w_mod)
```

```python
import functools
import jax
import jax.numpy as jnp
import numpy as np
from jax.experimental import pallas as pl
from jax.experimental.pallas import tpu as pltpu

S = 2048; M = 640; H = 32; D = 128; DC = 512; F = 1728
NP = H // 2
EPS = 1e-5
LOG2E = 1.4426950408889634
QSCALE = float(D ** -0.5 * LOG2E)
NEG = -1e30
bf16 = jnp.bfloat16; f32 = jnp.float32


def _ln(x):
    m = jnp.mean(x, axis=-1, keepdims=True)
    xc = x - m
    v = jnp.mean(xc * xc, axis=-1, keepdims=True)
    return xc * jax.lax.rsqrt(v + EPS)


def _gelu(x):
    c = 0.7978845608028654
    return 0.5 * x * (1.0 + jnp.tanh(c * (x + 0.044715 * (x * x * x))))


def _rcp(l):
    r = pl.reciprocal(l, approx=True)
    return r * (2.0 - l * r)


def _dot(a, b):
    return jnp.dot(a, b, preferred_element_type=f32)


def _unpack_pair(w32):
    lo = pltpu.bitcast(w32 << 16, f32).astype(bf16)
    hi = pltpu.bitcast(w32 & jnp.uint32(0xFFFF0000), f32).astype(bf16)
    return lo, hi


SCR_NAMES = ['x_v', 'ckv_v', 'h_v', 'wmod_v', 'mod_v', 'wq32', 'wk32', 'wv32', 'wq_s', 'wk_s', 'wv_s', 'q_v', 'kT_v', 'v_v', 'ctx_v', 'wo_v', 'w1_v', 'w2_v', 'w3_v', 'w4_v', 'u_v', 'x1_v', 'h2_v', 'o_v', 'sem', 'ksem', 'wsem', 'osem', 'fsem', 'zs_ref']


def scratch_order(cfg):
    first = cfg.get("ORD", [])
    last = cfg.get("ORL", [])
    return list(first) + [n for n in SCR_NAMES if n not in first and n not in last] + list(last)


def make_kernel(cfg):
    TQ = 128
    PR = cfg.get("PR", 128)
    TM = cfg.get("TM", 256)
    LR = cfg.get("LR", 64)
    NB = S // TM
    NCK = cfg.get("NCK", 4)
    KPI = cfg.get("KPI", 3); P0 = cfg.get("P0", 1)
    assert (NP - P0) % KPI == 0

    import contextlib
    def sc_(name):
        on = cfg.get("SCOPE")
        if name == "barrier": on = cfg.get("BAR", 1)
        if isinstance(on, str): on = name in on.split(",")
        return jax.named_scope(name) if on else contextlib.nullcontext()

    U32 = cfg.get("U32", "")
    def st_(val, key):
        return pltpu.bitcast(val, jnp.uint32) if key in U32 else val
    def ld_(val, key):
        return pltpu.bitcast(val, bf16) if key in U32 else val
    def rs_(r0, n, key):
        return slice(r0 // 2, (r0 + n) // 2) if key in U32 else slice(r0, r0 + n)

    def kernel(x_hbm, ckv_hbm, wq_hbm, wuk_hbm, wuv_hbm, wo_hbm, w1_hbm, w2_hbm, w3_hbm, w4_hbm, c_ref, wmod_hbm,
               out_hbm, *scr):
        R = dict(zip(scratch_order(cfg), scr))
        (x_v, ckv_v, h_v, wmod_v, mod_v, wq32, wk32, wv32, wq_s, wk_s, wv_s, q_v, kT_v, v_v, ctx_v, wo_v, w1_v, w2_v, w3_v, w4_v, u_v, x1_v, h2_v, o_v, sem, ksem, wsem, osem, fsem, zs_ref) = [R[n] for n in SCR_NAMES]
        def cp(src, dst, i):
            return pltpu.make_async_copy(src, dst, sem.at[i])

        def wkcopy(g):
            return pltpu.make_async_copy(wuk_hbm.bitcast(jnp.uint32).at[:, g, :], wk32.at[g], ksem.at[g])

        def wcopies(g, slot):
            return (pltpu.make_async_copy(wq_hbm.bitcast(jnp.uint32).at[:, g, :], wq32.at[slot], wsem.at[0, slot]),
                    pltpu.make_async_copy(wuv_hbm.bitcast(jnp.uint32).at[:, g, :], wv32.at[slot], wsem.at[1, slot]))

        CKB = cfg.get("CKB", [S * j // NCK for j in range(NCK + 1)])
        NCK_ = len(CKB) - 1
        if "C" in U32:
            c_ckv = [cp(ckv_hbm.bitcast(jnp.uint32).at[CKB[j] // 2:CKB[j + 1] // 2], ckv_v.at[CKB[j] // 2:CKB[j + 1] // 2], j) for j in range(NCK_)]
        else:
            c_ckv = [cp(ckv_hbm.at[CKB[j]:CKB[j + 1]], ckv_v.at[CKB[j]:CKB[j + 1]], j) for j in range(NCK_)]
        c_x = cp(x_hbm, x_v, 8); c_wmod = cp(wmod_hbm, wmod_v, 9)
        bc_ = (lambda r_: r_.bitcast(jnp.uint32)) if "W" in U32 else (lambda r_: r_)
        late = [cp(bc_(wo_hbm), wo_v, 10), cp(bc_(w1_hbm), w1_v, 11), cp(bc_(w2_hbm), w2_v, 12), cp(bc_(w3_hbm), w3_v, 13), cp(bc_(w4_hbm), w4_v, 14)]
        wkcopy(0).start(); c_ckv[0].start()
        def rest_start():
            for j in range(1, NCK_): c_ckv[j].start()
            for g2 in range(1, P0 + 1): wkcopy(g2).start()
        if not cfg.get("ST"): rest_start()

        AL = cfg.get("AL", "")
        def vref(bs, hh):
            return ctx_v.at[H + 2 * bs + hh] if "v" in AL else v_v.at[bs, hh]
        def wq_load():
            if "c" in AL:
                return jnp.concatenate([ctx_v[H + 4, 0:M, :], ctx_v[H + 4, M:2 * M, :]], axis=1)
            return ld_(wq_s[...], "w")
        def relayout_q(src):
            if "c" in AL:
                lo, hi = _unpack_pair(src[...])
                ctx_v[H + 4, 0:M, :] = lo
                ctx_v[H + 4, M:2 * M, :] = hi
            else:
                relayout(src, wq_s)

        def relayout(src, dst):
            lo, hi = _unpack_pair(src[...])
            dst[:, 0:128] = st_(lo, "w")
            dst[:, 128:256] = st_(hi, "w")

        def proj_k(g, par, r0):
            rows = slice(r0, r0 + PR)
            k = _dot(ld_(ckv_v[rs_(r0, PR, "C"), :], "C"), ld_(wk_s[par], "w"))
            for hh in range(2):
                for t in range(PR // 128):
                    kT_v[2 * g + hh, (r0 // 128) + t] = st_(k[t * 128:(t + 1) * 128, hh * 128:(hh + 1) * 128].T.astype(bf16), "k")

        def proj_v(bs, r0):
            rows = slice(r0, r0 + PR)
            v = _dot(ld_(ckv_v[rs_(r0, PR, "C"), :], "C"), ld_(wv_s[...], "w")).astype(bf16)
            for hh in range(2): vref(bs, hh)[rs_(r0, PR, "v"), :] = st_(v[:, hh * 128:(hh + 1) * 128], "v")

        def proj_q(bs, r0):
            rows = slice(r0, r0 + PR)
            q = (_dot(ld_(h_v[rs_(r0, PR, "h"), :], "h"), wq_load()) * QSCALE).astype(bf16)
            for hh in range(2): q_v[bs, hh, rs_(r0, PR, "q"), :] = st_(q[:, hh * 128:(hh + 1) * 128], "q")

        LAG = cfg.get("LAG", 0)
        nv_ = {}
        def never():
            return nv_["m"]
        tri = jax.lax.broadcasted_iota(jnp.int32, (128, 128), 1) <= jax.lax.broadcasted_iota(jnp.int32, (128, 128), 0)

        def qk(bs, g, hh, i):
            r0 = i * TQ; nt = i + 1
            q = ld_(q_v[bs, hh, rs_(r0, TQ, "q"), :], "q")
            tiles = [_dot(q, ld_(kT_v[(0 if cfg.get("KFIX") else 2 * g) + hh, t], "k")) for t in range(nt)]
            tiles[-1] = jnp.where(tri, tiles[-1], NEG)
            mx = tiles[0]
            for t in tiles[1:]:
                mx = jnp.maximum(mx, t)
            m = jnp.max(mx, axis=1, keepdims=True)
            return tiles, m

        def smpv(bs, g, hh, i, st):
            tiles, m = st
            r0 = i * TQ
            acc = None; ls = None
            FR = cfg.get("FR", 0) if nv_["on"] else 0
            rold = None
            if FR and len(nv_["rq"]) >= FR:
                rold = jnp.broadcast_to(nv_["rq"].pop(0), (TQ, 128))
            for t, s in enumerate(tiles):
                p = jnp.exp2(s - m)
                FK = cfg.get("FK", 0) if nv_["on"] else 0
                pm = p
                if FK == 1 and ls is not None:
                    pm = jnp.where(never(), ls, p)
                ls = p if ls is None else ls + p
                if FK == 2:
                    pm = jnp.where(never(), ls, p) if t > 0 else p
                if rold is not None and t == min(cfg.get("FRT", 0), len(tiles) - 1):
                    pm = jnp.where(never(), rold, pm)
                o = _dot(pm.astype(bf16), ld_(vref(bs, hh)[rs_(t * 128, 128, "v"), :], "v"))
                acc = o if acc is None else acc + o
            if FR:
                rr_ = _rcp(jnp.sum(ls, axis=1, keepdims=True))
                nv_["rq"].append(rr_)
            def fin():
                r = rr_ if FR else _rcp(jnp.sum(ls, axis=1, keepdims=True))
                ctx_v[2 * g + hh, rs_(r0, TQ, "c"), :] = st_((acc * r).astype(bf16), "c")
            return fin

        def attention(bs, g, items, pieces, fk=True):
            nv_["on"] = fk; nv_["rq"] = []
            if cfg.get("FK"):
                sv = mod_v[0:8, 0:128]
                nv_["m"] = jnp.broadcast_to((sv != sv)[0:1], (128, 128))
                nv_["m1"] = jnp.broadcast_to((sv != sv)[0:1, 0:1], (128, 1))
            st = qk(bs, g, *items[0])
            pend = []
            for n, it in enumerate(items):
                nxt = qk(bs, g, *items[n + 1]) if n + 1 < len(items) else None
                pend.append(smpv(bs, g, *it, st))
                if len(pend) > LAG:
                    pend.pop(0)()
                st = nxt
                if n in pieces:
                    if pieces[n][0] == "flush":
                        for f in pend: f()
                        pend = []
                    for f in pieces[n]:
                        if f != "flush": f()
            for f in pend: f()

        NI = S // TQ
        items_rev = [(hh, i) for hh in range(2) for i in reversed(range(NI))]


        def do_h(rr, dyn=None):
            rows = slice(rr, rr + LR) if dyn is None else pl.ds(pl.multiple_of(dyn + rr, LR), LR)
            hrows = rs_(rr, LR, "h") if dyn is None else rows
            h_v[hrows, :] = st_((_ln(x_v[rows, :].astype(f32)) * (1.0 + mod_v[0:1, M:2 * M]) + mod_v[0:1, 0:M]).astype(bf16), "h")

        def do_mod(a, b):
            cc = c_ref[...].astype(f32)
            sc = (cc * jax.nn.sigmoid(cc)).astype(bf16)
            mod_v[:, a:b] = _dot(jnp.broadcast_to(sc, (8, M)), wmod_v[:, a:b])

        HL = cfg.get("HL", 0)
        def kpair(g, par, nxt, npar, first=False, extra=None):
            for r in range(S // PR):
                if first and (r * PR) in CKB[:-1] and not (r == 0 and cfg.get("ST") == 2):
                    c_ckv[CKB.index(r * PR)].wait()
                proj_k(g, par, r * PR)
                if r == cfg.get("RLP", (S // PR) // 2):
                    if first:
                        for g2 in range(1, P0 + 1): wkcopy(g2).wait()
                        for g2 in range(P0 + 1, min(NP, P0 + 1 + cfg.get("WKE", 99))): wkcopy(g2).start()
                    relayout(wk32.at[nxt], wk_s.at[npar])
                if first and r == S // PR - 1:
                    for g2 in range(P0 + 1 + cfg.get("WKE", 99), NP): wkcopy(g2).start()
                if extra is not None and r in extra: extra[r]()

        with sc_("s1_kphase"):
          with sc_("s1_wait0"):
            wkcopy(0).wait()
            if cfg.get("ST") == 2: c_ckv[0].wait()
          if cfg.get("ST"): rest_start()
          relayout(wk32.at[0], wk_s.at[(0 - P0) % KPI])
          for g in range(P0):
              ex = {}
              if HL:
                  if g == 1:
                      def st1():
                          c_x.start(); c_wmod.start()
                      ex[0] = st1
                  if g == P0 - 2:
                      def st2():
                          for d in wcopies(0, 0): d.start()
                          for d in wcopies(1, 1): d.start()
                      ex[0] = st2
                  if g == P0 - 1:
                      def m1():
                          c_wmod.wait(); do_mod(0, 2 * M)
                      ex[2] = m1
                      ex[9] = lambda: do_mod(2 * M, 4 * M)
                      def m3():
                          do_mod(4 * M, 6 * M); c_x.wait()
                      ex[13] = m3
              kpair(g, (g - P0) % KPI, g + 1, (g + 1 - P0) % KPI, first=(g == 0), extra=ex)

          def kbody(j, carry):
            g = P0 + KPI * j
            c_g = [pltpu.make_async_copy(wuk_hbm.bitcast(jnp.uint32).at[:, jnp.minimum(g + k, NP - 1), :], wk32.at[jnp.minimum(g + k, NP - 1)],
                                         ksem.at[jnp.minimum(g + k, NP - 1)]) for k in range(1, KPI + 1)]
            for k in range(KPI - 1): c_g[k].wait()

            @pl.when(g + KPI < NP)
            def _():
                c_g[KPI - 1].wait()

            if not HL:
                @pl.when(j == cfg.get("XJ", 0))
                def _():
                    c_x.start(); c_wmod.start()
                    for d in wcopies(0, 0): d.start()
                    for d in wcopies(1, 1): d.start()
            NIT_ = (NP - P0) // KPI
            HR = S // NIT_
            nch = HR // LR
            with sc_("barrier"):
              for k in range(KPI):
                ex = {}
                if HL:
                    NR_ = S // PR
                    for ci in range(nch):
                        pos = (ci * KPI * NR_) // nch + 1
                        if pos // NR_ == k:
                            ex[pos % NR_] = functools.partial(do_h, ci * LR, j * HR)
                kpair(g + k, k, jnp.minimum(g + k + 1, NP - 1), (k + 1) % KPI, extra=ex)
            return carry
          with sc_("s1_kloop"):
            jax.lax.fori_loop(0, (NP - P0) // KPI, kbody, 0)

        with sc_("s2_vq0"):
            for d in wcopies(0, 0): d.wait()
            if not HL:
                c_x.wait(); c_wmod.wait()
            for d in late: d.start()
            relayout(wv32.at[0], wv_s); relayout_q(wq32.at[0])
            NR = S // PR
            def vstep(r):
                if r < NR: proj_v(0, r * PR)
                if HL:
                    if r < NR: proj_q(0, r * PR)
                    return
                if r == 0: do_mod(0, 2 * M)
                if r == cfg.get("MODB", NR // 2): do_mod(2 * M, 6 * M)
                if 1 <= r <= NR:
                    for rr in range((r - 1) * PR, r * PR, LR): do_h(rr)
                if r >= 2: proj_q(0, (r - 2) * PR)
            HS = cfg.get("HS", NR)
            if cfg.get("VQ2", 1) and not HL:
                with jax.named_scope("s2_a"):
                    do_mod(0, 2 * M)
                    for r in range(NR):
                        proj_v(0, r * PR)
                        if r < HS:
                            for rr in range(r * PR, (r + 1) * PR, LR): do_h(rr)
                with jax.named_scope("s2_b"):
                    if HS == 0:
                        for rr in range(0, PR * cfg.get("HLEAD", 1), LR): do_h(rr)
                    for r in range(NR):
                        hh_ = (HS if HS > 0 else cfg.get("HLEAD", 1)) + r
                        if HS == 0 and hh_ < NR:
                            for rr in range(hh_ * PR, (hh_ + 1) * PR, LR): do_h(rr)
                        proj_q(0, r * PR)
                        if HS > 0 and hh_ < NR:
                            for rr in range(hh_ * PR, (hh_ + 1) * PR, LR): do_h(rr)
                        if cfg.get("MODS", 1):
                            nt_ = 4 * M // 128
                            a_ = (r * nt_) // NR; b_ = ((r + 1) * nt_) // NR
                            if b_ > a_: do_mod(2 * M + a_ * 128, 2 * M + b_ * 128)
                        elif r == cfg.get("MODB", NR // 2): do_mod(2 * M, 6 * M)
            else:
                BV = cfg.get("BARV", 99)
                for r0_ in range(0, NR + 2, BV):
                    with jax.named_scope("vq%d" % r0_):
                        for r in range(r0_, min(NR + 2, r0_ + BV)): vstep(r)

        for d in late[0:0]: d.start()
        def body(g, carry):
            bs = g & 1
            ws = 1 - bs
            for d in wcopies(jnp.minimum(g + 2, NP - 1), bs): d.start()
            with sc_("sj_wait"):
                for d in wcopies(g + 1, ws): d.wait()
            with sc_("sk_relay"):
                relayout(wv32.at[ws], wv_s); relayout_q(wq32.at[ws])
            npieces = S // PR
            its = items_rev if cfg.get("REV", 1) == 1 else ([(hh, i) for hh in range(2) for i in range(NI)] if cfg.get("REV") == 0 else
                  [(0, i) for i in reversed(range(NI))] + [(1, i) for i in range(NI)])
            every = len(items_rev) // npieces
            pieces = {}
            for k in range(npieces):
                pieces[k * every + cfg.get("POFF", 1)] = [functools.partial(proj_v, ws, k * PR), functools.partial(proj_q, ws, k * PR)]
            with sc_("si_iter"):
                attention(bs, g, its, pieces)
            return carry
        with sc_("s5_main"):
            jax.lax.fori_loop(0, NP - 1, body, 0)
        for d in wcopies(NP - 1, (NP - 2) % 2): d.wait()

        for d in late: d.wait()
        zero8 = jnp.zeros((8, M), f32)
        u_v[0:8, :] = zero8; u_v[8 + S:16 + S, :] = zero8
        def modv(j): return mod_v[0:1, j * M:(j + 1) * M]

        def A1(r, slot):
            r0 = pl.multiple_of(r * TM, TM)
            if "c" in U32:
                r0h = pl.multiple_of(r * (TM // 2), TM // 2)
                cx = jnp.concatenate([ld_(ctx_v[hh, pl.ds(r0h, TM // 2), :], "c") for hh in range(H)], axis=1)
            else:
                cx = jnp.concatenate([ctx_v[hh, pl.ds(r0, TM), :] for hh in range(H)], axis=1)
            return _dot(cx, ld_(wo_v[...], "W"))

        def A2(r, slot, a):
            r0 = pl.multiple_of(r * TM, TM)
            outs = []
            for rr in range(0, TM, LR):
                x1 = x_v[pl.ds(r0 + rr, LR), :].astype(f32) + modv(2) * a[rr:rr + LR]
                h2 = _ln(x1) * (1.0 + modv(4)) + modv(3)
                x1_v[slot, rr:rr + LR, :] = x1; h2_v[slot, rr:rr + LR, :] = h2
                outs.append(_ln(h2).astype(bf16))
            return jnp.concatenate(outs, axis=0)

        def A3(r, slot, l2):
            r0 = pl.multiple_of(r * TM, TM)
            u_v[pl.ds(r0 + 8, TM), :] = _gelu(_dot(l2, ld_(w1_v[...], "W")))

        def B1(r, slot, ro=0, n=TM):
            r0 = pl.multiple_of(r * TM, TM) + ro
            lane = jax.lax.broadcasted_iota(jnp.int32, (n, 128), 1)
            def sh(delta, j):
                win = u_v[pl.ds(r0, n + 16), j * 128:(j + 1) * 128]
                return win[8 + delta:8 + delta + n]
            t0 = sh(-1, 0)
            t1 = jnp.where(lane < 32, sh(-1, 1), sh(1, 1))
            t2 = jnp.where(lane < 64, sh(1, 2), sh(-2, 2))
            t3 = jnp.where(lane < 96, sh(-2, 3), sh(2, 3))
            t4 = sh(2, 4)
            return jnp.concatenate([t0, t1, t2, t3, t4], axis=1).astype(bf16)

        def B2(r, slot, us):
            return _dot(us, ld_(w2_v[...], "W"))

        def B3(r, slot, hs, ro=0, n=TM):
            outs = []
            for rr in range(0, n, LR):
                xb1 = h2_v[slot, ro + rr:ro + rr + LR, :] + hs[rr:rr + LR]
                h2_v[slot, ro + rr:ro + rr + LR, :] = xb1
                outs.append(_ln(xb1).astype(bf16))
            return jnp.concatenate(outs, axis=0)

        def B4(r, slot, l3):
            return _gelu(jax.lax.dot_general(l3, ld_(w3_v[...], "W"), (((1,), (1,)), ((), ())), preferred_element_type=f32)).astype(bf16)

        def B5(r, slot, gg, osl, ro=0, n=TM):
            y = _dot(gg, ld_(w4_v[...], "W"))
            o_v[osl, ro:ro + n, :] = (x1_v[slot, ro:ro + n, :] + modv(5) * (h2_v[slot, ro:ro + n, :] + y)).astype(bf16)

        def ocopy(r, slot):
            r0 = pl.multiple_of(r * TM, TM)
            return pltpu.make_async_copy(o_v.at[slot], out_hbm.at[pl.ds(r0, TM)], osem.at[slot])

        with sc_("s6_attn_last"):
            nf = 2 * TM // TQ
            items = [(hh, i) for hh in range(2) for i in range(nf)] + [(hh, i) for hh in range(2) for i in reversed(range(nf, NI))]
            LO = cfg.get("LORD", 0)
            nlead = 0
            if LO == 1:
                lead = [(0, NI - 1)]
            elif LO == 2:
                lead = [(0, NI - 1), (1, NI - 1)]
            elif LO == 3:
                lead = []
            if LO:
                small = [(hh, i) for hh in range(2) for i in reversed(range(nf))]
                if LO == 2:
                    small = [x for p_ in zip([(0, i) for i in reversed(range(nf))], [(1, i) for i in reversed(range(nf))]) for x in p_]
                rest = [(hh, i) for hh in range(2) for i in reversed(range(nf, NI)) if (hh, i) not in lead]
                items = lead + small + rest
                nlead = len(lead)
            st = {}
            n0 = nlead + 2 * nf + cfg.get("A0POS", 1); dd = cfg.get("A0D", 4)
            pieces = {n0: ["flush", lambda: st.__setitem__("a0", A1(0, 0))],
                      n0 + dd: [lambda: st.__setitem__("l0", A2(0, 0, st["a0"]))],
                      n0 + 2 * dd: [lambda: st.__setitem__("a1", A1(1, 1))],
                      n0 + 3 * dd: [lambda: A3(0, 0, st["l0"])],
                      min(n0 + 4 * dd, len(items) - 1): [lambda: A3(1, 1, A2(1, 1, st["a1"]))]}
            assert len(pieces) == 5
            attention((NP - 1) % 2, NP - 1, items, pieces, fk=cfg.get("FKL", 0))

        def fbody(t, sa):
            sb = jnp.where(sa == 2, 0, sa + 1)
            osl = t & 1

            @pl.when(t >= 2)
            def _():
                ocopy(t - 2, osl).wait()
            st = {}
            ops = {
                "B1": lambda: st.__setitem__("us", B1(t, sb)),
                "A1": lambda: st.__setitem__("a", A1(t + 2, sa)),
                "B2": lambda: st.__setitem__("hs", B2(t, sb, st["us"])),
                "A2": lambda: st.__setitem__("l2", A2(t + 2, sa, st["a"])),
                "A3": lambda: A3(t + 2, sa, st["l2"]),
                "B3": lambda: st.__setitem__("l3", B3(t, sb, st["hs"])),
                "B4": lambda: st.__setitem__("gg", B4(t, sb, st["l3"])),
                "B5": lambda: B5(t, sb, st["gg"], osl),
            }
            for name in cfg.get("FORD", "B1 B2 A1 B3 B4 A2 A3 B5").split():
                ops[name]()
            ocopy(t, osl).start()
            return sb
        with sc_("s8_floop"):
            jax.lax.fori_loop(0, NB - 2, fbody, 2)
        with sc_("s9_Blast"):
            ocopy(NB - 4, 0).wait(); ocopy(NB - 3, 1).wait()
            rs2 = (NB - 2, NB - 1)
            hs = [B2(r, r % 3, B1(r, r % 3)) for r in rs2]
            gg = [B4(r, r % 3, B3(r, r % 3, hs[i])) for i, r in enumerate(rs2)]
            for i, r in enumerate(rs2):
                B5(r, r % 3, gg[i], r & 1)
                ocopy(r, r & 1).start()
        with sc_("sa_outwait"):
            ocopy(NB - 2, 0).wait()
            ocopy(NB - 1, 1).wait()

    return kernel


def build(cfg):
    TM = cfg.get("TM", 256)
    hbm = pl.BlockSpec(memory_space=pltpu.MemorySpace.HBM)
    def hv(shape, key):
        if key in cfg.get("U32", ""):
            return pltpu.VMEM(shape[:-2] + (shape[-2] // 2, shape[-1]), jnp.uint32)
        return pltpu.VMEM(shape, bf16)
    scratch = [
        pltpu.VMEM((S, M), bf16),
        hv((S, DC), "C"),
        hv((S, M), "h"),
        pltpu.VMEM((M, 6 * M), bf16),
        pltpu.VMEM((8, 6 * M), f32),
        pltpu.VMEM((2, M, D), jnp.uint32),
        pltpu.VMEM((NP, DC, D), jnp.uint32),
        pltpu.VMEM((2, DC, D), jnp.uint32),
        hv((M, 256), "w"), hv((max(2, cfg.get("KPI", 3)), DC, 256), "w"), hv((DC, 256), "w"),
        hv((2, 2, S, D), "q"),
        hv((H, S // 128, D, 128), "k"),
        hv((2, 2, S, D), "v"),
        hv((H + (5 if cfg.get("AL") else 0), S, D), "c"),
        hv((H * D, M), "W"),
        hv((M, M), "W"), hv((M, M), "W"), hv((F, M), "W"), hv((F, M), "W"),
        pltpu.VMEM((S + 16, M), f32),
        pltpu.VMEM((3, TM, M), f32), pltpu.VMEM((3, TM, M), f32), pltpu.VMEM((2, TM, M), bf16),
        pltpu.SemaphoreType.DMA((16,)), pltpu.SemaphoreType.DMA((NP,)), pltpu.SemaphoreType.DMA((2, 2)), pltpu.SemaphoreType.DMA((2,)), pltpu.SemaphoreType.DMA((4,)), pltpu.SMEM((1,), jnp.int32),
    ]
    sd = dict(zip(SCR_NAMES, scratch))
    assert len(scratch) == len(SCR_NAMES)
    scratch = [sd[n] if n in sd else pltpu.VMEM((8 * int(n.split("_")[1]), 128), f32) for n in scratch_order(cfg)]
    return pl.pallas_call(
        make_kernel(cfg),
        out_shape=jax.ShapeDtypeStruct((S, M), bf16),
        in_specs=[hbm] * 10 + [pl.BlockSpec(memory_space=pltpu.VMEM), hbm],
        out_specs=hbm,
        scratch_shapes=scratch,
        compiler_params=pltpu.CompilerParams(vmem_limit_bytes=cfg.get("VMEM", 120) * 2**20),
        name="fused_block",
    )


def run(cfg, A_x, A_c_kv, A_w_q, A_w_uk, A_w_uv, A_w_o, B_x, B_w1, B_w2, B_w3, B_w4, c, w_mod):
    out = build(cfg)(A_x.reshape(S, M), A_c_kv.reshape(S, DC), A_w_q, A_w_uk, A_w_uv, A_w_o.reshape(H * D, M),
                     B_w1, B_w2, B_w3.T, B_w4, c, w_mod)
    return out.reshape(1, S, M)


_CFG = {'U32': 'kvwhCcW', 'ORD': ['ctx_v', 'kT_v'], 'ST': 0, 'NCK': 4, 'A0POS': 2, 'A0D': 4, 'HS': 0, 'FK': 2, 'PR': 256, 'POFF': 1, 'RLP': 4, 'WKE': 3, 'CKB': [0, 1024, 2048], 'FORD': 'B1 B2 B3 A1 B4 A2 B5 A3'}


@jax.jit
def pallas_adaLN_cond__compressed_kv_cla__mixer_s_mlp__prompt_kernel(A_x, A_c_kv, A_w_q, A_w_uk, A_w_uv, A_w_o, B_x, B_w1, B_w2, B_w3, B_w4, c, w_mod):
    return run(_CFG, A_x, A_c_kv, A_w_q, A_w_uk, A_w_uv, A_w_o, B_x, B_w1, B_w2, B_w3, B_w4, c, w_mod)
```

```python
import functools
import jax
import jax.numpy as jnp
import numpy as np
from jax.experimental import pallas as pl
from jax.experimental.pallas import tpu as pltpu

S = 2048; M = 640; H = 32; D = 128; DC = 512; F = 1728
NP = H // 2
EPS = 1e-5
LOG2E = 1.4426950408889634
QSCALE = float(D ** -0.5 * LOG2E)
NEG = -1e30
bf16 = jnp.bfloat16; f32 = jnp.float32


def _ln(x):
    m = jnp.mean(x, axis=-1, keepdims=True)
    xc = x - m
    v = jnp.mean(xc * xc, axis=-1, keepdims=True)
    return xc * jax.lax.rsqrt(v + EPS)


def _gelu(x):
    c = 0.7978845608028654
    return 0.5 * x * (1.0 + jnp.tanh(c * (x + 0.044715 * (x * x * x))))


def _rcp(l):
    r = pl.reciprocal(l, approx=True)
    return r * (2.0 - l * r)


def _dot(a, b):
    return jnp.dot(a, b, preferred_element_type=f32)


def _unpack_pair(w32):
    lo = pltpu.bitcast(w32 << 16, f32).astype(bf16)
    hi = pltpu.bitcast(w32 & jnp.uint32(0xFFFF0000), f32).astype(bf16)
    return lo, hi


SCR_NAMES = ['x_v', 'ckv_v', 'h_v', 'wmod_v', 'mod_v', 'wq32', 'wk32', 'wv32', 'wq_s', 'wk_s', 'wv_s', 'q_v', 'kT_v', 'v_v', 'ctx_v', 'wo_v', 'w1_v', 'w2_v', 'w3_v', 'w4_v', 'u_v', 'x1_v', 'h2_v', 'o_v', 'sem', 'ksem', 'wsem', 'osem', 'fsem', 'zs_ref']


def scratch_order(cfg):
    first = cfg.get("ORD", [])
    last = cfg.get("ORL", [])
    return list(first) + [n for n in SCR_NAMES if n not in first and n not in last] + list(last)


def make_kernel(cfg):
    TQ = 128
    PR = cfg.get("PR", 128)
    TM = cfg.get("TM", 256)
    LR = cfg.get("LR", 64)
    NB = S // TM
    NCK = cfg.get("NCK", 4)
    KPI = cfg.get("KPI", 3); P0 = cfg.get("P0", 1)
    assert (NP - P0) % KPI == 0

    import contextlib
    def sc_(name):
        on = cfg.get("SCOPE")
        if name == "barrier": on = cfg.get("BAR", 1)
        if isinstance(on, str): on = name in on.split(",")
        return jax.named_scope(name) if on else contextlib.nullcontext()

    U32 = cfg.get("U32", "")
    def st_(val, key):
        return pltpu.bitcast(val, jnp.uint32) if key in U32 else val
    def ld_(val, key):
        return pltpu.bitcast(val, bf16) if key in U32 else val
    def rs_(r0, n, key):
        return slice(r0 // 2, (r0 + n) // 2) if key in U32 else slice(r0, r0 + n)

    def kernel(x_hbm, ckv_hbm, wq_hbm, wuk_hbm, wuv_hbm, wo_hbm, w1_hbm, w2_hbm, w3_hbm, w4_hbm, c_ref, wmod_hbm,
               out_hbm, *scr):
        R = dict(zip(scratch_order(cfg), scr))
        (x_v, ckv_v, h_v, wmod_v, mod_v, wq32, wk32, wv32, wq_s, wk_s, wv_s, q_v, kT_v, v_v, ctx_v, wo_v, w1_v, w2_v, w3_v, w4_v, u_v, x1_v, h2_v, o_v, sem, ksem, wsem, osem, fsem, zs_ref) = [R[n] for n in SCR_NAMES]
        def cp(src, dst, i):
            return pltpu.make_async_copy(src, dst, sem.at[i])

        def wkcopy(g):
            return pltpu.make_async_copy(wuk_hbm.bitcast(jnp.uint32).at[:, g, :], wk32.at[g], ksem.at[g])

        def wcopies(g, slot):
            return (pltpu.make_async_copy(wq_hbm.bitcast(jnp.uint32).at[:, g, :], wq32.at[slot], wsem.at[0, slot]),
                    pltpu.make_async_copy(wuv_hbm.bitcast(jnp.uint32).at[:, g, :], wv32.at[slot], wsem.at[1, slot]))

        CKB = cfg.get("CKB", [S * j // NCK for j in range(NCK + 1)])
        NCK_ = len(CKB) - 1
        if "C" in U32:
            c_ckv = [cp(ckv_hbm.bitcast(jnp.uint32).at[CKB[j] // 2:CKB[j + 1] // 2], ckv_v.at[CKB[j] // 2:CKB[j + 1] // 2], j) for j in range(NCK_)]
        else:
            c_ckv = [cp(ckv_hbm.at[CKB[j]:CKB[j + 1]], ckv_v.at[CKB[j]:CKB[j + 1]], j) for j in range(NCK_)]
        c_x = cp(x_hbm, x_v, 8); c_wmod = cp(wmod_hbm, wmod_v, 9)
        bc_ = (lambda r_: r_.bitcast(jnp.uint32)) if "W" in U32 else (lambda r_: r_)
        late = [cp(bc_(wo_hbm), wo_v, 10), cp(bc_(w1_hbm), w1_v, 11), cp(bc_(w2_hbm), w2_v, 12), cp(bc_(w3_hbm), w3_v, 13), cp(bc_(w4_hbm), w4_v, 14)]
        wkcopy(0).start(); c_ckv[0].start()
        def rest_start():
            for j in range(1, NCK_): c_ckv[j].start()
            for g2 in range(1, P0 + 1): wkcopy(g2).start()
        if not cfg.get("ST"): rest_start()

        AL = cfg.get("AL", "")
        def vref(bs, hh):
            return ctx_v.at[H + 2 * bs + hh] if "v" in AL else v_v.at[bs, hh]
        def wq_load():
            if "c" in AL:
                return jnp.concatenate([ctx_v[H + 4, 0:M, :], ctx_v[H + 4, M:2 * M, :]], axis=1)
            return ld_(wq_s[...], "w")
        def relayout_q(src):
            if "c" in AL:
                lo, hi = _unpack_pair(src[...])
                ctx_v[H + 4, 0:M, :] = lo
                ctx_v[H + 4, M:2 * M, :] = hi
            else:
                relayout(src, wq_s)

        def relayout(src, dst):
            lo, hi = _unpack_pair(src[...])
            dst[:, 0:128] = st_(lo, "w")
            dst[:, 128:256] = st_(hi, "w")

        def proj_k(g, par, r0):
            rows = slice(r0, r0 + PR)
            k = _dot(ld_(ckv_v[rs_(r0, PR, "C"), :], "C"), ld_(wk_s[par], "w"))
            for hh in range(2):
                for t in range(PR // 128):
                    kT_v[2 * g + hh, (r0 // 128) + t] = st_(k[t * 128:(t + 1) * 128, hh * 128:(hh + 1) * 128].T.astype(bf16), "k")

        def proj_v(bs, r0):
            rows = slice(r0, r0 + PR)
            v = _dot(ld_(ckv_v[rs_(r0, PR, "C"), :], "C"), ld_(wv_s[...], "w")).astype(bf16)
            for hh in range(2): vref(bs, hh)[rs_(r0, PR, "v"), :] = st_(v[:, hh * 128:(hh + 1) * 128], "v")

        def proj_q(bs, r0):
            rows = slice(r0, r0 + PR)
            q = (_dot(ld_(h_v[rs_(r0, PR, "h"), :], "h"), wq_load()) * QSCALE).astype(bf16)
            for hh in range(2): q_v[bs, hh, rs_(r0, PR, "q"), :] = st_(q[:, hh * 128:(hh + 1) * 128], "q")

        LAG = cfg.get("LAG", 0)
        nv_ = {}
        def never():
            return nv_["m"]
        tri = jax.lax.broadcasted_iota(jnp.int32, (128, 128), 1) <= jax.lax.broadcasted_iota(jnp.int32, (128, 128), 0)

        def qk(bs, g, hh, i):
            r0 = i * TQ; nt = i + 1
            q = ld_(q_v[bs, hh, rs_(r0, TQ, "q"), :], "q")
            tiles = [_dot(q, ld_(kT_v[(0 if cfg.get("KFIX") else 2 * g) + hh, t], "k")) for t in range(nt)]
            tiles[-1] = jnp.where(tri, tiles[-1], NEG)
            mx = tiles[0]
            for t in tiles[1:]:
                mx = jnp.maximum(mx, t)
            m = jnp.max(mx, axis=1, keepdims=True)
            return tiles, m

        def smpv(bs, g, hh, i, st):
            tiles, m = st
            r0 = i * TQ
            acc = None; ls = None
            FR = cfg.get("FR", 0) if nv_["on"] else 0
            rold = None
            if FR and len(nv_["rq"]) >= FR:
                rold = jnp.broadcast_to(nv_["rq"].pop(0), (TQ, 128))
            for t, s in enumerate(tiles):
                p = jnp.exp2(s - m)
                FK = cfg.get("FK", 0) if nv_["on"] else 0
                pm = p
                if FK == 1 and ls is not None:
                    pm = jnp.where(never(), ls, p)
                ls = p if ls is None else ls + p
                if FK == 2:
                    pm = jnp.where(never(), ls, p) if t > 0 else p
                if rold is not None and t == min(cfg.get("FRT", 0), len(tiles) - 1):
                    pm = jnp.where(never(), rold, pm)
                o = _dot(pm.astype(bf16), ld_(vref(bs, hh)[rs_(t * 128, 128, "v"), :], "v"))
                acc = o if acc is None else acc + o
            if FR:
                rr_ = _rcp(jnp.sum(ls, axis=1, keepdims=True))
                nv_["rq"].append(rr_)
            def fin():
                r = rr_ if FR else _rcp(jnp.sum(ls, axis=1, keepdims=True))
                ctx_v[2 * g + hh, rs_(r0, TQ, "c"), :] = st_((acc * r).astype(bf16), "c")
            return fin

        def attention(bs, g, items, pieces, fk=True):
            nv_["on"] = fk; nv_["rq"] = []
            if cfg.get("FK"):
                sv = mod_v[0:8, 0:128]
                nv_["m"] = jnp.broadcast_to((sv != sv)[0:1], (128, 128))
                nv_["m1"] = jnp.broadcast_to((sv != sv)[0:1, 0:1], (128, 1))
            DEP = cfg.get("DEPM" if fk else "DEPL", 1)
            sts = [qk(bs, g, *items[k]) for k in range(min(DEP, len(items)))]
            pend = []
            for n, it in enumerate(items):
                if n + DEP < len(items): sts.append(qk(bs, g, *items[n + DEP]))
                pend.append(smpv(bs, g, *it, sts.pop(0)))
                if len(pend) > LAG:
                    pend.pop(0)()
                if n in pieces:
                    if pieces[n][0] == "flush":
                        for f in pend: f()
                        pend = []
                    for f in pieces[n]:
                        if f != "flush": f()
            for f in pend: f()

        NI = S // TQ
        items_rev = [(hh, i) for hh in range(2) for i in reversed(range(NI))]


        def do_h(rr, dyn=None):
            rows = slice(rr, rr + LR) if dyn is None else pl.ds(pl.multiple_of(dyn + rr, LR), LR)
            hrows = rs_(rr, LR, "h") if dyn is None else rows
            h_v[hrows, :] = st_((_ln(x_v[rows, :].astype(f32)) * (1.0 + mod_v[0:1, M:2 * M]) + mod_v[0:1, 0:M]).astype(bf16), "h")

        def do_mod(a, b):
            cc = c_ref[...].astype(f32)
            sc = (cc * jax.nn.sigmoid(cc)).astype(bf16)
            mod_v[:, a:b] = _dot(jnp.broadcast_to(sc, (8, M)), wmod_v[:, a:b])

        HL = cfg.get("HL", 0)
        def kpair(g, par, nxt, npar, first=False, extra=None):
            for r in range(S // PR):
                if first and (r * PR) in CKB[:-1] and not (r == 0 and cfg.get("ST") == 2):
                    c_ckv[CKB.index(r * PR)].wait()
                proj_k(g, par, r * PR)
                if r == cfg.get("RLP", (S // PR) // 2):
                    if first:
                        for g2 in range(1, P0 + 1): wkcopy(g2).wait()
                        for g2 in range(P0 + 1, min(NP, P0 + 1 + cfg.get("WKE", 99))): wkcopy(g2).start()
                    relayout(wk32.at[nxt], wk_s.at[npar])
                if first and r == S // PR - 1:
                    for g2 in range(P0 + 1 + cfg.get("WKE", 99), NP): wkcopy(g2).start()
                if extra is not None and r in extra: extra[r]()

        with sc_("s1_kphase"):
          with sc_("s1_wait0"):
            wkcopy(0).wait()
            if cfg.get("ST") == 2: c_ckv[0].wait()
          if cfg.get("ST"): rest_start()
          relayout(wk32.at[0], wk_s.at[(0 - P0) % KPI])
          for g in range(P0):
              ex = {}
              if HL:
                  if g == 1:
                      def st1():
                          c_x.start(); c_wmod.start()
                      ex[0] = st1
                  if g == P0 - 2:
                      def st2():
                          for d in wcopies(0, 0): d.start()
                          for d in wcopies(1, 1): d.start()
                      ex[0] = st2
                  if g == P0 - 1:
                      def m1():
                          c_wmod.wait(); do_mod(0, 2 * M)
                      ex[2] = m1
                      ex[9] = lambda: do_mod(2 * M, 4 * M)
                      def m3():
                          do_mod(4 * M, 6 * M); c_x.wait()
                      ex[13] = m3
              kpair(g, (g - P0) % KPI, g + 1, (g + 1 - P0) % KPI, first=(g == 0), extra=ex)

          def kbody(j, carry):
            g = P0 + KPI * j
            c_g = [pltpu.make_async_copy(wuk_hbm.bitcast(jnp.uint32).at[:, jnp.minimum(g + k, NP - 1), :], wk32.at[jnp.minimum(g + k, NP - 1)],
                                         ksem.at[jnp.minimum(g + k, NP - 1)]) for k in range(1, KPI + 1)]
            for k in range(KPI - 1): c_g[k].wait()

            @pl.when(g + KPI < NP)
            def _():
                c_g[KPI - 1].wait()

            if not HL:
                @pl.when(j == cfg.get("XJ", 0))
                def _():
                    c_x.start(); c_wmod.start()
                    for d in wcopies(0, 0): d.start()
                    for d in wcopies(1, 1): d.start()
            NIT_ = (NP - P0) // KPI
            HR = S // NIT_
            nch = HR // LR
            with sc_("barrier"):
              for k in range(KPI):
                ex = {}
                if HL:
                    NR_ = S // PR
                    for ci in range(nch):
                        pos = (ci * KPI * NR_) // nch + 1
                        if pos // NR_ == k:
                            ex[pos % NR_] = functools.partial(do_h, ci * LR, j * HR)
                kpair(g + k, k, jnp.minimum(g + k + 1, NP - 1), (k + 1) % KPI, extra=ex)
            return carry
          with sc_("s1_kloop"):
            jax.lax.fori_loop(0, (NP - P0) // KPI, kbody, 0)

        with sc_("s2_vq0"):
            for d in wcopies(0, 0): d.wait()
            if not HL:
                c_x.wait(); c_wmod.wait()
            for d in late: d.start()
            relayout(wv32.at[0], wv_s); relayout_q(wq32.at[0])
            NR = S // PR
            def vstep(r):
                if r < NR: proj_v(0, r * PR)
                if HL:
                    if r < NR: proj_q(0, r * PR)
                    return
                if r == 0: do_mod(0, 2 * M)
                if r == cfg.get("MODB", NR // 2): do_mod(2 * M, 6 * M)
                if 1 <= r <= NR:
                    for rr in range((r - 1) * PR, r * PR, LR): do_h(rr)
                if r >= 2: proj_q(0, (r - 2) * PR)
            HS = cfg.get("HS", NR)
            if cfg.get("VQ2", 1) and not HL:
                with jax.named_scope("s2_a"):
                    do_mod(0, 2 * M)
                    for r in range(NR):
                        proj_v(0, r * PR)
                        if r < HS:
                            for rr in range(r * PR, (r + 1) * PR, LR): do_h(rr)
                with jax.named_scope("s2_b"):
                    if HS == 0:
                        for rr in range(0, PR * cfg.get("HLEAD", 1), LR): do_h(rr)
                    for r in range(NR):
                        hh_ = (HS if HS > 0 else cfg.get("HLEAD", 1)) + r
                        if HS == 0 and hh_ < NR:
                            for rr in range(hh_ * PR, (hh_ + 1) * PR, LR): do_h(rr)
                        proj_q(0, r * PR)
                        if HS > 0 and hh_ < NR:
                            for rr in range(hh_ * PR, (hh_ + 1) * PR, LR): do_h(rr)
                        if cfg.get("MODS", 1):
                            nt_ = 4 * M // 128
                            a_ = (r * nt_) // NR; b_ = ((r + 1) * nt_) // NR
                            if b_ > a_: do_mod(2 * M + a_ * 128, 2 * M + b_ * 128)
                        elif r == cfg.get("MODB", NR // 2): do_mod(2 * M, 6 * M)
            else:
                BV = cfg.get("BARV", 99)
                for r0_ in range(0, NR + 2, BV):
                    with jax.named_scope("vq%d" % r0_):
                        for r in range(r0_, min(NR + 2, r0_ + BV)): vstep(r)

        for d in late[0:0]: d.start()
        def body(g, carry):
            bs = g & 1
            ws = 1 - bs
            for d in wcopies(jnp.minimum(g + 2, NP - 1), bs): d.start()
            with sc_("sj_wait"):
                for d in wcopies(g + 1, ws): d.wait()
            with sc_("sk_relay"):
                relayout(wv32.at[ws], wv_s); relayout_q(wq32.at[ws])
            npieces = S // PR
            its = items_rev if cfg.get("REV", 1) == 1 else ([(hh, i) for hh in range(2) for i in range(NI)] if cfg.get("REV") == 0 else
                  [(0, i) for i in reversed(range(NI))] + [(1, i) for i in range(NI)])
            every = len(items_rev) // npieces
            pieces = {}
            for k in range(npieces):
                if "VQ" in cfg:
                    pieces.setdefault(k * every + cfg["VQ"][0], []).append(functools.partial(proj_v, ws, k * PR))
                    pieces.setdefault(k * every + cfg["VQ"][1], []).append(functools.partial(proj_q, ws, k * PR))
                    continue
                pieces[k * every + cfg.get("POFF", 1)] = [functools.partial(proj_v, ws, k * PR), functools.partial(proj_q, ws, k * PR)]
            with sc_("si_iter"):
                attention(bs, g, its, pieces)
            return carry
        with sc_("s5_main"):
            jax.lax.fori_loop(0, NP - 1, body, 0)
        for d in wcopies(NP - 1, (NP - 2) % 2): d.wait()

        for d in late: d.wait()
        zero8 = jnp.zeros((8, M), f32)
        u_v[0:8, :] = zero8; u_v[8 + S:16 + S, :] = zero8
        def modv(j): return mod_v[0:1, j * M:(j + 1) * M]

        def A1(r, slot):
            r0 = pl.multiple_of(r * TM, TM)
            if "c" in U32:
                r0h = pl.multiple_of(r * (TM // 2), TM // 2)
                cx = jnp.concatenate([ld_(ctx_v[hh, pl.ds(r0h, TM // 2), :], "c") for hh in range(H)], axis=1)
            else:
                cx = jnp.concatenate([ctx_v[hh, pl.ds(r0, TM), :] for hh in range(H)], axis=1)
            return _dot(cx, ld_(wo_v[...], "W"))

        def A2(r, slot, a):
            r0 = pl.multiple_of(r * TM, TM)
            outs = []
            for rr in range(0, TM, LR):
                x1 = x_v[pl.ds(r0 + rr, LR), :].astype(f32) + modv(2) * a[rr:rr + LR]
                h2 = _ln(x1) * (1.0 + modv(4)) + modv(3)
                x1_v[slot, rr:rr + LR, :] = x1; h2_v[slot, rr:rr + LR, :] = h2
                outs.append(_ln(h2).astype(bf16))
            return jnp.concatenate(outs, axis=0)

        def A3(r, slot, l2):
            r0 = pl.multiple_of(r * TM, TM)
            u_v[pl.ds(r0 + 8, TM), :] = _gelu(_dot(l2, ld_(w1_v[...], "W")))

        def B1(r, slot, ro=0, n=TM):
            r0 = pl.multiple_of(r * TM, TM) + ro
            lane = jax.lax.broadcasted_iota(jnp.int32, (n, 128), 1)
            def sh(delta, j):
                win = u_v[pl.ds(r0, n + 16), j * 128:(j + 1) * 128]
                return win[8 + delta:8 + delta + n]
            t0 = sh(-1, 0)
            t1 = jnp.where(lane < 32, sh(-1, 1), sh(1, 1))
            t2 = jnp.where(lane < 64, sh(1, 2), sh(-2, 2))
            t3 = jnp.where(lane < 96, sh(-2, 3), sh(2, 3))
            t4 = sh(2, 4)
            return jnp.concatenate([t0, t1, t2, t3, t4], axis=1).astype(bf16)

        def B2(r, slot, us):
            return _dot(us, ld_(w2_v[...], "W"))

        def B3(r, slot, hs, ro=0, n=TM):
            outs = []
            for rr in range(0, n, LR):
                xb1 = h2_v[slot, ro + rr:ro + rr + LR, :] + hs[rr:rr + LR]
                h2_v[slot, ro + rr:ro + rr + LR, :] = xb1
                outs.append(_ln(xb1).astype(bf16))
            return jnp.concatenate(outs, axis=0)

        def B4(r, slot, l3):
            return _gelu(jax.lax.dot_general(l3, ld_(w3_v[...], "W"), (((1,), (1,)), ((), ())), preferred_element_type=f32)).astype(bf16)

        def B5(r, slot, gg, osl, ro=0, n=TM):
            y = _dot(gg, ld_(w4_v[...], "W"))
            o_v[osl, ro:ro + n, :] = (x1_v[slot, ro:ro + n, :] + modv(5) * (h2_v[slot, ro:ro + n, :] + y)).astype(bf16)

        def ocopy(r, slot):
            r0 = pl.multiple_of(r * TM, TM)
            return pltpu.make_async_copy(o_v.at[slot], out_hbm.at[pl.ds(r0, TM)], osem.at[slot])

        with sc_("s6_attn_last"):
            nf = 2 * TM // TQ
            items = [(hh, i) for hh in range(2) for i in range(nf)] + [(hh, i) for hh in range(2) for i in reversed(range(nf, NI))]
            LO = cfg.get("LORD", 0)
            nlead = 0
            if LO == 1:
                lead = [(0, NI - 1)]
            elif LO == 2:
                lead = [(0, NI - 1), (1, NI - 1)]
            elif LO == 3:
                lead = []
            if LO:
                small = [(hh, i) for hh in range(2) for i in reversed(range(nf))]
                if LO == 2:
                    small = [x for p_ in zip([(0, i) for i in reversed(range(nf))], [(1, i) for i in reversed(range(nf))]) for x in p_]
                rest = [(hh, i) for hh in range(2) for i in reversed(range(nf, NI)) if (hh, i) not in lead]
                items = lead + small + rest
                nlead = len(lead)
            st = {}
            n0 = nlead + 2 * nf + cfg.get("A0POS", 1); dd = cfg.get("A0D", 4)
            pieces = {n0: ["flush", lambda: st.__setitem__("a0", A1(0, 0))],
                      n0 + dd: [lambda: st.__setitem__("l0", A2(0, 0, st["a0"]))],
                      n0 + 2 * dd: [lambda: st.__setitem__("a1", A1(1, 1))],
                      n0 + 3 * dd: [lambda: A3(0, 0, st["l0"])],
                      min(n0 + 4 * dd, len(items) - 1): [lambda: A3(1, 1, A2(1, 1, st["a1"]))]}
            assert len(pieces) == 5
            attention((NP - 1) % 2, NP - 1, items, pieces, fk=cfg.get("FKL", 0))

        def fbody(t, sa):
            sb = jnp.where(sa == 2, 0, sa + 1)
            osl = t & 1

            @pl.when(t >= 2)
            def _():
                ocopy(t - 2, osl).wait()
            st = {}
            ops = {
                "B1": lambda: st.__setitem__("us", B1(t, sb)),
                "A1": lambda: st.__setitem__("a", A1(t + 2, sa)),
                "B2": lambda: st.__setitem__("hs", B2(t, sb, st["us"])),
                "A2": lambda: st.__setitem__("l2", A2(t + 2, sa, st["a"])),
                "A3": lambda: A3(t + 2, sa, st["l2"]),
                "B3": lambda: st.__setitem__("l3", B3(t, sb, st["hs"])),
                "B4": lambda: st.__setitem__("gg", B4(t, sb, st["l3"])),
                "B5": lambda: B5(t, sb, st["gg"], osl),
            }
            for name in cfg.get("FORD", "B1 B2 A1 B3 B4 A2 A3 B5").split():
                ops[name]()
            ocopy(t, osl).start()
            return sb
        with sc_("s8_floop"):
            jax.lax.fori_loop(0, NB - 2, fbody, 2)
        with sc_("s9_Blast"):
            ocopy(NB - 4, 0).wait(); ocopy(NB - 3, 1).wait()
            rs2 = (NB - 2, NB - 1)
            hs = [B2(r, r % 3, B1(r, r % 3)) for r in rs2]
            gg = [B4(r, r % 3, B3(r, r % 3, hs[i])) for i, r in enumerate(rs2)]
            for i, r in enumerate(rs2):
                B5(r, r % 3, gg[i], r & 1)
                ocopy(r, r & 1).start()
        with sc_("sa_outwait"):
            ocopy(NB - 2, 0).wait()
            ocopy(NB - 1, 1).wait()

    return kernel


def build(cfg):
    TM = cfg.get("TM", 256)
    hbm = pl.BlockSpec(memory_space=pltpu.MemorySpace.HBM)
    def hv(shape, key):
        if key in cfg.get("U32", ""):
            return pltpu.VMEM(shape[:-2] + (shape[-2] // 2, shape[-1]), jnp.uint32)
        return pltpu.VMEM(shape, bf16)
    scratch = [
        pltpu.VMEM((S, M), bf16),
        hv((S, DC), "C"),
        hv((S, M), "h"),
        pltpu.VMEM((M, 6 * M), bf16),
        pltpu.VMEM((8, 6 * M), f32),
        pltpu.VMEM((2, M, D), jnp.uint32),
        pltpu.VMEM((NP, DC, D), jnp.uint32),
        pltpu.VMEM((2, DC, D), jnp.uint32),
        hv((M, 256), "w"), hv((max(2, cfg.get("KPI", 3)), DC, 256), "w"), hv((DC, 256), "w"),
        hv((2, 2, S, D), "q"),
        hv((H, S // 128, D, 128), "k"),
        hv((2, 2, S, D), "v"),
        hv((H + (5 if cfg.get("AL") else 0), S, D), "c"),
        hv((H * D, M), "W"),
        hv((M, M), "W"), hv((M, M), "W"), hv((F, M), "W"), hv((F, M), "W"),
        pltpu.VMEM((S + 16, M), f32),
        pltpu.VMEM((3, TM, M), f32), pltpu.VMEM((3, TM, M), f32), pltpu.VMEM((2, TM, M), bf16),
        pltpu.SemaphoreType.DMA((16,)), pltpu.SemaphoreType.DMA((NP,)), pltpu.SemaphoreType.DMA((2, 2)), pltpu.SemaphoreType.DMA((2,)), pltpu.SemaphoreType.DMA((4,)), pltpu.SMEM((1,), jnp.int32),
    ]
    sd = dict(zip(SCR_NAMES, scratch))
    assert len(scratch) == len(SCR_NAMES)
    scratch = [sd[n] if n in sd else pltpu.VMEM((8 * int(n.split("_")[1]), 128), f32) for n in scratch_order(cfg)]
    return pl.pallas_call(
        make_kernel(cfg),
        out_shape=jax.ShapeDtypeStruct((S, M), bf16),
        in_specs=[hbm] * 10 + [pl.BlockSpec(memory_space=pltpu.VMEM), hbm],
        out_specs=hbm,
        scratch_shapes=scratch,
        compiler_params=pltpu.CompilerParams(vmem_limit_bytes=cfg.get("VMEM", 120) * 2**20),
        name="fused_block",
    )


def run(cfg, A_x, A_c_kv, A_w_q, A_w_uk, A_w_uv, A_w_o, B_x, B_w1, B_w2, B_w3, B_w4, c, w_mod):
    out = build(cfg)(A_x.reshape(S, M), A_c_kv.reshape(S, DC), A_w_q, A_w_uk, A_w_uv, A_w_o.reshape(H * D, M),
                     B_w1, B_w2, B_w3.T, B_w4, c, w_mod)
    return out.reshape(1, S, M)


_CFG = {'U32': 'kvwhCW', 'ORD': ['ctx_v', 'kT_v'], 'ST': 0, 'NCK': 4, 'A0POS': 2, 'A0D': 4, 'HS': 0, 'FK': 2, 'PR': 256, 'POFF': 1, 'RLP': 4, 'WKE': 3, 'CKB': [0, 1024, 2048], 'FORD': 'B1 B2 B3 A1 B4 A2 B5 A3', 'LR': 256, 'VQ': [2, 1]}


@jax.jit
def pallas_adaLN_cond__compressed_kv_cla__mixer_s_mlp__prompt_kernel(A_x, A_c_kv, A_w_q, A_w_uk, A_w_uv, A_w_o, B_x, B_w1, B_w2, B_w3, B_w4, c, w_mod):
    return run(_CFG, A_x, A_c_kv, A_w_q, A_w_uk, A_w_uv, A_w_o, B_x, B_w1, B_w2, B_w3, B_w4, c, w_mod)
```

```python
import functools

import jax
import jax.numpy as jnp
from jax.experimental import pallas as pl
from jax.experimental.pallas import tpu as pltpu

S = 2048
M = 640
H = 32
D = 128
DC = 512
F = 1728
NP = H // 2
EPS = 1e-5
LOG2E = 1.4426950408889634
QSCALE = float(D ** -0.5 * LOG2E)
NEG = -1e30
TQ = 128
PR = 256
TM = 256
NB = S // TM
NR = S // PR
NI = S // TQ
KPI = 3
CKB = (0, 1024, 2048)
bf16 = jnp.bfloat16
f32 = jnp.float32
u32 = jnp.uint32


def _ln(x):
    m = jnp.mean(x, axis=-1, keepdims=True)
    xc = x - m
    v = jnp.mean(xc * xc, axis=-1, keepdims=True)
    return xc * jax.lax.rsqrt(v + EPS)


def _gelu(x):
    c = 0.7978845608028654
    return 0.5 * x * (1.0 + jnp.tanh(c * (x + 0.044715 * (x * x * x))))


def _rcp(l):
    r = pl.reciprocal(l, approx=True)
    return r * (2.0 - l * r)


def _dot(a, b):
    return jnp.dot(a, b, preferred_element_type=f32)


def _st(val):
    return pltpu.bitcast(val, u32)


def _ld(val):
    return pltpu.bitcast(val, bf16)


def _unpack_pair(w32):
    lo = pltpu.bitcast(w32 << 16, f32).astype(bf16)
    hi = pltpu.bitcast(w32 & jnp.uint32(0xFFFF0000), f32).astype(bf16)
    return lo, hi


def _kernel(x_hbm, ckv_hbm, wq_hbm, wuk_hbm, wuv_hbm, wo_hbm, w1_hbm, w2_hbm, w3_hbm, w4_hbm, c_ref, wmod_hbm,
            out_hbm,
            ctx_v, kT_v, x_v, ckv_v, h_v, wmod_v, mod_v, wq32, wk32, wv32, wq_s, wk_s, wv_s, q_v, v_v,
            wo_v, w1_v, w2_v, w3_v, w4_v, u_v, x1_v, h2_v, o_v, sem, ksem, wsem, osem):
    def cp(src, dst, i):
        return pltpu.make_async_copy(src, dst, sem.at[i])

    def wkcopy(g):
        return pltpu.make_async_copy(wuk_hbm.bitcast(u32).at[:, g, :], wk32.at[g], ksem.at[g])

    def wcopies(g, slot):
        return (pltpu.make_async_copy(wq_hbm.bitcast(u32).at[:, g, :], wq32.at[slot], wsem.at[0, slot]),
                pltpu.make_async_copy(wuv_hbm.bitcast(u32).at[:, g, :], wv32.at[slot], wsem.at[1, slot]))

    c_ckv = [cp(ckv_hbm.bitcast(u32).at[CKB[j] // 2:CKB[j + 1] // 2], ckv_v.at[CKB[j] // 2:CKB[j + 1] // 2], j)
             for j in range(len(CKB) - 1)]
    c_x = cp(x_hbm, x_v, 8)
    c_wmod = cp(wmod_hbm, wmod_v, 9)
    late = [cp(wo_hbm.bitcast(u32), wo_v, 10), cp(w1_hbm.bitcast(u32), w1_v, 11), cp(w2_hbm.bitcast(u32), w2_v, 12),
            cp(w3_hbm.bitcast(u32), w3_v, 13), cp(w4_hbm.bitcast(u32), w4_v, 14)]
    wkcopy(0).start()
    c_ckv[0].start()
    c_ckv[1].start()
    wkcopy(1).start()

    def half(r0, n):
        return slice(r0 // 2, (r0 + n) // 2)

    def relayout(src, dst):
        lo, hi = _unpack_pair(src[...])
        dst[:, 0:128] = _st(lo)
        dst[:, 128:256] = _st(hi)

    def proj_k(g, par, r0):
        k = _dot(_ld(ckv_v[half(r0, PR), :]), _ld(wk_s[par]))
        for hh in range(2):
            for t in range(PR // 128):
                kT_v[2 * g + hh, (r0 // 128) + t] = _st(k[t * 128:(t + 1) * 128, hh * 128:(hh + 1) * 128].T.astype(bf16))

    def proj_v(bs, r0):
        v = _dot(_ld(ckv_v[half(r0, PR), :]), _ld(wv_s[...])).astype(bf16)
        for hh in range(2):
            v_v[bs, hh, half(r0, PR), :] = _st(v[:, hh * 128:(hh + 1) * 128])

    def proj_q(bs, r0):
        q = (_dot(_ld(h_v[half(r0, PR), :]), _ld(wq_s[...])) * QSCALE).astype(bf16)
        for hh in range(2):
            q_v[bs, hh, r0:r0 + PR, :] = q[:, hh * 128:(hh + 1) * 128]

    tri = jax.lax.broadcasted_iota(jnp.int32, (128, 128), 1) <= jax.lax.broadcasted_iota(jnp.int32, (128, 128), 0)

    def qk(bs, g, hh, i):
        r0 = i * TQ
        q = q_v[bs, hh, r0:r0 + TQ, :]
        tiles = [_dot(q, _ld(kT_v[2 * g + hh, t])) for t in range(i + 1)]
        tiles[-1] = jnp.where(tri, tiles[-1], NEG)
        mx = tiles[0]
        for t in tiles[1:]:
            mx = jnp.maximum(mx, t)
        return tiles, jnp.max(mx, axis=1, keepdims=True)

    def smpv(bs, g, hh, i, st, never):
        tiles, m = st
        r0 = i * TQ
        acc = None
        ls = None
        for t, s in enumerate(tiles):
            p = jnp.exp2(s - m)
            pm = p
            ls = p if ls is None else ls + p
            if never is not None:
                pm = jnp.where(never, ls, p) if t > 0 else p
            o = _dot(pm.astype(bf16), _ld(v_v[bs, hh, half(t * 128, 128), :]))
            acc = o if acc is None else acc + o
        r = _rcp(jnp.sum(ls, axis=1, keepdims=True))
        ctx_v[2 * g + hh, r0:r0 + TQ, :] = (acc * r).astype(bf16)

    def attention(bs, g, items, pieces, steer):
        never = None
        if steer:
            sv = mod_v[0:8, 0:128]
            never = jnp.broadcast_to((sv != sv)[0:1], (128, 128))
        sts = [qk(bs, g, *items[0])]
        for n, it in enumerate(items):
            if n + 1 < len(items):
                sts.append(qk(bs, g, *items[n + 1]))
            smpv(bs, g, *it, sts.pop(0), never)
            for f in pieces.get(n, []):
                f()

    items_rev = [(hh, i) for hh in range(2) for i in reversed(range(NI))]

    def do_h(r0):
        h_v[half(r0, PR), :] = _st((_ln(x_v[r0:r0 + PR, :].astype(f32)) * (1.0 + mod_v[0:1, M:2 * M]) + mod_v[0:1, 0:M]).astype(bf16))

    def do_mod(a, b):
        cc = c_ref[...].astype(f32)
        sc = (cc * jax.nn.sigmoid(cc)).astype(bf16)
        mod_v[:, a:b] = _dot(jnp.broadcast_to(sc, (8, M)), wmod_v[:, a:b])

    def kpair(g, par, nxt, npar, first=False):
        for r in range(NR):
            if first and (r * PR) in CKB[:-1]:
                c_ckv[CKB.index(r * PR)].wait()
            proj_k(g, par, r * PR)
            if r == NR // 2:
                if first:
                    wkcopy(1).wait()
                    for g2 in range(2, 2 + KPI):
                        wkcopy(g2).start()
                relayout(wk32.at[nxt], wk_s.at[npar])
            if first and r == NR - 1:
                for g2 in range(2 + KPI, NP):
                    wkcopy(g2).start()

    wkcopy(0).wait()
    relayout(wk32.at[0], wk_s.at[KPI - 1])
    kpair(0, KPI - 1, 1, 0, first=True)

    def kbody(j, carry):
        g = 1 + KPI * j
        c_g = [wkcopy(jnp.minimum(g + k, NP - 1)) for k in range(1, KPI + 1)]
        for k in range(KPI - 1):
            c_g[k].wait()

        @pl.when(g + KPI < NP)
        def _():
            c_g[KPI - 1].wait()

        @pl.when(j == 0)
        def _():
            c_x.start()
            c_wmod.start()
            for d in wcopies(0, 0):
                d.start()
            for d in wcopies(1, 1):
                d.start()
        with jax.named_scope("k_pairs"):
            for k in range(KPI):
                kpair(g + k, k, jnp.minimum(g + k + 1, NP - 1), (k + 1) % KPI)
        return carry
    jax.lax.fori_loop(0, (NP - 1) // KPI, kbody, 0)

    for d in wcopies(0, 0):
        d.wait()
    c_x.wait()
    c_wmod.wait()
    for d in late:
        d.start()
    relayout(wv32.at[0], wv_s)
    relayout(wq32.at[0], wq_s)
    with jax.named_scope("v0"):
        do_mod(0, 2 * M)
        for r in range(NR):
            proj_v(0, r * PR)
    with jax.named_scope("hq0"):
        do_h(0)
        nt = 4 * M // 128
        for r in range(NR):
            if r + 1 < NR:
                do_h((r + 1) * PR)
            proj_q(0, r * PR)
            a, b = (r * nt) // NR, ((r + 1) * nt) // NR
            if b > a:
                do_mod(2 * M + a * 128, 2 * M + b * 128)

    def body(g, carry):
        bs = g & 1
        ws = 1 - bs
        for d in wcopies(jnp.minimum(g + 2, NP - 1), bs):
            d.start()
        for d in wcopies(g + 1, ws):
            d.wait()
        relayout(wv32.at[ws], wv_s)
        relayout(wq32.at[ws], wq_s)
        every = len(items_rev) // NR
        pieces = {}
        for k in range(NR):
            pieces.setdefault(k * every + 2, []).append(functools.partial(proj_v, ws, k * PR))
            pieces.setdefault(k * every + 1, []).append(functools.partial(proj_q, ws, k * PR))
        attention(bs, g, items_rev, pieces, True)
        return carry
    jax.lax.fori_loop(0, NP - 1, body, 0)
    for d in wcopies(NP - 1, (NP - 2) % 2):
        d.wait()

    for d in late:
        d.wait()
    zero8 = jnp.zeros((8, M), f32)
    u_v[0:8, :] = zero8
    u_v[8 + S:16 + S, :] = zero8

    def modv(j):
        return mod_v[0:1, j * M:(j + 1) * M]

    def A1(r):
        r0 = pl.multiple_of(r * TM, TM)
        cx = jnp.concatenate([ctx_v[hh, pl.ds(r0, TM), :] for hh in range(H)], axis=1)
        return _dot(cx, _ld(wo_v[...]))

    def A2(r, slot, a):
        r0 = pl.multiple_of(r * TM, TM)
        x1 = x_v[pl.ds(r0, TM), :].astype(f32) + modv(2) * a
        h2 = _ln(x1) * (1.0 + modv(4)) + modv(3)
        x1_v[slot] = x1
        h2_v[slot] = h2
        return _ln(h2).astype(bf16)

    def A3(r, l2):
        r0 = pl.multiple_of(r * TM, TM)
        u_v[pl.ds(r0 + 8, TM), :] = _gelu(_dot(l2, _ld(w1_v[...])))

    def B1(r):
        r0 = pl.multiple_of(r * TM, TM)
        lane = jax.lax.broadcasted_iota(jnp.int32, (TM, 128), 1)

        def sh(delta, j):
            win = u_v[pl.ds(r0, TM + 16), j * 128:(j + 1) * 128]
            return win[8 + delta:8 + delta + TM]
        t0 = sh(-1, 0)
        t1 = jnp.where(lane < 32, sh(-1, 1), sh(1, 1))
        t2 = jnp.where(lane < 64, sh(1, 2), sh(-2, 2))
        t3 = jnp.where(lane < 96, sh(-2, 3), sh(2, 3))
        t4 = sh(2, 4)
        return jnp.concatenate([t0, t1, t2, t3, t4], axis=1).astype(bf16)

    def B2(us):
        return _dot(us, _ld(w2_v[...]))

    def B3(slot, hs):
        xb1 = h2_v[slot] + hs
        h2_v[slot] = xb1
        return _ln(xb1).astype(bf16)

    def B4(l3):
        z = jax.lax.dot_general(l3, _ld(w3_v[...]), (((1,), (1,)), ((), ())), preferred_element_type=f32)
        return _gelu(z).astype(bf16)

    def B5(slot, gg, osl):
        y = _dot(gg, _ld(w4_v[...]))
        o_v[osl] = (x1_v[slot] + modv(5) * (h2_v[slot] + y)).astype(bf16)

    def ocopy(r, slot):
        r0 = pl.multiple_of(r * TM, TM)
        return pltpu.make_async_copy(o_v.at[slot], out_hbm.at[pl.ds(r0, TM)], osem.at[slot])

    nf = 2 * TM // TQ
    items = ([(hh, i) for hh in range(2) for i in range(nf)]
             + [(hh, i) for hh in range(2) for i in reversed(range(nf, NI))])
    st = {}
    n0, dd = 2 * nf + 2, 4
    pieces = {n0: [lambda: st.__setitem__("a0", A1(0))],
              n0 + dd: [lambda: st.__setitem__("l0", A2(0, 0, st["a0"]))],
              n0 + 2 * dd: [lambda: st.__setitem__("a1", A1(1))],
              n0 + 3 * dd: [lambda: A3(0, st["l0"])],
              n0 + 4 * dd: [lambda: A3(1, A2(1, 1, st["a1"]))]}
    attention((NP - 1) % 2, NP - 1, items, pieces, False)

    def fbody(t, sa):
        sb = jnp.where(sa == 2, 0, sa + 1)
        osl = t & 1

        @pl.when(t >= 2)
        def _():
            ocopy(t - 2, osl).wait()
        l3 = B3(sb, B2(B1(t)))
        a = A1(t + 2)
        gg = B4(l3)
        l2 = A2(t + 2, sa, a)
        B5(sb, gg, osl)
        A3(t + 2, l2)
        ocopy(t, osl).start()
        return sb
    jax.lax.fori_loop(0, NB - 2, fbody, 2)

    ocopy(NB - 4, 0).wait()
    ocopy(NB - 3, 1).wait()
    last = (NB - 2, NB - 1)
    hs = [B2(B1(r)) for r in last]
    gg = [B4(B3(r % 3, hs[i])) for i, r in enumerate(last)]
    for i, r in enumerate(last):
        B5(r % 3, gg[i], r & 1)
        ocopy(r, r & 1).start()
    ocopy(NB - 2, 0).wait()
    ocopy(NB - 1, 1).wait()


def _pv(shape):
    return pltpu.VMEM(shape[:-2] + (shape[-2] // 2, shape[-1]), u32)


def _call():
    hbm = pl.BlockSpec(memory_space=pltpu.MemorySpace.HBM)
    scratch = [
        pltpu.VMEM((H, S, D), bf16),
        _pv((H, S // 128, D, 128)),
        pltpu.VMEM((S, M), bf16),
        _pv((S, DC)),
        _pv((S, M)),
        pltpu.VMEM((M, 6 * M), bf16),
        pltpu.VMEM((8, 6 * M), f32),
        pltpu.VMEM((2, M, D), u32),
        pltpu.VMEM((NP, DC, D), u32),
        pltpu.VMEM((2, DC, D), u32),
        _pv((M, 256)), _pv((KPI, DC, 256)), _pv((DC, 256)),
        pltpu.VMEM((2, 2, S, D), bf16),
        _pv((2, 2, S, D)),
        _pv((H * D, M)),
        _pv((M, M)), _pv((M, M)), _pv((F, M)), _pv((F, M)),
        pltpu.VMEM((S + 16, M), f32),
        pltpu.VMEM((3, TM, M), f32), pltpu.VMEM((3, TM, M), f32), pltpu.VMEM((2, TM, M), bf16),
        pltpu.SemaphoreType.DMA((16,)), pltpu.SemaphoreType.DMA((NP,)), pltpu.SemaphoreType.DMA((2, 2)),
        pltpu.SemaphoreType.DMA((2,)),
    ]
    return pl.pallas_call(
        _kernel,
        out_shape=jax.ShapeDtypeStruct((S, M), bf16),
        in_specs=[hbm] * 10 + [pl.BlockSpec(memory_space=pltpu.VMEM), hbm],
        out_specs=hbm,
        scratch_shapes=scratch,
        compiler_params=pltpu.CompilerParams(vmem_limit_bytes=120 * 2**20),
        name="fused_block",
    )


@jax.jit
def pallas_adaLN_cond__compressed_kv_cla__mixer_s_mlp__prompt_kernel(
        A_x, A_c_kv, A_w_q, A_w_uk, A_w_uv, A_w_o, B_x, B_w1, B_w2, B_w3, B_w4, c, w_mod):
    del B_x
    out = _call()(A_x.reshape(S, M), A_c_kv.reshape(S, DC), A_w_q, A_w_uk, A_w_uv, A_w_o.reshape(H * D, M),
                  B_w1, B_w2, B_w3.T, B_w4, c, w_mod)
    return out.reshape(1, S, M)
```
